```python
import jax
import jax.numpy as jnp

def _softmax(x, axis=-1):
    return jax.nn.softmax(x, axis=axis)

def _gelu(x):
    return jax.nn.gelu(x, approximate=True)

def _silu(x):
    return jax.nn.silu(x)

def _sigmoid(x):
    return jax.nn.sigmoid(x)

def _layernorm(x, axis=-1, eps=1e-05):
    m = jnp.mean(x, axis=axis, keepdims=True)
    v = jnp.var(x, axis=axis, keepdims=True)
    return (x - m) / jnp.sqrt(v + eps)

def _scatter_add(tgt, idx, src, axis=0):
    return tgt.at[idx].add(src)

def _segment_sum(src, seg, n):
    return jax.ops.segment_sum(src, seg, n)

class _Rng:

    def __init__(self, key):
        self._k = key

    def _next(self):
        self._k, sub = jax.random.split(self._k)
        return sub

    def normal(self, shape):
        return jax.random.normal(self._next(), shape, dtype=jnp.bfloat16)

    def randint(self, lo, hi, shape):
        return jax.random.randint(self._next(), shape, lo, hi, dtype=jnp.int32)

    def uniform(self, shape, lo=0.0, hi=1.0):
        return jax.random.uniform(self._next(), shape, jnp.bfloat16, lo, hi)

    def permutation(self, n):
        return jax.random.permutation(self._next(), n)
kernel_name = 'sequential_preLN__memory_aug_recurrent_mem_tr__mixer_s_mlp__prompt'

def setup_inputs():
    _rng = _Rng(jax.random.key(int.from_bytes(__import__("os").urandom(4), "little")))
    _w = lambda a: (lambda t: t.astype(jnp.bfloat16) if jnp.issubdtype(t.dtype, jnp.floating) else t)(jnp.asarray(a))

    def _A_setup():
        B, S, Dm = (1, 2048, 1024)
        H, Dh = (32, 128)
        M, seg = (8, 32)
        seg = min(seg, S)
        S = S // seg * seg
        return {'x': _w((lambda *s: _rng.normal(s) * 0.05)(B, S, Dm)), 'mem0': _w((lambda *s: _rng.normal(s) * 0.05)(B, M, Dm)), 'Wq': _w((lambda *s: _rng.normal(s) * 0.05)(Dm, H, Dh) * Dm ** (-0.5)), 'Wk': _w((lambda *s: _rng.normal(s) * 0.05)(Dm, H, Dh) * Dm ** (-0.5)), 'Wv': _w((lambda *s: _rng.normal(s) * 0.05)(Dm, H, Dh) * Dm ** (-0.5)), 'Wo': _w((lambda *s: _rng.normal(s) * 0.05)(H, Dh, Dm) * (H * Dh) ** (-0.5)), 'seg_len': seg}
    _A_in = _A_setup()

    def _B_setup():
        B, S, D, F = (1, 2048, 1024, 3584)
        return {'x': _w((lambda *s: _rng.normal(s) * 0.05)(B, S, D)), 'w1': _w((lambda *s: _rng.normal(s) * 0.05)(D, D) * D ** (-0.5)), 'w2': _w((lambda *s: _rng.normal(s) * 0.05)(D, D) * D ** (-0.5)), 'w3': _w((lambda *s: _rng.normal(s) * 0.05)(D, F) * D ** (-0.5)), 'w4': _w((lambda *s: _rng.normal(s) * 0.05)(F, D) * F ** (-0.5))}
    _B_in = _B_setup()
    return {'A_x': _A_in['x'], 'A_mem0': _A_in['mem0'], 'A_Wq': _A_in['Wq'], 'A_Wk': _A_in['Wk'], 'A_Wv': _A_in['Wv'], 'A_Wo': _A_in['Wo'], 'A_seg_len': _A_in['seg_len'], 'B_x': _B_in['x'], 'B_w1': _B_in['w1'], 'B_w2': _B_in['w2'], 'B_w3': _B_in['w3'], 'B_w4': _B_in['w4']}

def reference(A_x, A_mem0, A_Wq, A_Wk, A_Wv, A_Wo, A_seg_len, B_x, B_w1, B_w2, B_w3, B_w4):

    def _A_ref(x, mem0, Wq, Wk, Wv, Wo, seg_len):
        B, S, Dm = x.shape
        H, Dh = (Wq.shape[1], Wq.shape[2])
        M = mem0.shape[1]
        scale = Dh ** (-0.5)
        n_seg = S // seg_len
        L = M + seg_len
        idx = jnp.arange(L)
        mask = (idx[:, None] < M) | (idx[:, None] >= idx[None, :])
        mem = mem0
        outs = []
        for s in range(n_seg):
            xs = x[:, s * seg_len:(s + 1) * seg_len, :].copy()
            h = jnp.concatenate([mem, xs], axis=1)
            q = jnp.einsum('btd,dhe->bhte', h, Wq)
            k = jnp.einsum('btd,dhe->bhte', h, Wk)
            v = jnp.einsum('btd,dhe->bhte', h, Wv)
            scores = jnp.einsum('bhqe,bhke->bhqk', q, k) * scale
            scores = jnp.where(mask[None, None], scores, -1000000000.0)
            p = _softmax(scores, axis=-1)
            o = jnp.einsum('bhqk,bhke->bhqe', p, v)
            o = jnp.einsum('bhte,hed->btd', o, Wo)
            mem = o[:, :M, :].copy()
            outs.append(o[:, M:, :])
        return jnp.concatenate(outs, axis=1)

    def _B_ref(x, w1, w2, w3, w4):
        B, S, D = x.shape
        h = _gelu(_layernorm(x, axis=-1) @ w1)
        c = D // 4
        g0 = jnp.pad(h[:, :, 0 * c:1 * c], ((0, 0), (1, 0), (0, 0)))[:, :S, :]
        g1 = jnp.pad(h[:, :, 1 * c:2 * c], ((0, 0), (0, 1), (0, 0)))[:, 1:, :]
        g2 = jnp.pad(h[:, :, 2 * c:3 * c], ((0, 0), (2, 0), (0, 0)))[:, :S, :]
        g3 = jnp.pad(h[:, :, 3 * c:], ((0, 0), (0, 2), (0, 0)))[:, 2:, :]
        hs = jnp.concatenate([g0, g1, g2, g3], axis=-1) @ w2
        x1 = x + hs
        h2 = _gelu(_layernorm(x1, axis=-1) @ w3) @ w4
        return x1 + h2
    x = A_x
    h = x + _A_ref(_layernorm(x, axis=-1), A_mem0, A_Wq, A_Wk, A_Wv, A_Wo, A_seg_len)
    h2 = h + _B_ref(_layernorm(h, axis=-1), B_w1, B_w2, B_w3, B_w4)
    return h2
```

```python
import functools
import itertools

import jax
import jax.numpy as jnp
from jax import lax
import jax.experimental.pallas as pl
import jax.experimental.pallas.tpu as pltpu

S = 2048
D = 1024
H = 32
DH = 128
MEM = 8
SEG = 32
F = 3584
NSEG = S // SEG
NP = H // 2
HD = D // 2
C4 = D // 4
F4 = F // 4
HALO = 8
R = 64
RB = 4 * R
NB = S // RB
EPS = 1e-5
NEG = -1000000000.0

W1_AT, W2_AT, W3_AT, W4_AT = 0, 2 * C4, 4 * C4, 11 * C4
WROWS = W4_AT + 2 * F4
NSTRIP = 13

LAG_QK, LAG_PV, LAG_WO = 2, 4, 5
FILL = (17, 19, 99)

bf16 = jnp.bfloat16
f32 = jnp.float32
u32 = jnp.uint32

SEM_XP, SEM_X, SEM_WO, SEM_STRIP, SEM_OUT, SEM_W = 0, 1, 3, 7, 9, 9 + 2 * NB
NSEM = SEM_W + 12


def _mult(i, n):
    return i if isinstance(i, int) else pl.multiple_of(i, n)


def _ln_stats(x):
    m = jnp.mean(x, axis=-1, keepdims=True)
    d = x - m
    v = jnp.mean(d * d, axis=-1, keepdims=True)
    return m, lax.rsqrt(v + EPS)


def _ln(x):
    m, r = _ln_stats(x)
    return (x - m) * r


def _gelu_of_double(y):
    c = 0.7978845608028654
    return y + y * jnp.tanh(y * (2 * c + (8 * c * 0.044715) * (y * y)))


def _dot(a, b):
    return jnp.dot(a, b, preferred_element_type=f32)


def _load(ref, *idx, r0=0, n=None):
    n = ref.shape[-2] if n is None else n
    return pltpu.bitcast(
        ref.bitcast(u32)[(*idx, pl.ds(_mult(r0 // 2, 8), n // 2), slice(None))], bf16)


def _sums_a(a11, a12, a21, a22):
    return [lambda: a12 - a22, lambda: a11 + a12, lambda: a11, lambda: a11 + a22,
            lambda: a22, lambda: a21 + a22, lambda: a21 - a11]


def _sums_b(b11, b12, b21, b22):
    return [lambda: b21 + b22, lambda: b22, lambda: b12 - b22, lambda: b11 + b22,
            lambda: b21 - b11, lambda: b11, lambda: b11 + b12]


def _combine(product, emit):
    c11 = product(0)
    c12 = product(1)
    c11 = c11 - c12
    c22 = product(2)
    emit(0, 1, c12 + c22)
    t = product(3)
    c11 = c11 + t
    c22 = c22 + t
    c21 = product(4)
    emit(0, 0, c11 + c21)
    t = product(5)
    emit(1, 0, c21 + t)
    c22 = c22 - t
    emit(1, 1, c22 + product(6))


def _sums2(sums, x, emit):
    outer = [sums(x[i][j], x[i][2 + j], x[2 + i][j], x[2 + i][2 + j])
             for i in range(2) for j in range(2)]
    for p in range(7):
        for q, v in enumerate(sums(*(o[p]() for o in outer))):
            emit(7 * p + q, v)
        yield


def _spread(tasks, pieces, slots):
    todo = itertools.chain(*tasks)
    calls = itertools.count(1)

    def advance():
        k = next(calls)
        for _ in range(pieces * k // slots - pieces * (k - 1) // slots):
            next(todo)
        if k == slots:
            assert next(todo, "done") == "done"
    return advance


def _upper_operands(a11, a12, a22):
    k = a11.shape[0] - a22.shape[0]
    ops = [jnp.concatenate([a12[:k], a12[k:] - a22], axis=0), a11 + a12, a11,
           jnp.concatenate([a11[:k], a11[k:] + a22], axis=0)]
    return [v.astype(bf16) for v in ops]


PLAIN = {40: 0, 36: 1, 12: 2, 8: 3}
OTHER = [n for n in range(49) if n not in PLAIN]
RAW_SLOT = dict(zip(OTHER[2::3], [(k, j) for k in range(4) for j in range(4) if k != j]))
RAW_SLOT.update({n: (k, k) for n, k in PLAIN.items()})


def _kernel(x_hbm, mem0_ref, wq_hbm, wk_hbm, wv_hbm, wo_hbm, w1_hbm, w2_hbm,
            w3_hbm, w4_hbm, out_hbm, hbuf, hstat, sems, zero_ref, *wbufs):
    zero_ref[0] = 0
    raw, spare = wbufs[:4], wbufs[4:]
    wsum = {n: (raw[j], k) for n, (k, j) in RAW_SLOT.items()}
    wsum.update({n: (b,) for n, b in zip((n for n in OTHER if n not in RAW_SLOT), spare)})

    def load_h(rows):
        return jnp.concatenate([hbuf[c, rows, :] for c in range(8)], axis=1)

    def h_stats(r0):
        rows = pl.ds(_mult(r0, 16), 16)
        hv = load_h(rows)
        m1, r1 = _ln_stats(hv)
        m2, r2 = _ln_stats((hv - m1) * r1)
        for k, v in enumerate((m1 + m2 / r1, r1, 0.5 * r1 * r2)):
            hstat[k, rows, :] = jnp.broadcast_to(v, (16, 128))
        yield

    def strip_copies(u, fn):
        for lo, hi, w, at in ((0, 2, w1_hbm, W1_AT), (2, 4, w2_hbm, W2_AT),
                              (4, 11, w3_hbm, W3_AT), (11, 13, w4_hbm, W4_AT)):
            def run(lo=lo, w=w, at=at):
                n = w.shape[1]
                for j in range(4):
                    cols = pl.ds(_mult(j * (w.shape[2] // 4) + (u - lo) * 128, 128), 128)
                    fn(pltpu.make_async_copy(
                        w.at[:, :, cols],
                        raw[j].at[:, pl.ds(_mult(at + (u - lo) * n, 128), n), :],
                        sems.at[SEM_STRIP + u % 2]))
            if isinstance(u, int):
                if lo <= u < hi:
                    run()
            else:
                pl.when((u >= lo) & (u < hi))(run)

    def weight_sums(r0):
        x = [[_load(raw[j], k, r0=r0, n=16).astype(f32) for j in range(4)]
             for k in range(4)]

        def emit(n, v):
            if n not in PLAIN:
                ref, *idx = wsum[n]
                ref[(*idx, pl.ds(_mult(r0, 16), 16), slice(None))] = v().astype(bf16)
        yield from _sums2(_sums_b, x, emit)

    def block_a(xb, xn, lo, *bufs):
        w_on, low, wo_s = bufs[0:3], bufs[3:6], bufs[6:13]
        w_hbm = (wq_hbm, wk_hbm, wv_hbm)
        stage = hbuf.reshape(8, S // 8 + 1, 8, DH)
        lhs = spare[2:5]
        w_low = [spare[5 + 3 * m:8 + 3 * m] for m in range(3)]

        def x_copy(i):
            return pltpu.make_async_copy(x_hbm.at[pl.ds(2 * i, 2)], xb.at[i % 2],
                                         sems.at[SEM_X + i % 2])

        def wo_copies(n):
            return [pltpu.make_async_copy(
                wo_hbm.at[:, i, :, pl.ds(_mult(j * HD + n * 128, 128), 128)],
                wo_s[slot].at[n], sems.at[SEM_WO + n])
                for slot, i, j in ((5, 0, 0), (2, 0, 1), (4, 1, 0), (1, 1, 1))]

        def chunk_copies(g, m):
            src = w_hbm[m].bitcast(f32)
            return [pltpu.make_async_copy(
                src.at[:, :, pl.ds(_mult(16 * par + 4 * g, 4), 4), :],
                stage.at[pl.ds(2 * m, 2), pl.ds(0, S // 8), pl.ds(4 * par, 4), :],
                sems.at[SEM_W + 3 * g + m]) for par in range(2)]

        def start(copies):
            for c in copies:
                c.start()

        def wait(copies):
            for c in copies:
                c.wait()

        def qkv_sums(g, m, pair, d0):
            b = []
            for half in range(2):
                w = pltpu.bitcast(
                    hbuf[2 * m + half, pl.ds(4 * d0 + pair, 16, stride=4), :], u32)
                b += [pltpu.bitcast(w << 16, f32),
                      pltpu.bitcast(w & jnp.uint32(0xFFFF0000), f32)]
            for k, v in enumerate(_sums_b(*b)):
                if k < 4:
                    w_on[m][4 * g + pair, k, pl.ds(d0, 16), :] = v().astype(bf16)
                else:
                    w_low[m][k - 4][pl.ds(_mult(pair * HD + d0, 16), 16), :] = v().astype(bf16)

        def wo_sums(n, t, e0):
            b = [_load(wo_s[k], n, t, r0=e0, n=16).astype(f32) for k in (5, 2, 4, 1)]
            for k, v in enumerate(_sums_b(*b)):
                if k not in (1, 5):
                    wo_s[k][n, t, pl.ds(e0, 16), :] = v().astype(bf16)

        def prologue(xpb):
            xp_copy = pltpu.make_async_copy(x_hbm.at[:, pl.ds(16, 16), :], xpb,
                                            sems.at[SEM_XP])
            xp_copy.start()
            start(chunk_copies(0, 0))
            start(chunk_copies(0, 1))
            start(wo_copies(0))
            start(chunk_copies(0, 2))
            lo[...] = jnp.zeros(lo.shape, f32)
            xp_copy.wait()

            @pl.loop(0, NSEG // 8)
            def _(i):
                for j in range(4):
                    a = [_ln(_load(xpb, 8 * i + 2 * j + k).astype(f32)) for k in range(2)]
                    a1 = jnp.concatenate([a[0][:8], a[1][:8]], axis=0)
                    a2 = jnp.concatenate([a[0][8:], a[1][8:]], axis=0)
                    ops = _sums_a(a1[:, :HD], a1[:, HD:], a2[:, :HD], a2[:, HD:])
                    ops = [v() for v in ops[4:]]
                    for k in range(3):
                        for c in range(4):
                            rows = pl.ds(pl.multiple_of(c * 8 * NSEG + 64 * i + 16 * j, 16), 16)
                            lhs[k][rows, :] = ops[k][:, c * 128:(c + 1) * 128].astype(bf16)

        if not 0:
            pl.run_scoped(prologue, pltpu.VMEM((NSEG, 16, D), bf16))
            wait(chunk_copies(0, 0))

            @pl.loop(0, 4)
            def _(pair):
                for d0 in range(0, HD, 16):
                    qkv_sums(0, 0, pair, d0)

        def lower_products(g, m):
            m1 = (m + 1) % 3
            g1 = jnp.minimum(g + (1 if m == 2 else 0), 3)
            side = [functools.partial(qkv_sums, g1, m1, pair, d0)
                    for d0 in range(0, HD, 16) for pair in range(4)]
            wait_at = 5
            span = 12 - wait_at
            early = []
            if m > 0:
                ts = range(0, 4) if m == 1 else range(4, NP)
                early = [functools.partial(wo_sums, g, t, e0)
                         for t in ts for e0 in range(0, DH, 16)]
            if m == 1:
                side, early = side + early, []
            for j in range(12):
                pair, k = divmod(j, 3)
                if j >= wait_at:
                    todo = side[len(side) * (j - wait_at) // span:
                                len(side) * (j - wait_at + 1) // span]
                else:
                    todo = early[len(early) * j // wait_at:len(early) * (j + 1) // wait_at]
                for fn in todo:
                    fn()
                a = jnp.concatenate(
                    [_load(lhs[k], r0=c * 8 * NSEG, n=8 * NSEG) for c in range(4)], axis=1)
                res = _dot(a, _load(w_low[m][k], r0=pair * HD, n=HD))
                if j == wait_at - 1:
                    pl.when(3 * g + m < 11)(lambda: wait(chunk_copies(g1, m1)))
                    if m == 1:
                        wait(wo_copies(g))

                    @pl.when(g < 3)
                    def _():
                        start(chunk_copies(g + 1, m))
                        if m == 1:
                            start(wo_copies(g + 1))
                    if m == 0:
                        @pl.when(g == 3)
                        def _():
                            x_copy(0).start()
                            x_copy(1).start()
                            strip_copies(0, lambda c: c.start())
                if k == 0:
                    m4 = res
                    low[m][4 * g + pair, 0] = m4.astype(bf16)
                elif k == 1:
                    m2 = res
                    low[m][4 * g + pair, 1] = (m2 + m4).astype(bf16)
                else:
                    low[m][4 * g + pair, 2] = (res - m2).astype(bf16)

        if not 0:
            @pl.loop(0, 4)
            def _(g):
                for m in range(3):
                    lower_products(g, m)

        def norm_tokens(i, k):
            for r0 in range(0, SEG, 16):
                xn[k, pl.ds(r0, 16), :] = _ln(_load(xb, i % 2, k, r0=r0, n=16).astype(f32))
                yield

        def lower_wo(grp, n, parts, state):
            for k in parts:
                w = jnp.concatenate([_load(wo_s[4 + k], n, t) for t in range(NP)], axis=0)
                state[k] = _dot(lo[grp % 2, k].astype(bf16), w)
            if 2 in parts:
                m4, m2, m6 = state[0], state[1], state[2]
                base = jnp.maximum(grp, 0) * (4 * SEG)
                for j in range(4):
                    seg = slice(8 * j, 8 * j + 8)
                    upper = pl.ds(pl.multiple_of(base + j * SEG + 16, 8), 8)
                    lower = pl.ds(pl.multiple_of(base + j * SEG + 24, 8), 8)
                    hbuf[n, upper, :] += m4[seg]
                    hbuf[n, lower, :] += m2[seg] + m4[seg]
                    hbuf[4 + n, lower, :] += m6[seg] - m2[seg]

        def attention_mask():
            def split(axis):
                r = lax.broadcasted_iota(jnp.int32, (80, 80), axis)
                return (jnp.where(r < 64, r >> 5, (r - 64) >> 3),
                        jnp.where(r < 64, r & 31, 32 + (r & 7)))
            (hq, pq), (hk, pk) = split(0), split(1)
            visible = (pq < MEM) | (pq >= pk)
            return jnp.where(hq == hk, jnp.where(visible, 0.0, NEG), -jnp.inf)

        def step(i, k, mem, fill, side):
            s = 2 * i + k
            tok = xn[k]
            xv = _load(xb, i % 2, k).astype(f32)
            for c in range(8):
                hbuf[c, pl.ds(pl.multiple_of(s * SEG, SEG), SEG), :] = xv[:, c * 128:(c + 1) * 128]
            a1 = jnp.concatenate([mem, tok[:24]], axis=0)
            ops = _upper_operands(a1[:, :HD], a1[:, HD:], tok[24:, HD:])
            qkvs, scores, outs, lower = {}, {}, {}, {}
            total = [None] * 4

            def qkv(t):
                res = []
                for m in range(3):
                    m7, m5, m3, m1 = [_dot(ops[j], _load(w_on[m], t, j)) for j in range(4)]
                    m4, c21, m62 = [
                        _load(low[m], t, j, r0=16 * i, n=16).astype(f32)[8 * k:8 * k + 8]
                        for j in range(3)]
                    side()
                    c11 = m7 - m5 + m1
                    res.append(jnp.concatenate(
                        [c11[:24], c11[24:] + m4, m5 + m3, c21, m3[24:] + m62 + m1[24:]],
                        axis=0).astype(bf16))
                qkvs[t] = res

            def qk(t):
                q, kk, v = qkvs.pop(t)
                sc = lax.dot_general(q, kk, (((1,), (1,)), ((), ())),
                                     preferred_element_type=f32)
                scores[t] = (sc, v)

            def pv(t):
                sc, v = scores.pop(t)
                sc = jnp.where(fill == 0.0, sc * (DH ** -0.5), fill)
                mx = jnp.max(sc, axis=1, keepdims=True)
                e = jnp.exp(sc - mx)
                den = jnp.sum(e, axis=1, keepdims=True)
                inv = pl.reciprocal(den, approx=True)
                inv = inv * (2.0 - den * inv)
                outs[t] = _dot(e.astype(bf16), v) * inv

            def wo(t):
                o = outs.pop(t)
                a11, a12, a21, a22 = o[:32], o[32:64], o[64:72], o[72:]
                rows = pl.ds(pl.multiple_of(8 * (s % 4), 8), 8)
                for j, v in enumerate((a22, a21 + a22, a21 - a11[24:])):
                    lo[(s // 4) % 2, j, rows, pl.ds(t * DH, DH)] = v
                for j, a in enumerate(_upper_operands(a11, a12, a22)):
                    w = jnp.concatenate([_load(wo_s[j], n, t) for n in range(4)], axis=1)
                    r = _dot(a, w)
                    total[j] = r if total[j] is None else total[j] + r

            G = 1
            for t in range(NP + LAG_WO):
                if t % G == 0:
                    for u in range(t - G + 1, t + 1):
                        if 0 <= u - LAG_QK < NP:
                            qk(u - LAG_QK)
                    for u in range(t - G + 1, t + 1):
                        if 0 <= u - LAG_PV < NP:
                            pv(u - LAG_PV)
                if t < NP:
                    qkv(t)
                lower_wo(s // 4 - 1, s % 4, [j for j in range(3) if FILL[j] == t], lower)
                if 0 <= t - LAG_WO < NP:
                    wo(t - LAG_WO)
            lower_wo(s // 4 - 1, s % 4, [j for j in range(3) if j not in lower], lower)

            m7, m5, m3, m1 = total
            upper = jnp.concatenate([m7 - m5 + m1, m5 + m3], axis=1)
            c22 = m3[24:] + m1[24:]
            for c in range(8):
                hbuf[c, pl.ds(pl.multiple_of(s * SEG, SEG), 24), :] += (
                    upper[MEM:, c * 128:(c + 1) * 128])
            for c in range(4):
                hbuf[4 + c, pl.ds(pl.multiple_of(s * SEG + 24, 8), 8), :] += (
                    c22[:, c * 128:(c + 1) * 128])
            return upper[:MEM]

        fill = attention_mask()
        n_it = NSEG // 2
        per_it = WROWS // 16 // n_it

        def steps(i, mem):
            pl.when(i + 1 < n_it)(lambda: x_copy(i + 1).wait())

            @pl.when(i < NSTRIP)
            def _():
                strip_copies(i, lambda c: c.wait())
                strip_copies(i + 1, lambda c: c.start())

            sums = [weight_sums(16 * (per_it * i + j)) for j in range(per_it)]
            for k, part in enumerate((sums[:5], sums[5:])):
                r0 = jnp.maximum(2 * i + k - 8, 0) * SEG
                mem = step(i, k, mem, fill, _spread(
                    [h_stats(r0), part[0], h_stats(r0 + 16), *part[1:], norm_tokens(i + 1, k)],
                    7 * len(part) + 4, 3 * NP))
            pl.when(i + 2 < n_it)(lambda: x_copy(i + 2).start())
            return mem

        if not 0:
            x_copy(0).wait()
            _spread([norm_tokens(0, 0), norm_tokens(0, 1)], 4, 1)()
            lax.fori_loop(0, n_it, steps, mem0_ref[...].astype(f32))
            for n in range(4):
                lower_wo(NSEG // 4 - 1, n, [0, 1, 2], {})

    pl.run_scoped(
        block_a,
        pltpu.VMEM((2, 2, SEG, D), bf16),
        pltpu.VMEM((2, SEG, D), f32),
        pltpu.VMEM((2, 3, 32, NP * DH), f32),
        *[pltpu.VMEM((NP, 4, HD, DH), bf16)] * 3,
        *[pltpu.VMEM((NP, 3, 8 * NSEG, DH), bf16)] * 3,
        *[pltpu.VMEM((4, NP, DH, 128), bf16)] * 7,
    )

    def block_b(gbuf, ub, hs, res, obuf, yc, hc, db, nb0, nb1, ac0, ac1, pb0, pb1):
        def weights(n, at, rows, strips):
            return jnp.concatenate(
                [_load(*wsum[n], r0=at + k * rows[0] + rows[1], n=rows[2])
                 for k in strips], axis=1)

        zero = zero_ref[0]
        results = []
        running = []

        def mark(ref, value, n):
            rows = pl.ds(pl.multiple_of(ref.shape[-2] - n + zero, n), n)
            ref[(0,) * (len(ref.shape) - 2) + (rows, pl.ds(0, 128))] = (
                value[:n, :128].astype(ref.dtype))

        def after(ref, back):
            if 0 < back <= len(results):
                mark(ref, results[-back], 8)

        def before_next(value):
            if running:
                n = (running[0] + 1) % 49
                while n in RAW_SLOT:
                    n = (n + 1) % 49
                mark(wsum[n][0], value, 16)

        def operand(ref, n, cols):
            running[:] = [n]
            return jnp.concatenate([_load(ref, n, c, n=R) for c in cols], axis=1)

        def store_sums(dst, r, c, x):
            def emit(n, v):
                v = v().astype(bf16)
                dst[n, c, pl.ds(16 * r, 16), :] = v
                if n % 7 == 6 and dst is not hc and 0:
                    before_next(v)
            return _sums2(_sums_a, x, emit)

        def inner(dst, p, product, side, add=False):
            def emit(a, b, v):
                dst[p, 2 * a + b, :R] = dst[p, 2 * a + b, :R] + v if add else v

            def run(k):
                r = product(7 * p + k)
                results.append(r)
                side()
                return r
            _combine(run, emit)

        def outer(src, r, cols, emit):
            for a in range(2):
                for b in range(2):
                    if 0 and (src is pb0 or src is pb1):
                        after(src, 0)
                    _combine(lambda p: src[p, 2 * a + b, pl.ds(16 * r, 16), cols],
                             lambda i, j, v: emit(2 * i + a, 2 * j + b, v))
                    yield

        def rows_of(i, g, r):
            return pl.ds(_mult(i * RB + g * R + 16 * r, 16), 16)

        def last_stats(i, r):
            for g in range(4):
                after(hbuf, 1)
                yield from h_stats(i * RB + g * R + 16 * r)
                yield from range(3)

        def pre1(i, r):
            for c in range(2):
                after(hbuf, 0)
                x = []
                for g in range(4):
                    rows = rows_of(i, g, r)
                    x.append([(hbuf[2 * k + c, rows, :] - hstat[0, rows, :]) * hstat[2, rows, :]
                              for k in range(4)])
                yield from range(3)
                yield from store_sums(ac0, r, c, x)

        def post1(i, r):
            def emit(g, j, v):
                v = _gelu_of_double(v)
                gbuf[2 * j + c, pl.ds(HALO + i * RB + g * R + 16 * r, 16), :] = v
                if g >= 2 and j >= 2 and 0:
                    before_next(v)
            for c in range(2):
                for _ in outer(pb0, r, pl.ds(c * 128, 128), emit):
                    yield
                    yield

        def pre2(i, r):
            for c in range(2):
                after(gbuf, 0)
                x = [[gbuf[2 * k + c, pl.ds(HALO + i * RB + g * R + 16 * r + off, 16), :]
                      for k, off in enumerate((-1, 1, -2, 2))] for g in range(4)]
                yield from store_sums(ac1, r, c, x)

        def post2(i, r):
            def emit(g, j, v):
                hs[rows_of(i, g, r), pl.ds(j * C4, C4)] = v
            for _ in outer(pb1, r, slice(None), emit):
                yield
                yield

        def pre3(i, r):
            for g in range(4):
                rows = rows_of(i, g, r)
                after(hbuf, 1)
                m1, r1 = hstat[0, rows, :], hstat[1, rows, :]
                x1 = []
                for c in range(8):
                    hv = hbuf[c, rows, :]
                    v = (hv - m1) * r1 + hs[rows, pl.ds(c * 128, 128)]
                    res[rows, pl.ds(c * 128, 128)] = hv + v
                    ub[c, rows_of(0, g, r), :] = v
                    x1.append(v)
                m, rs = _ln_stats(jnp.concatenate(x1, axis=1))
                ub[8, rows_of(0, g, r), :] = jnp.broadcast_to(m, (16, 128))
                ub[9, rows_of(0, g, r), :] = jnp.broadcast_to(0.5 * rs, (16, 128))
                if 0:
                    before_next(x1[-1])
                yield from range(4)

        def sums3(i, r):
            for c in range(2):
                after(ub, 1)
                x = [[(ub[2 * k + c, rows, :] - ub[8, rows, :]) * ub[9, rows, :]
                      for k in range(4)] for rows in (rows_of(0, g, r) for g in range(4))]
                yield from store_sums(yc, r, c, x)

        pieces = {pre1: 20, last_stats: 16, post1: 16, pre2: 14, post2: 8, pre3: 16, sums3: 14}

        def spread(stages, slots):
            stages = [(fn, i) for fn, i in stages if not isinstance(i, int) or 0 <= i < NB]
            return _spread([fn(i, r) for fn, i in stages for r in range(R // 16)],
                           sum(pieces[fn] for fn, _ in stages) * (R // 16), slots)

        def mixer(i, src, at, dst, stages):
            if not 0 <= i < NB:
                running.clear()
                return spread(stages, 1)()
            side = spread(stages, 46)
            calls = itertools.count()
            for p in range(7):
                inner(dst, p, lambda n: _dot(operand(src, n, (0, 1)),
                                             weights(n, at, (C4, 0, C4), (0, 1))),
                      lambda: next(calls) < 46 and side())

        if not 0:
            for c in range(8):
                gbuf[c, pl.ds(0, HALO), :] = jnp.zeros((HALO, 128), f32)
                gbuf[c, pl.ds(HALO + S, HALO), :] = jnp.zeros((HALO, 128), f32)
            for i in range(-1, NB + 3):
                mixer(i, ac0, W1_AT, pb0, [(pre2, i - 2), (post2, i - 3)]
                      + {1: [(last_stats, NB - 1)], NB - 1: [(pre3, 0)]}.get(i, []))
                mixer(i - 2, ac1, W2_AT, pb1, [(pre1, i + 1), (post1, i)]
                      + {NB: [(sums3, 0)]}.get(i, []))

        def out_copy(i):
            rows = pl.ds(_mult(i * (RB // 2), RB // 2), RB // 2)
            return pltpu.make_async_copy(obuf.at[rows], out_hbm.at[rows],
                                         sems.at[SEM_OUT + i])

        nb = (nb0, nb1)

        def mlp_block(i):
            results.clear()

            def activate(c, r):
                act = [[None] * 4 for _ in range(4)]

                def emit(g, j, v):
                    act[g][j] = _gelu_of_double(v)
                for _ in outer(nb[c % 2], r, slice(None), emit):
                    yield
                    yield
                yield from store_sums(hc, r, c, act)

            pieces[activate] = 15

            def down(p, side, k0=0, k1=F4):
                inner(db, p, lambda n: _dot(operand(hc, n, range(k0 // 128, k1 // 128)),
                                            weights(n, W4_AT, (F4, k0, k1 - k0), (0, 1))),
                      side, add=k0 > 0)

            def finish(bi, bj, plus, minus=()):
                for a in range(2):
                    for b in range(2):
                        rows = pl.ds(pl.multiple_of(i * RB + (2 * bi + a) * R, R), R)
                        cols = pl.ds((2 * bj + b) * C4, C4)
                        v = res[rows, cols]
                        for p in minus:
                            v = v - db[p, 2 * a + b, :R]
                        for p in plus:
                            v = v + db[p, 2 * a + b, :R]
                        obuf[rows, cols] = v.astype(bf16)

            for c in range(7):
                side = spread([(activate, c - 1)], 49)
                for p in range(7):
                    inner(nb[c % 2], p, lambda n: _dot(
                        operand(yc, n, (0, 1)), weights(n, W3_AT, (C4, 0, C4), (c,))), side)
            side = spread([(activate, 6)], 6)
            calls = itertools.count()
            down(0, lambda: next(calls) < 6 and side(), 0, F4 - 128)
            down(0, lambda: None, F4 - 128)
            side = spread([(pre3, jnp.minimum(i + 1, NB - 1)), (sums3, 0)], 35)
            for p in range(1, 7):
                down(p, side if p < 6 else lambda: None)
                if p == 3:
                    finish(0, 1, (1, 2))
                if p == 5:
                    finish(0, 0, (0, 3, 4), (1,))
            finish(1, 0, (4, 5))
            finish(1, 1, (2, 3, 6), (5,))
            out_copy(2 * i).start()
            out_copy(2 * i + 1).start()

        if not 0:
            pl.loop(0, NB)(mlp_block)
            for i in range(2 * NB):
                out_copy(i).wait()

    pl.run_scoped(
        block_b,
        pltpu.VMEM((8, S + 2 * HALO + 8, 128), f32),
        pltpu.VMEM((10, RB + 8, 128), f32),
        pltpu.VMEM((S, D), f32),
        pltpu.VMEM((S, D), f32),
        pltpu.VMEM((S, D), bf16),
        pltpu.VMEM((49, 2, R, 128), bf16),
        pltpu.VMEM((49, 7, R, 128), bf16),
        pltpu.VMEM((7, 4, R + 8, C4), f32),
        *[pltpu.VMEM((7, 4, R + 8, 128), f32)] * 2,
        *[pltpu.VMEM((49, 2, R, 128), bf16)] * 2,
        *[pltpu.VMEM((7, 4, R + 8, C4), f32)] * 2,
    )


@jax.jit
def pallas_sequential_preLN__memory_aug_recurrent_mem_tr__mixer_s_mlp__prompt_kernel(
    A_x: jax.Array,
    A_mem0: jax.Array,
    A_Wq: jax.Array,
    A_Wk: jax.Array,
    A_Wv: jax.Array,
    A_Wo: jax.Array,
    A_seg_len: jax.Array,
    B_x: jax.Array,
    B_w1: jax.Array,
    B_w2: jax.Array,
    B_w3: jax.Array,
    B_w4: jax.Array,
):
    del A_seg_len, B_x
    hbm = pl.BlockSpec(memory_space=pl.ANY)
    vmem = pl.BlockSpec(memory_space=pltpu.VMEM)
    scratch = [
        pltpu.VMEM((8, S + 8, 128), f32),
        pltpu.VMEM((3, S, 128), f32),
        pltpu.SemaphoreType.DMA((NSEM,)),
        pltpu.SMEM((1,), jnp.int32),
    ] + [pltpu.VMEM((4, WROWS, 128), bf16)] * 4 + [pltpu.VMEM((WROWS + 16, 128), bf16)] * 33
    out = pl.pallas_call(
        _kernel,
        out_shape=jax.ShapeDtypeStruct((S, D), A_x.dtype),
        in_specs=[hbm, vmem] + [hbm] * 8,
        out_specs=hbm,
        scratch_shapes=scratch,
        compiler_params=pltpu.CompilerParams(vmem_limit_bytes=128 * 1024 * 1024),
    )(A_x.reshape(NSEG, SEG, D), A_mem0.reshape(MEM, D),
      A_Wq.reshape(2, D // 4, 2 * H, DH), A_Wk.reshape(2, D // 4, 2 * H, DH),
      A_Wv.reshape(2, D // 4, 2 * H, DH), A_Wo.reshape(NP, 2, DH, D),
      B_w1.reshape(4, C4, D), B_w2.reshape(4, C4, D),
      B_w3.reshape(4, C4, F), B_w4.reshape(4, F4, D))
    return out.reshape(A_x.shape)
```

```python
import functools
import itertools

import jax
import jax.numpy as jnp
from jax import lax
import jax.experimental.pallas as pl
import jax.experimental.pallas.tpu as pltpu

S = 2048
D = 1024
H = 32
DH = 128
MEM = 8
SEG = 32
F = 3584
NSEG = S // SEG
NP = H // 2
HD = D // 2
C4 = D // 4
F4 = F // 4
HALO = 8
R = 64
RB = 4 * R
NB = S // RB
EPS = 1e-5
NEG = -1000000000.0
LOG2E = 1.4426950408889634

W1_AT, W2_AT, W3_AT, W4_AT = 0, 2 * C4, 4 * C4, 11 * C4
WROWS = W4_AT + 2 * F4
NSTRIP = 13

LAG_QK, LAG_PV, LAG_WO = 2, 4, 6
FILL = (17, 19, 99)

bf16 = jnp.bfloat16
f32 = jnp.float32
u32 = jnp.uint32

SEM_XP, SEM_X, SEM_WO, SEM_STRIP, SEM_OUT, SEM_W = 0, 8, 10, 14, 16, 16 + 2 * NB
NSEM = SEM_W + 12


def _mult(i, n):
    return i if isinstance(i, int) else pl.multiple_of(i, n)


def _ln_stats(x):
    m = jnp.mean(x, axis=-1, keepdims=True)
    d = x - m
    v = jnp.mean(d * d, axis=-1, keepdims=True)
    return m, lax.rsqrt(v + EPS)


def _ln_stages(x):
    m = jnp.mean(x, axis=-1, keepdims=True)
    yield m
    d = x - m
    r = lax.rsqrt(jnp.mean(d * d, axis=-1, keepdims=True) + EPS)
    return m, r


def _ln(x):
    m, r = _ln_stats(x)
    return (x - m) * r


def _gelu_of_double(y):
    c = 0.7978845608028654
    return y + y * jnp.tanh(y * (2 * c + (8 * c * 0.044715) * (y * y)))


def _dot(a, b):
    return jnp.dot(a, b, preferred_element_type=f32)


def _load(ref, *idx, r0=0, n=None):
    n = ref.shape[-2] if n is None else n
    return pltpu.bitcast(
        ref.bitcast(u32)[(*idx, pl.ds(_mult(r0 >> 1, 8), n // 2), slice(None))], bf16)


def _sums_a(a11, a12, a21, a22):
    return [lambda: a12 - a22, lambda: a11 + a12, lambda: a11, lambda: a11 + a22,
            lambda: a22, lambda: a21 + a22, lambda: a21 - a11]


def _sums_b(b11, b12, b21, b22):
    return [lambda: b21 + b22, lambda: b22, lambda: b12 - b22, lambda: b11 + b22,
            lambda: b21 - b11, lambda: b11, lambda: b11 + b12]


def _combine(product, emit):
    c11 = product(0)
    c12 = product(1)
    c11 = c11 - c12
    c22 = product(2)
    emit(0, 1, c12 + c22)
    t = product(3)
    c11 = c11 + t
    c22 = c22 + t
    c21 = product(4)
    emit(0, 0, c11 + c21)
    t = product(5)
    emit(1, 0, c21 + t)
    c22 = c22 - t
    emit(1, 1, c22 + product(6))


def _sums2(sums, x, emit):
    outer = [sums(x[i][j], x[i][2 + j], x[2 + i][j], x[2 + i][2 + j])
             for i in range(2) for j in range(2)]
    for p in range(7):
        for q, v in enumerate(sums(*(o[p]() for o in outer))):
            emit(7 * p + q, v)
        yield


def _spread(tasks, pieces, slots):
    todo = itertools.chain(*tasks)
    calls = itertools.count(1)

    def advance():
        k = next(calls)
        if k > slots:
            return
        for _ in range(pieces * k // slots - pieces * (k - 1) // slots):
            next(todo)
        if k == slots:
            assert next(todo, todo) is todo
    return advance


def _upper_operands(a11, a12, a22):
    k = a11.shape[0] - a22.shape[0]
    ops = [jnp.concatenate([a12[:k], a12[k:] - a22], axis=0), a11 + a12, a11,
           jnp.concatenate([a11[:k], a11[k:] + a22], axis=0)]
    return [v.astype(bf16) for v in ops]


PLAIN = {40: 0, 36: 1, 12: 2, 8: 3}
OTHER = [n for n in range(49) if n not in PLAIN]
RAW_SLOT = dict(zip(OTHER[2::3], [(k, j) for k in range(4) for j in range(4) if k != j]))
RAW_SLOT.update({n: (k, k) for n, k in PLAIN.items()})


def _kernel(x_hbm, mem0_ref, wq_hbm, wk_hbm, wv_hbm, wo_hbm, w1_hbm, w2_hbm,
            w3_hbm, w4_hbm, out_hbm, hbuf, hstat, sems, zero_ref, *wbufs):
    zero_ref[0] = 0
    raw, spare = wbufs[:4], wbufs[4:]
    wsum = {n: (raw[j], k) for n, (k, j) in RAW_SLOT.items()}
    wsum.update({n: (b,) for n, b in zip((n for n in OTHER if n not in RAW_SLOT), spare)})

    def load_h(rows):
        return jnp.concatenate([hbuf[c, rows, :] for c in range(8)], axis=1)

    def h_stats(r0, n=16):
        rows = pl.ds(_mult(r0, 16), n)
        hv = load_h(rows)
        m1, r1 = yield from _ln_stages(hv)
        yield r1
        m2, r2 = yield from _ln_stages((hv - m1) * r1)
        stats = (m1 + m2 / r1, r1, 0.5 * r1 * r2)
        for k, v in enumerate(stats):
            hstat[k, rows, :] = jnp.broadcast_to(v, (n, 128))
        yield stats[0] + stats[2]

    def strip_copies(u, fn):
        for lo, hi, w, at in ((0, 2, w1_hbm, W1_AT), (2, 4, w2_hbm, W2_AT),
                              (4, 11, w3_hbm, W3_AT), (11, 13, w4_hbm, W4_AT)):
            def run(lo=lo, w=w, at=at):
                n = w.shape[1]
                for j in range(4):
                    cols = pl.ds(_mult(j * (w.shape[2] // 4) + (u - lo) * 128, 128), 128)
                    fn(pltpu.make_async_copy(
                        w.at[:, :, cols],
                        raw[j].at[:, pl.ds(_mult(at + (u - lo) * n, 128), n), :],
                        sems.at[SEM_STRIP + (u & 1)]))
            if isinstance(u, int):
                if lo <= u < hi:
                    run()
            else:
                pl.when((u >= lo) & (u < hi))(run)

    def weight_sums(r0):
        x = [[_load(raw[j], k, r0=r0, n=16).astype(f32) for j in range(4)]
             for k in range(4)]

        def emit(n, v):
            if n not in PLAIN:
                ref, *idx = wsum[n]
                ref[(*idx, pl.ds(_mult(r0, 16), 16), slice(None))] = v().astype(bf16)
        yield from _sums2(_sums_b, x, emit)

    def block_a(xb, xn, lo, *bufs):
        w_on, low, wo_s = bufs[0:3], bufs[3:6], bufs[6:13]
        w_hbm = (wq_hbm, wk_hbm, wv_hbm)
        stage = hbuf.reshape(8, hbuf.shape[1] // 8, 8, DH)
        lhs = spare[2:5]
        w_low = [spare[5 + 3 * m:8 + 3 * m] for m in range(3)]

        def x_copy(i):
            return pltpu.make_async_copy(x_hbm.at[pl.ds(2 * i, 2)], xb.at[i & 3],
                                         sems.at[SEM_X + (i & 1)])

        def wo_copies(n):
            return [pltpu.make_async_copy(
                wo_hbm.at[:, i, :, pl.ds(_mult(j * HD + n * 128, 128), 128)],
                wo_s[slot].at[n], sems.at[SEM_WO + n])
                for slot, i, j in ((5, 0, 0), (2, 0, 1), (4, 1, 0), (1, 1, 1))]

        def chunk_copies(g, m):
            src = w_hbm[m].bitcast(f32)
            return [pltpu.make_async_copy(
                src.at[:, :, pl.ds(_mult(16 * par + 4 * g, 4), 4), :],
                stage.at[pl.ds(2 * m, 2), pl.ds(0, S // 8), pl.ds(4 * par, 4), :],
                sems.at[SEM_W + 3 * g + m]) for par in range(2)]

        def start(copies):
            for c in copies:
                c.start()

        def wait(copies):
            for c in copies:
                c.wait()

        def qkv_sums(g, m, pair, d0):
            b = []
            for half in range(2):
                w = pltpu.bitcast(
                    hbuf[2 * m + half, pl.ds(4 * d0 + pair, 16, stride=4), :], u32)
                b += [pltpu.bitcast(w << 16, f32),
                      pltpu.bitcast(w & jnp.uint32(0xFFFF0000), f32)]
            for k, v in enumerate(_sums_b(*b)):
                if k < 4:
                    w_on[m][4 * g + pair, k, pl.ds(d0, 16), :] = v().astype(bf16)
                else:
                    w_low[m][k - 4][pl.ds(_mult(pair * HD + d0, 16), 16), :] = v().astype(bf16)

        def wo_sums(n, t, e0):
            b = [_load(wo_s[k], n, t, r0=e0, n=16).astype(f32) for k in (5, 2, 4, 1)]
            for k, v in enumerate(_sums_b(*b)):
                if k not in (1, 5):
                    wo_s[k][n, t, pl.ds(e0, 16), :] = v().astype(bf16)

        def prologue(xpb):
            def xp_copy(i):
                segs = pl.ds(8 * i, 8)
                return pltpu.make_async_copy(x_hbm.at[segs, pl.ds(16, 16), :], xpb.at[segs],
                                             sems.at[SEM_XP + i])

            start(chunk_copies(0, 0))
            start([xp_copy(i) for i in range(NSEG // 8)])
            start(chunk_copies(0, 1))
            start(chunk_copies(0, 2))
            lo[...] = jnp.zeros(lo.shape, f32)
            for k in (5, 2, 4, 1):
                wo_s[k][3] = jnp.zeros(wo_s[k].shape[1:], bf16)
            wait(chunk_copies(0, 0))

            @pl.loop(0, 4)
            def _(pair):
                for d0 in range(0, HD, 16):
                    qkv_sums(0, 0, pair, d0)

            @pl.loop(0, NSEG // 8)
            def _(i):
                xp_copy(i).wait()
                for j in range(4):
                    a = [_ln(_load(xpb, 8 * i + 2 * j + k).astype(f32)) for k in range(2)]
                    a1 = jnp.concatenate([a[0][:8], a[1][:8]], axis=0)
                    a2 = jnp.concatenate([a[0][8:], a[1][8:]], axis=0)
                    ops = _sums_a(a1[:, :HD], a1[:, HD:], a2[:, :HD], a2[:, HD:])
                    ops = [v() for v in ops[4:]]
                    for k in range(3):
                        for c in range(4):
                            rows = pl.ds(pl.multiple_of(c * 8 * NSEG + 64 * i + 16 * j, 16), 16)
                            lhs[k][rows, :] = ops[k][:, c * 128:(c + 1) * 128].astype(bf16)

        if not 0:
            pl.run_scoped(prologue, pltpu.VMEM((NSEG, 16, D), bf16))

        def lower_products(g, m):
            m1 = (m + 1) % 3
            g1 = jnp.minimum(g + (1 if m == 2 else 0), 3)
            side = [functools.partial(qkv_sums, g1, m1, pair, d0)
                    for d0 in range(0, HD, 16) for pair in range(4)]
            wait_at = 7
            span = 12 - wait_at
            early = [functools.partial(wo_sums, (g + 3) & 3, t, e0)
                     for t in ((), range(0, 8), range(8, NP))[m] for e0 in range(0, DH, 16)]
            for j in range(12):
                pair, k = divmod(j, 3)
                if j >= wait_at:
                    todo = side[len(side) * (j - wait_at) // span:
                                len(side) * (j - wait_at + 1) // span]
                else:
                    todo = early[len(early) * j // wait_at:len(early) * (j + 1) // wait_at]
                for fn in todo:
                    fn()
                a = jnp.concatenate(
                    [_load(lhs[k], r0=c * 8 * NSEG, n=8 * NSEG) for c in range(4)], axis=1)
                res = _dot(a, _load(w_low[m][k], r0=pair * HD, n=HD))
                if j == wait_at - 1:
                    pl.when(3 * g + m < 11)(lambda: wait(chunk_copies(g1, m1)))
                    pl.when(g < 3)(lambda: start(chunk_copies(g + 1, m)))
                    if m == 0:
                        pl.when(g > 0)(lambda: wait(wo_copies(g - 1)))
                        start(wo_copies(g))

                        @pl.when(g == 3)
                        def _():
                            x_copy(0).start()
                            x_copy(1).start()
                            strip_copies(0, lambda c: c.start())
                if k == 0:
                    m4 = res
                    low[m][4 * g + pair, 0] = m4.astype(bf16)
                elif k == 1:
                    m2 = res
                    low[m][4 * g + pair, 1] = (m2 + m4).astype(bf16)
                else:
                    low[m][4 * g + pair, 2] = (res - m2).astype(bf16)

        if not 0:
            @pl.loop(0, 4)
            def _(g):
                for m in range(3):
                    lower_products(g, m)

        def norm_tokens(i, k):
            for r0 in range(0, SEG, 16):
                v = _load(xb, jnp.minimum(i, NSEG // 2 - 1) & 3, k, r0=r0, n=16).astype(f32)
                m, r = yield from _ln_stages(v)
                xn[k, pl.ds(r0, 16), :] = (v - m) * r
                yield r

        def lower_wo(grp, n, parts, state):
            for k in parts:
                w = jnp.concatenate([_load(wo_s[4 + k], n, t) for t in range(NP)], axis=0)
                state[k] = _dot(lo[grp & 1, k].astype(bf16), w)
            if 2 in parts:
                m4, m2, m6 = state[0], state[1], state[2]
                base = jnp.maximum(grp, 0) * (4 * SEG)
                for j in range(4):
                    seg = slice(8 * j, 8 * j + 8)
                    upper = pl.ds(pl.multiple_of(base + j * SEG + 16, 8), 8)
                    lower = pl.ds(pl.multiple_of(base + j * SEG + 24, 8), 8)
                    hbuf[n, upper, :] += m4[seg]
                    hbuf[n, lower, :] += m2[seg] + m4[seg]
                    hbuf[4 + n, lower, :] += m6[seg] - m2[seg]

        def attention_mask():
            def split(axis):
                r = lax.broadcasted_iota(jnp.int32, (80, 80), axis)
                return (jnp.where(r < 64, r >> 5, (r - 64) >> 3),
                        jnp.where(r < 64, r & 31, 32 + (r & 7)))
            (hq, pq), (hk, pk) = split(0), split(1)
            visible = (pq < MEM) | (pq >= pk)
            return jnp.where(hq == hk, jnp.where(visible, 0.0, NEG * DH ** 0.5), -jnp.inf)

        def step(i, k, mem, fill, side):
            tok = xn[k]
            r0 = jnp.maximum(2 * i + k - 8, 0) * SEG
            norms = itertools.chain(h_stats(r0), h_stats(r0 + 16), norm_tokens(i + 1, k))
            s = 2 * i + k
            xv = _load(xb, jnp.minimum(i, NSEG // 2 - 1) & 3, k).astype(f32)
            for c in range(8):
                hbuf[c, pl.ds(pl.multiple_of(s * SEG, SEG), SEG), :] = xv[:, c * 128:(c + 1) * 128]
            a1 = jnp.concatenate([mem, tok[:24]], axis=0)
            ops = _upper_operands(a1[:, :HD], a1[:, HD:], tok[24:, HD:])
            qkvs, scores, outs, lower = {}, {}, {}, {}
            total = [None] * 4

            def qkv(t):
                res = []
                for m in range(3):
                    m7, m5, m3, m1 = [_dot(ops[j], _load(w_on[m], t, j)) for j in range(4)]
                    m4, c21, m62 = [
                        _load(low[m], t, j, r0=16 * i, n=16).astype(f32)[8 * k:8 * k + 8]
                        for j in range(3)]
                    side()
                    c11 = m7 - m5 + m1
                    res.append(jnp.concatenate(
                        [c11[:24], c11[24:] + m4, m5 + m3, c21, m3[24:] + m62 + m1[24:]],
                        axis=0).astype(bf16))
                qkvs[t] = res

            def qk(t):
                q, kk, v = qkvs.pop(t)
                sc = lax.dot_general(q, kk, (((1,), (1,)), ((), ())),
                                     preferred_element_type=f32)
                scores[t] = (sc, v)

            def pv(t):
                sc, v = scores.pop(t)
                sc = jnp.where(fill == 0.0, sc, fill)
                tie = next(norms, None) if t >= 0 else None
                if tie is not None:
                    sc = jnp.concatenate([jnp.where(never, tie, sc[:16]), sc[16:]], axis=0)
                mx = jnp.max(sc, axis=1, keepdims=True)
                e = jnp.exp2((sc - mx) * (DH ** -0.5 * LOG2E))
                den = jnp.sum(e, axis=1, keepdims=True)
                inv = pl.reciprocal(den, approx=True)
                inv = inv * (2.0 - den * inv)
                outs[t] = _dot(e.astype(bf16), v) * inv

            def wo(t):
                o = outs.pop(t)
                a11, a12, a21, a22 = o[:32], o[32:64], o[64:72], o[72:]
                rows = pl.ds(pl.multiple_of(8 * (s & 3), 8), 8)
                for j, v in enumerate((a22, a21 + a22, a21 - a11[24:])):
                    lo[(s >> 2) & 1, j, rows, pl.ds(t * DH, DH)] = v
                r = [_dot(a, jnp.concatenate([_load(wo_s[j], n, t) for n in range(4)], axis=1))
                     for j, a in enumerate(_upper_operands(a11, a12, a22))]
                if 0:
                    r = [r[0] - r[1] + r[3], r[1] + r[2], r[2][24:] + r[3][24:]]
                for j, v in enumerate(r):
                    total[j] = v if total[j] is None else total[j] + v

            def attend(t):
                if t % 2 == 1:
                    todo = [(qk, LAG_QK), (pv, LAG_PV)]
                    for fn, lag in todo[::-1] if 0 else todo:
                        for u in (t - 1 - lag, t - lag):
                            if 0 <= u < NP:
                                fn(u)

            for t in range(NP + LAG_WO):
                if 1 == 0:
                    attend(t)
                if t < NP:
                    qkv(t)
                lower_wo((s >> 2) - 1, s & 3, [j for j in range(3) if FILL[j] == t], lower)
                if 1 == 1:
                    attend(t)
                if 0 <= t - LAG_WO < NP:
                    wo(t - LAG_WO)
            lower_wo((s >> 2) - 1, s & 3, [j for j in range(3) if j not in lower], lower)

            if 0:
                upper, c22 = jnp.concatenate(total[:2], axis=1), total[2]
            else:
                m7, m5, m3, m1 = total
                upper = jnp.concatenate([m7 - m5 + m1, m5 + m3], axis=1)
                c22 = m3[24:] + m1[24:]
            for c in range(8):
                hbuf[c, pl.ds(pl.multiple_of(s * SEG, SEG), 24), :] += (
                    upper[MEM:, c * 128:(c + 1) * 128])
            for c in range(4):
                hbuf[4 + c, pl.ds(pl.multiple_of(s * SEG + 24, 8), 8), :] += (
                    c22[:, c * 128:(c + 1) * 128])
            return upper[:MEM]

        fill = attention_mask()
        never = jnp.full((16, 80), zero_ref[0]) != 0
        n_it = NSEG // 2
        per_it = WROWS // 16 // n_it

        def steps(i, mem):
            pl.when(i + 1 < n_it)(lambda: x_copy(i + 1).wait())
            pl.when(i + 2 < n_it)(lambda: x_copy(i + 2).start())

            @pl.when(i < NSTRIP)
            def _():
                strip_copies(i, lambda c: c.wait())
                strip_copies(i + 1, lambda c: c.start())

            side = _spread([weight_sums(16 * (per_it * i + j)) for j in range(per_it)],
                           7 * per_it, 72)
            for k in range(2):
                mem = step(i, k, mem, fill, side)
            return mem

        if not 0:
            wait(wo_copies(3))

            @pl.loop(0, NP)
            def _(t):
                for e0 in range(0, DH, 16):
                    wo_sums(3, t, e0)

            x_copy(0).wait()
            _spread([norm_tokens(0, 0), norm_tokens(0, 1)], 8, 1)()
            lax.fori_loop(0, n_it, steps, mem0_ref[...].astype(f32))
            for n in range(4):
                lower_wo(NSEG // 4 - 1, n, [0, 1, 2], {})

    pl.run_scoped(
        block_a,
        pltpu.VMEM((4, 2, SEG, D), bf16),
        pltpu.VMEM((2, SEG, D), f32),
        pltpu.VMEM((2, 3, 32, NP * DH), f32),
        *[pltpu.VMEM((NP, 4, HD, DH), bf16)] * 3,
        *[pltpu.VMEM((NP, 3, 8 * NSEG, DH), bf16)] * 3,
        *[pltpu.VMEM((4, NP, DH, 128), bf16)] * 7,
    )

    def block_b(gbuf, ustat, x1, obuf, yc, hc, db, nb0, nb1, ac0, ac1, pb0, pb1):
        def weights(n, at, rows, strips):
            return jnp.concatenate(
                [_load(*wsum[n], r0=at + k * rows[0] + rows[1], n=rows[2])
                 for k in strips], axis=1)

        ties = []
        never = jnp.full((8, 128), zero_ref[0]) != 0

        def before_next(value):
            value = jnp.broadcast_to(value, (16, 128))
            ties.append(pltpu.bitcast(value[:8] + value[8:], u32))

        def operand(ref, n, cols):
            words = [ref.bitcast(u32)[n, c] for c in cols]
            while ties:
                head = jnp.where(never, ties.pop(), words[-1][:8])
                words[-1] = jnp.concatenate([head, words[-1][8:]], axis=0)
            return jnp.concatenate([pltpu.bitcast(w, bf16) for w in words], axis=1)

        def store_sums(dst, r, c, x):
            def emit(n, v):
                v = v()
                dst[n, c, pl.ds(16 * r, 16), :] = v.astype(bf16)
                if n % 7 == 3 and 1 & (1 if dst is yc else 0 if dst is hc else 2):
                    before_next(v)
            return _sums2(_sums_a, x, emit)

        def inner(dst, p, product, side, add=False):
            def emit(a, b, v):
                dst[p, 2 * a + b] = dst[p, 2 * a + b] + v if add else v

            def run(k):
                r = product(7 * p + k)
                side()
                return r
            _combine(run, emit)

        def outer(src, r, cols, emit):
            for a in range(2):
                for b in range(2):
                    _combine(lambda p: src[p, 2 * a + b, pl.ds(16 * r, 16), cols],
                             lambda i, j, v: emit(2 * i + a, 2 * j + b, v))
                    yield

        def rows_of(i, g, r):
            return pl.ds(_mult(i * RB + g * R + 16 * r, 16), 16)

        def tied(stages):
            while True:
                try:
                    before_next(next(stages))
                except StopIteration as stop:
                    return stop.value
                yield
                yield

        def last_stats(i, r):
            return tied(h_stats(S - RB + i * R + 16 * r))

        def pre1(i, r):
            for c in range(2):
                x = []
                for g in range(4):
                    rows = rows_of(i, g, r)
                    x.append([(hbuf[2 * k + c, rows, :] - hstat[0, rows, :]) * hstat[2, rows, :]
                              for k in range(4)])
                yield from range(3)
                yield from store_sums(ac0, r, c, x)

        def post1(i, r):
            def emit(g, j, v):
                v = _gelu_of_double(v)
                gbuf[2 * j + c, pl.ds(HALO + i * RB + g * R + 16 * r, 16), :] = v
                if g >= 2 and j >= 2 and 0:
                    before_next(v)
            for c in range(2):
                for _ in outer(pb0, r, pl.ds(c * 128, 128), emit):
                    yield
                    yield

        def pre2(i, r):
            for c in range(2):
                x = [[gbuf[2 * k + c, pl.ds(HALO + i * RB + g * R + 16 * r + off, 16), :]
                      for k, off in enumerate((-1, 1, -2, 2))] for g in range(4)]
                yield from store_sums(ac1, r, c, x)

        def post2(i, r):
            def emit(g, j, v):
                rows = rows_of(i, g, r)
                x1[rows, pl.ds(j * C4, C4)] = v + jnp.concatenate(
                    [(hbuf[c, rows, :] - hstat[0, rows, :]) * hstat[1, rows, :]
                     for c in (2 * j, 2 * j + 1)], axis=1)
            for _ in outer(pb1, r, slice(None), emit):
                yield
                yield

        def pre3(i, r):
            for g in range(4):
                rows = rows_of(i, g, r)
                m, rs = yield from tied(_ln_stages(x1[rows, :]))
                ustat[0, rows_of(0, g, r), :] = jnp.broadcast_to(m, (16, 128))
                ustat[1, rows_of(0, g, r), :] = jnp.broadcast_to(0.5 * rs, (16, 128))
                before_next(rs)
                yield
                yield

        def sums3(i, r):
            for c in range(2):
                x = [[(x1[rows_of(i, g, r), pl.ds(k * C4 + c * 128, 128)]
                       - ustat[0, rows_of(0, g, r), :]) * ustat[1, rows_of(0, g, r), :]
                      for k in range(4)] for g in range(4)]
                yield from store_sums(yc, r, c, x)

        pieces = {pre1: 20, last_stats: 8, post1: 16, pre2: 14, post2: 8, pre3: 16, sums3: 14}

        def spread(stages, slots):
            stages = [(fn, i) for fn, i in stages if not isinstance(i, int) or 0 <= i < NB]
            return _spread([fn(i, r) for fn, i in stages for r in range(R // 16)],
                           sum(pieces[fn] for fn, _ in stages) * (R // 16), slots)

        def mixer(i, src, at, dst, stages):
            if not 0 <= i < NB:
                return spread(stages, 1)()
            side = spread(stages, 49)
            for p in range(7):
                inner(dst, p, lambda n: _dot(operand(src, n, (0, 1)),
                                             weights(n, at, (C4, 0, C4), (0, 1))),
                      side)

        if not 0:
            for c in range(8):
                gbuf[c, pl.ds(0, HALO), :] = jnp.zeros((HALO, 128), f32)
                gbuf[c, pl.ds(HALO + S, HALO), :] = jnp.zeros((HALO, 128), f32)
            for i in range(-1, NB + 3):
                mixer(i, ac0, W1_AT, pb0, [(pre2, i - 2), (post2, i - 3)]
                      + ([(last_stats, i)] if i < 4 else [(pre3, 0)] if i == NB - 1 else []))
                mixer(i - 2, ac1, W2_AT, pb1, [(pre1, i + 1), (post1, i)]
                      + {9: [(sums3, 0)]}.get(i, []))

        def out_copy(i):
            rows = pl.ds(_mult(i * (RB // 2), RB // 2), RB // 2)
            return pltpu.make_async_copy(obuf.at[rows], out_hbm.at[rows],
                                         sems.at[SEM_OUT + i])

        nb = (nb0, nb1)

        def activate(c, r):
            act = [[None] * 4 for _ in range(4)]

            def emit(g, j, v):
                act[g][j] = _gelu_of_double(v)
            for _ in outer(nb[c % 2], r, slice(None), emit):
                yield
                yield
            yield from store_sums(hc, r, c, act)

        pieces[activate] = 15

        def mlp_up():
            for c in range(7):
                side = spread([(activate, c - 1)], 49)
                for p in range(7):
                    inner(nb[c % 2], p, lambda n: _dot(
                        operand(yc, n, (0, 1)), weights(n, W3_AT, (C4, 0, C4), (c,))), side)

        def mlp_down(i, stages):
            def down(p, side, k0=0, k1=F4):
                inner(db, p, lambda n: _dot(operand(hc, n, range(k0 // 128, k1 // 128)),
                                            weights(n, W4_AT, (F4, k0, k1 - k0), (0, 1))),
                      side, add=k0 > 0)

            def finish(bi, bj, plus, minus=()):
                for a in range(2):
                    for b in range(2):
                        rows = pl.ds(_mult(i * RB + (2 * bi + a) * R, R), R)
                        cols = pl.ds((2 * bj + b) * C4, C4)
                        v = x1[rows, cols] + jnp.concatenate(
                            [hbuf[4 * bj + 2 * b + c, rows, :] for c in range(2)], axis=1)
                        for p in minus:
                            v = v - db[p, 2 * a + b]
                        for p in plus:
                            v = v + db[p, 2 * a + b]
                        obuf[rows, cols] = v.astype(bf16)

            down(0, spread([(activate, 6)], 6), 0, F4 - 128)
            down(0, lambda: None, F4 - 128)
            side = spread(stages, 35)
            for p in range(1, 7):
                down(p, side)
                if p == 3:
                    finish(0, 1, (1, 2))
                if p == 5:
                    finish(0, 0, (0, 3, 4), (1,))
            finish(1, 0, (4, 5))
            finish(1, 1, (2, 3, 6), (5,))

        if not 0:
            @pl.loop(0, NB)
            def _(i):
                ties.clear()
                mlp_up()
                nxt = jnp.minimum(i + 1, NB - 1)
                mlp_down(i, [(pre3, nxt), (sums3, nxt)])
                out_copy(2 * i).start()
                out_copy(2 * i + 1).start()

            for i in range(2 * NB):
                out_copy(i).wait()

    if 0:
        hbuf[0, :16] = sum(_load(*wsum[n], n=16).astype(f32) for n in range(49)) + hbuf[0, :16] + hstat[0, :16]
        cp = pltpu.make_async_copy(hbuf.at[0], hbuf.at[1], sems.at[0]); cp.start(); cp.wait()
    pl.run_scoped(
        block_b,
        pltpu.VMEM((8, S + 2 * HALO, 128), f32),
        pltpu.VMEM((2, RB, 128), f32),
        pltpu.VMEM((S, D), f32),
        pltpu.VMEM((S, D), bf16),
        pltpu.VMEM((49, 2, R, 128), bf16),
        pltpu.VMEM((49, 7, R, 128), bf16),
        pltpu.VMEM((7, 4, R, C4), f32),
        *[pltpu.VMEM((7, 4, R, 128), f32)] * 2,
        *[pltpu.VMEM((49, 2, R, 128), bf16)] * 2,
        *[pltpu.VMEM((7, 4, R, C4), f32)] * 2,
    )


@jax.jit
def pallas_sequential_preLN__memory_aug_recurrent_mem_tr__mixer_s_mlp__prompt_kernel(
    A_x: jax.Array,
    A_mem0: jax.Array,
    A_Wq: jax.Array,
    A_Wk: jax.Array,
    A_Wv: jax.Array,
    A_Wo: jax.Array,
    A_seg_len: jax.Array,
    B_x: jax.Array,
    B_w1: jax.Array,
    B_w2: jax.Array,
    B_w3: jax.Array,
    B_w4: jax.Array,
):
    del A_seg_len, B_x
    hbm = pl.BlockSpec(memory_space=pl.ANY)
    vmem = pl.BlockSpec(memory_space=pltpu.VMEM)
    scratch = [
        pltpu.VMEM((8, S, 128), f32),
        pltpu.VMEM((3, S, 128), f32),
        pltpu.SemaphoreType.DMA((NSEM,)),
        pltpu.SMEM((1,), jnp.int32),
    ] + [pltpu.VMEM((4, WROWS, 128), bf16)] * 4 + [pltpu.VMEM((WROWS, 128), bf16)] * 33
    out = pl.pallas_call(
        _kernel,
        out_shape=jax.ShapeDtypeStruct((S, D), A_x.dtype),
        in_specs=[hbm, vmem] + [hbm] * 8,
        out_specs=hbm,
        scratch_shapes=scratch,
        compiler_params=pltpu.CompilerParams(vmem_limit_bytes=128 * 1024 * 1024),
    )(A_x.reshape(NSEG, SEG, D), A_mem0.reshape(MEM, D),
      A_Wq.reshape(2, D // 4, 2 * H, DH), A_Wk.reshape(2, D // 4, 2 * H, DH),
      A_Wv.reshape(2, D // 4, 2 * H, DH), A_Wo.reshape(NP, 2, DH, D),
      B_w1.reshape(4, C4, D), B_w2.reshape(4, C4, D),
      B_w3.reshape(4, C4, F), B_w4.reshape(4, F4, D))
    return out.reshape(A_x.shape)
```

```python
import functools
import itertools

import jax
import jax.numpy as jnp
from jax import lax
import jax.experimental.pallas as pl
import jax.experimental.pallas.tpu as pltpu

S = 2048
D = 1024
H = 32
DH = 128
MEM = 8
SEG = 32
F = 3584
NSEG = S // SEG
NP = H // 2
HD = D // 2
C4 = D // 4
F4 = F // 4
HALO = 8
R = 64
RB = 4 * R
NB = S // RB
EPS = 1e-5
NEG = -1000000000.0
LOG2E = 1.4426950408889634

W1_AT, W2_AT, W3_AT, W4_AT = 0, 2 * C4, 4 * C4, 11 * C4
WROWS = W4_AT + 2 * F4
NSTRIP = 13

LAG_QK, LAG_PV, LAG_WO = 2, 4, 6
FILL = (17, 19, 99)

bf16 = jnp.bfloat16
f32 = jnp.float32
u32 = jnp.uint32

SEM_XP, SEM_X, SEM_WO, SEM_STRIP, SEM_OUT, SEM_W = 0, 8, 10, 14, 16, 16 + 2 * NB
NSEM = SEM_W + 12


def _mult(i, n):
    return i if isinstance(i, int) else pl.multiple_of(i, n)


def _ln_stats(x):
    m = jnp.mean(x, axis=-1, keepdims=True)
    d = x - m
    v = jnp.mean(d * d, axis=-1, keepdims=True)
    return m, lax.rsqrt(v + EPS)


def _ln_stages(x):
    m = jnp.mean(x, axis=-1, keepdims=True)
    yield m
    d = x - m
    r = lax.rsqrt(jnp.mean(d * d, axis=-1, keepdims=True) + EPS)
    return m, r


def _ln(x):
    m, r = _ln_stats(x)
    return (x - m) * r


def _gelu_of_double(y):
    c = 0.7978845608028654
    return y + y * jnp.tanh(y * (2 * c + (8 * c * 0.044715) * (y * y)))


def _dot(a, b):
    return jnp.dot(a, b, preferred_element_type=f32)


def _load(ref, *idx, r0=0, n=None):
    n = ref.shape[-2] if n is None else n
    return pltpu.bitcast(
        ref.bitcast(u32)[(*idx, pl.ds(_mult(r0 >> 1, 8), n // 2), slice(None))], bf16)


def _sums_a(a11, a12, a21, a22):
    return [lambda: a12 - a22, lambda: a11 + a12, lambda: a11, lambda: a11 + a22,
            lambda: a22, lambda: a21 + a22, lambda: a21 - a11]


def _sums_b(b11, b12, b21, b22):
    return [lambda: b21 + b22, lambda: b22, lambda: b12 - b22, lambda: b11 + b22,
            lambda: b21 - b11, lambda: b11, lambda: b11 + b12]


def _combine(product, emit):
    c11 = product(0)
    c12 = product(1)
    c11 = c11 - c12
    c22 = product(2)
    emit(0, 1, c12 + c22)
    t = product(3)
    c11 = c11 + t
    c22 = c22 + t
    c21 = product(4)
    emit(0, 0, c11 + c21)
    t = product(5)
    emit(1, 0, c21 + t)
    c22 = c22 - t
    emit(1, 1, c22 + product(6))


def _sums2(sums, x, emit):
    outer = [sums(x[i][j], x[i][2 + j], x[2 + i][j], x[2 + i][2 + j])
             for i in range(2) for j in range(2)]
    for p in range(7):
        for q, v in enumerate(sums(*(o[p]() for o in outer))):
            emit(7 * p + q, v)
        yield


def _spread(tasks, pieces, slots):
    todo = itertools.chain(*tasks)
    calls = itertools.count(1)

    def advance():
        k = next(calls)
        if k > slots:
            return
        for _ in range(pieces * k // slots - pieces * (k - 1) // slots):
            next(todo)
        if k == slots:
            assert next(todo, todo) is todo
    return advance


def _tie(never, words, values, first=0):
    regs = [[w[r:r + 8] for r in range(0, w.shape[0], 8)] for w in words]
    per = len(regs[0])
    for n, v in enumerate(values):
        c, r = divmod(first + (len(regs) * per - first) * n // len(values), per)
        regs[c][r] = jnp.where(never, pltpu.bitcast(v, u32), regs[c][r])
    return [jnp.concatenate(w, axis=0) for w in regs] if values else words


def _upper_operands(a11, a12, a22):
    k = a11.shape[0] - a22.shape[0]
    ops = [jnp.concatenate([a12[:k], a12[k:] - a22], axis=0), a11 + a12, a11,
           jnp.concatenate([a11[:k], a11[k:] + a22], axis=0)]
    return [v.astype(bf16) for v in ops]


PLAIN = {40: 0, 36: 1, 12: 2, 8: 3}
OTHER = [n for n in range(49) if n not in PLAIN]
RAW_SLOT = dict(zip(OTHER[2::3], [(k, j) for k in range(4) for j in range(4) if k != j]))
RAW_SLOT.update({n: (k, k) for n, k in PLAIN.items()})


def _kernel(x_hbm, mem0_ref, wq_hbm, wk_hbm, wv_hbm, wo_hbm, w1_hbm, w2_hbm,
            w3_hbm, w4_hbm, out_hbm, hbuf, hstat, sems, zero_ref, *wbufs):
    zero_ref[0] = 0
    raw, spare = wbufs[:4], wbufs[4:]
    wsum = {n: (raw[j], k) for n, (k, j) in RAW_SLOT.items()}
    wsum.update({n: (b,) for n, b in zip((n for n in OTHER if n not in RAW_SLOT), spare)})

    def load_h(rows):
        return jnp.concatenate([hbuf[c, rows, :] for c in range(8)], axis=1)

    def h_stats(r0, n=16):
        rows = pl.ds(_mult(r0, 16), n)
        hv = load_h(rows)
        m1, r1 = yield from _ln_stages(hv)
        yield r1
        m2, r2 = yield from _ln_stages((hv - m1) * r1)
        stats = (m1 + m2 / r1, r1, 0.5 * r1 * r2)
        for k, v in enumerate(stats):
            hstat[k, rows, :] = jnp.broadcast_to(v, (n, 128))
        yield stats[0] + stats[2]

    def strip_copies(u, fn):
        for lo, hi, w, at in ((0, 2, w1_hbm, W1_AT), (2, 4, w2_hbm, W2_AT),
                              (4, 11, w3_hbm, W3_AT), (11, 13, w4_hbm, W4_AT)):
            def run(lo=lo, w=w, at=at):
                n = w.shape[1]
                for j in range(4):
                    cols = pl.ds(_mult(j * (w.shape[2] // 4) + (u - lo) * 128, 128), 128)
                    fn(pltpu.make_async_copy(
                        w.at[:, :, cols],
                        raw[j].at[:, pl.ds(_mult(at + (u - lo) * n, 128), n), :],
                        sems.at[SEM_STRIP + (u & 1)]))
            if isinstance(u, int):
                if lo <= u < hi:
                    run()
            else:
                pl.when((u >= lo) & (u < hi))(run)

    def weight_sums(r0):
        x = [[_load(raw[j], k, r0=r0, n=16).astype(f32) for j in range(4)]
             for k in range(4)]

        def emit(n, v):
            if n not in PLAIN:
                ref, *idx = wsum[n]
                ref[(*idx, pl.ds(_mult(r0, 16), 16), slice(None))] = v().astype(bf16)
        yield from _sums2(_sums_b, x, emit)

    def block_a(xb, xn, lo, *bufs):
        w_on, low, wo_s = bufs[0:3], bufs[3:6], bufs[6:13]
        w_hbm = (wq_hbm, wk_hbm, wv_hbm)
        stage = hbuf.reshape(8, hbuf.shape[1] // 8, 8, DH)
        lhs = spare[2:5]
        w_low = [spare[5 + 3 * m:8 + 3 * m] for m in range(3)]

        def x_copy(i):
            return pltpu.make_async_copy(x_hbm.at[pl.ds(2 * i, 2)], xb.at[i & 3],
                                         sems.at[SEM_X + (i & 1)])

        def wo_copies(n):
            return [pltpu.make_async_copy(
                wo_hbm.at[:, i, :, pl.ds(_mult(j * HD + n * 128, 128), 128)],
                wo_s[slot].at[n], sems.at[SEM_WO + n])
                for slot, i, j in ((5, 0, 0), (2, 0, 1), (4, 1, 0), (1, 1, 1))]

        def chunk_copies(g, m):
            src = w_hbm[m].bitcast(f32)
            return [pltpu.make_async_copy(
                src.at[:, :, pl.ds(_mult(16 * par + 4 * g, 4), 4), :],
                stage.at[pl.ds(2 * m, 2), pl.ds(0, S // 8), pl.ds(4 * par, 4), :],
                sems.at[SEM_W + 3 * g + m]) for par in range(2)]

        def start(copies):
            for c in copies:
                c.start()

        def wait(copies):
            for c in copies:
                c.wait()

        def qkv_sums(g, m, pair, d0):
            b = []
            for half in range(2):
                w = pltpu.bitcast(
                    hbuf[2 * m + half, pl.ds(4 * d0 + pair, 16, stride=4), :], u32)
                b += [pltpu.bitcast(w << 16, f32),
                      pltpu.bitcast(w & jnp.uint32(0xFFFF0000), f32)]
            for k, v in enumerate(_sums_b(*b)):
                v = v()
                if k < 4:
                    w_on[m][4 * g + pair, k, pl.ds(d0, 16), :] = v.astype(bf16)
                else:
                    w_low[m][k - 4][pl.ds(_mult(pair * HD + d0, 16), 16), :] = v.astype(bf16)
            return v

        def wo_sums(n, t, e0):
            b = [_load(wo_s[k], n, t, r0=e0, n=16).astype(f32) for k in (5, 2, 4, 1)]
            for k, v in enumerate(_sums_b(*b)):
                if k not in (1, 5):
                    v = v()
                    wo_s[k][n, t, pl.ds(e0, 16), :] = v.astype(bf16)
            return v

        def prologue(xpb):
            def xp_copy(i):
                segs = pl.ds(8 * i, 8)
                return pltpu.make_async_copy(x_hbm.at[segs, pl.ds(16, 16), :], xpb.at[segs],
                                             sems.at[SEM_XP + i])

            start(chunk_copies(0, 0))
            start([xp_copy(i) for i in range(NSEG // 8)])
            start(chunk_copies(0, 1))
            start(chunk_copies(0, 2))
            lo[...] = jnp.zeros(lo.shape, f32)
            for k in (5, 2, 4, 1):
                wo_s[k][3] = jnp.zeros(wo_s[k].shape[1:], bf16)
            wait(chunk_copies(0, 0))

            @pl.loop(0, 4)
            def _(pair):
                for d0 in range(0, HD, 16):
                    qkv_sums(0, 0, pair, d0)

            @pl.loop(0, NSEG // 8)
            def _(i):
                xp_copy(i).wait()
                for j in range(4):
                    a = [_ln(_load(xpb, 8 * i + 2 * j + k).astype(f32)) for k in range(2)]
                    a1 = jnp.concatenate([a[0][:8], a[1][:8]], axis=0)
                    a2 = jnp.concatenate([a[0][8:], a[1][8:]], axis=0)
                    ops = _sums_a(a1[:, :HD], a1[:, HD:], a2[:, :HD], a2[:, HD:])
                    ops = [v() for v in ops[4:]]
                    for k in range(3):
                        for c in range(4):
                            rows = pl.ds(pl.multiple_of(c * 8 * NSEG + 64 * i + 16 * j, 16), 16)
                            lhs[k][rows, :] = ops[k][:, c * 128:(c + 1) * 128].astype(bf16)

        if not 0:
            pl.run_scoped(prologue, pltpu.VMEM((NSEG, 16, D), bf16))

        def lower_products(g, m):
            m1 = (m + 1) % 3
            never = jnp.full((8, 128), zero_ref[0]) != 0
            g1 = jnp.minimum(g + (1 if m == 2 else 0), 3)
            side = [functools.partial(qkv_sums, g1, m1, pair, d0)
                    for d0 in range(0, HD, 16) for pair in range(4)]
            wait_at = 7
            span = 12 - wait_at
            early = [functools.partial(wo_sums, (g + 3) & 3, t, e0)
                     for t in ((), range(0, 8), range(8, NP))[m] for e0 in range(0, DH, 16)]
            for j in range(12):
                pair, k = divmod(j, 3)
                if j >= wait_at:
                    todo = side[len(side) * (j - wait_at) // span:
                                len(side) * (j - wait_at + 1) // span]
                else:
                    todo = early[len(early) * j // wait_at:len(early) * (j + 1) // wait_at]
                a = [lhs[k].bitcast(u32)[pl.ds(c * 4 * NSEG, 4 * NSEG), :] for c in range(4)]
                a[3:] = _tie(never, a[3:], [fn()[8:] for fn in todo], 8)
                a = jnp.concatenate([pltpu.bitcast(v, bf16) for v in a], axis=1)
                res = _dot(a, _load(w_low[m][k], r0=pair * HD, n=HD))
                if j == wait_at - 1:
                    pl.when(3 * g + m < 11)(lambda: wait(chunk_copies(g1, m1)))
                    pl.when(g < 3)(lambda: start(chunk_copies(g + 1, m)))
                    if m == 0:
                        pl.when(g > 0)(lambda: wait(wo_copies(g - 1)))
                        start(wo_copies(g))

                        @pl.when(g == 3)
                        def _():
                            x_copy(0).start()
                            x_copy(1).start()
                            strip_copies(0, lambda c: c.start())
                if k == 0:
                    m4 = res
                    low[m][4 * g + pair, 0] = m4.astype(bf16)
                elif k == 1:
                    m2 = res
                    low[m][4 * g + pair, 1] = (m2 + m4).astype(bf16)
                else:
                    low[m][4 * g + pair, 2] = (res - m2).astype(bf16)

        if not 0:
            @pl.loop(0, 4)
            def _(g):
                for m in range(3):
                    lower_products(g, m)

        def norm_tokens(i, k):
            for r0 in range(0, SEG, 16):
                v = _load(xb, jnp.minimum(i, NSEG // 2 - 1) & 3, k, r0=r0, n=16).astype(f32)
                m, r = yield from _ln_stages(v)
                xn[k, pl.ds(r0, 16), :] = (v - m) * r
                yield r

        def lower_wo(grp, n, parts, state):
            for k in parts:
                w = jnp.concatenate([_load(wo_s[4 + k], n, t) for t in range(NP)], axis=0)
                state[k] = _dot(lo[grp & 1, k].astype(bf16), w)
            if 2 in parts:
                m4, m2, m6 = state[0], state[1], state[2]
                base = jnp.maximum(grp, 0) * (4 * SEG)
                for j in range(4):
                    seg = slice(8 * j, 8 * j + 8)
                    upper = pl.ds(pl.multiple_of(base + j * SEG + 16, 8), 8)
                    lower = pl.ds(pl.multiple_of(base + j * SEG + 24, 8), 8)
                    hbuf[n, upper, :] += m4[seg]
                    hbuf[n, lower, :] += m2[seg] + m4[seg]
                    hbuf[4 + n, lower, :] += m6[seg] - m2[seg]

        def attention_mask():
            def split(axis):
                r = lax.broadcasted_iota(jnp.int32, (80, 80), axis)
                return (jnp.where(r < 64, r >> 5, (r - 64) >> 3),
                        jnp.where(r < 64, r & 31, 32 + (r & 7)))
            (hq, pq), (hk, pk) = split(0), split(1)
            visible = (pq < MEM) | (pq >= pk)
            return jnp.where(hq == hk, jnp.where(visible, 0.0, NEG * DH ** 0.5), -jnp.inf)

        def step(i, k, mem, fill, side):
            tok = xn[k]
            r0 = jnp.maximum(2 * i + k - 8, 0) * SEG
            norms = itertools.chain(h_stats(r0), h_stats(r0 + 16), norm_tokens(i + 1, k))
            s = 2 * i + k
            xv = _load(xb, jnp.minimum(i, NSEG // 2 - 1) & 3, k).astype(f32)
            for c in range(8):
                hbuf[c, pl.ds(pl.multiple_of(s * SEG, SEG), SEG), :] = xv[:, c * 128:(c + 1) * 128]
            a1 = jnp.concatenate([mem, tok[:24]], axis=0)
            ops = _upper_operands(a1[:, :HD], a1[:, HD:], tok[24:, HD:])
            qkvs, scores, outs, lower = {}, {}, {}, {}
            total = [None] * 4

            def qkv(t):
                res = []
                for m in range(3):
                    m7, m5, m3, m1 = [_dot(ops[j], _load(w_on[m], t, j)) for j in range(4)]
                    m4, c21, m62 = [
                        _load(low[m], t, j, r0=16 * i, n=16).astype(f32)[8 * k:8 * k + 8]
                        for j in range(3)]
                    side()
                    c11 = m7 - m5 + m1
                    res.append(jnp.concatenate(
                        [c11[:24], c11[24:] + m4, m5 + m3, c21, m3[24:] + m62 + m1[24:]],
                        axis=0).astype(bf16))
                qkvs[t] = res

            def qk(t):
                q, kk, v = qkvs.pop(t)
                sc = lax.dot_general(q, kk, (((1,), (1,)), ((), ())),
                                     preferred_element_type=f32)
                scores[t] = (sc, v)

            def pv(t):
                sc, v = scores.pop(t)
                sc = jnp.where(fill == 0.0, sc, fill)
                tie = next(norms, None) if t >= 0 else None
                if tie is not None:
                    sc = jnp.concatenate([jnp.where(never, tie, sc[:16]), sc[16:]], axis=0)
                mx = jnp.max(sc, axis=1, keepdims=True)
                e = jnp.exp2((sc - mx) * (DH ** -0.5 * LOG2E))
                den = jnp.sum(e, axis=1, keepdims=True)
                inv = pl.reciprocal(den, approx=True)
                inv = inv * (2.0 - den * inv)
                outs[t] = _dot(e.astype(bf16), v) * inv

            def wo(t):
                o = outs.pop(t)
                a11, a12, a21, a22 = o[:32], o[32:64], o[64:72], o[72:]
                rows = pl.ds(pl.multiple_of(8 * (s & 3), 8), 8)
                for j, v in enumerate((a22, a21 + a22, a21 - a11[24:])):
                    lo[(s >> 2) & 1, j, rows, pl.ds(t * DH, DH)] = v
                r = [_dot(a, jnp.concatenate([_load(wo_s[j], n, t) for n in range(4)], axis=1))
                     for j, a in enumerate(_upper_operands(a11, a12, a22))]
                if 0:
                    r = [r[0] - r[1] + r[3], r[1] + r[2], r[2][24:] + r[3][24:]]
                for j, v in enumerate(r):
                    total[j] = v if total[j] is None else total[j] + v

            def attend(t):
                if t % 2 == 1:
                    todo = [(qk, LAG_QK), (pv, LAG_PV)]
                    for fn, lag in todo[::-1] if 0 else todo:
                        for u in (t - 1 - lag, t - lag):
                            if 0 <= u < NP:
                                fn(u)

            for t in range(NP + LAG_WO):
                if 1 == 0:
                    attend(t)
                if t < NP:
                    qkv(t)
                lower_wo((s >> 2) - 1, s & 3, [j for j in range(3) if FILL[j] == t], lower)
                if 1 == 1:
                    attend(t)
                if 0 <= t - LAG_WO < NP:
                    wo(t - LAG_WO)
            lower_wo((s >> 2) - 1, s & 3, [j for j in range(3) if j not in lower], lower)

            if 0:
                upper, c22 = jnp.concatenate(total[:2], axis=1), total[2]
            else:
                m7, m5, m3, m1 = total
                upper = jnp.concatenate([m7 - m5 + m1, m5 + m3], axis=1)
                c22 = m3[24:] + m1[24:]
            for c in range(8):
                hbuf[c, pl.ds(pl.multiple_of(s * SEG, SEG), 24), :] += (
                    upper[MEM:, c * 128:(c + 1) * 128])
            for c in range(4):
                hbuf[4 + c, pl.ds(pl.multiple_of(s * SEG + 24, 8), 8), :] += (
                    c22[:, c * 128:(c + 1) * 128])
            return upper[:MEM]

        fill = attention_mask()
        never = jnp.full((16, 80), zero_ref[0]) != 0
        n_it = NSEG // 2
        per_it = WROWS // 16 // n_it

        def steps(i, mem):
            pl.when(i + 1 < n_it)(lambda: x_copy(i + 1).wait())
            pl.when(i + 2 < n_it)(lambda: x_copy(i + 2).start())

            @pl.when(i < NSTRIP)
            def _():
                strip_copies(i, lambda c: c.wait())
                strip_copies(i + 1, lambda c: c.start())

            side = _spread([weight_sums(16 * (per_it * i + j)) for j in range(per_it)],
                           7 * per_it, 72)
            for k in range(2):
                mem = step(i, k, mem, fill, side)
            return mem

        if 0:
            hbuf[0, :16] = sum(b[0, 0, :16].astype(f32) for b in bufs)
        else:
            wait(wo_copies(3))

            @pl.loop(0, NP)
            def _(t):
                for e0 in range(0, DH, 16):
                    wo_sums(3, t, e0)

            x_copy(0).wait()
            _spread([norm_tokens(0, 0), norm_tokens(0, 1)], 8, 1)()
            lax.fori_loop(0, n_it, steps, mem0_ref[...].astype(f32))
            for n in range(4):
                lower_wo(NSEG // 4 - 1, n, [0, 1, 2], {})

    pl.run_scoped(
        block_a,
        pltpu.VMEM((4, 2, SEG, D), bf16),
        pltpu.VMEM((2, SEG, D), f32),
        pltpu.VMEM((2, 3, 32, NP * DH), f32),
        *[pltpu.VMEM((NP, 4, HD, DH), bf16)] * 3,
        *[pltpu.VMEM((NP, 3, 8 * NSEG, DH), bf16)] * 3,
        *[pltpu.VMEM((4, NP, DH, 128), bf16)] * 7,
    )

    def block_b(gbuf, ustat, x1, obuf, yc, hc, db, nb0, nb1, ac0, ac1, pb0, pb1):
        def weights(n, at, rows, strips):
            return jnp.concatenate(
                [_load(*wsum[n], r0=at + k * rows[0] + rows[1], n=rows[2])
                 for k in strips], axis=1)

        ties = []
        never = jnp.full((8, 128), zero_ref[0]) != 0

        def before_next(value):
            if value.shape[1] == 1:
                value = jnp.broadcast_to(value[:8] + value[8:], (8, 128))
            ties.append(value[-8:, -128:])

        def operand(ref, n, cols):
            words = [ref.bitcast(u32)[n, c] for c in cols]
            words = _tie(never, words, ties)
            ties.clear()
            return jnp.concatenate([pltpu.bitcast(w, bf16) for w in words], axis=1)

        def store_sums(dst, r, c, x, tie=True):
            def emit(n, v):
                v = v()
                dst[n, c, pl.ds(16 * r, 16), :] = v.astype(bf16)
                if tie and n % 2:
                    before_next(v)
            return _sums2(_sums_a, x, emit)

        def inner(dst, p, product, side, add=False):
            def emit(a, b, v):
                dst[p, 2 * a + b] = dst[p, 2 * a + b] + v if add else v

            def run(k):
                r = product(7 * p + k)
                side()
                return r
            _combine(run, emit)

        def outer(src, r, cols, emit):
            for a in range(2):
                for b in range(2):
                    _combine(lambda p: src[p, 2 * a + b, pl.ds(16 * r, 16), cols],
                             lambda i, j, v: emit(2 * i + a, 2 * j + b, v))
                    yield

        def rows_of(i, g, r):
            return pl.ds(_mult(i * RB + g * R + 16 * r, 16), 16)

        def tied(stages):
            while True:
                try:
                    before_next(next(stages))
                except StopIteration as stop:
                    return stop.value
                yield
                yield

        def last_stats(i, r):
            return tied(h_stats(S - RB + i * R + 16 * r))

        def pre1(i, r):
            for c in range(2):
                x = []
                for g in range(4):
                    rows = rows_of(i, g, r)
                    x.append([(hbuf[2 * k + c, rows, :] - hstat[0, rows, :]) * hstat[2, rows, :]
                              for k in range(4)])
                yield from range(3)
                yield from store_sums(ac0, r, c, x)

        def post1(i, r):
            def emit(g, j, v):
                v = _gelu_of_double(v)
                gbuf[2 * j + c, pl.ds(HALO + i * RB + g * R + 16 * r, 16), :] = v
            for c in range(2):
                for _ in outer(pb0, r, pl.ds(c * 128, 128), emit):
                    yield
                    yield

        def pre2(i, r):
            for c in range(2):
                x = [[gbuf[2 * k + c, pl.ds(HALO + i * RB + g * R + 16 * r + off, 16), :]
                      for k, off in enumerate((-1, 1, -2, 2))] for g in range(4)]
                yield from store_sums(ac1, r, c, x)

        def post2(i, r):
            def emit(g, j, v):
                rows = rows_of(i, g, r)
                v = v + jnp.concatenate(
                    [(hbuf[c, rows, :] - hstat[0, rows, :]) * hstat[1, rows, :]
                     for c in (2 * j, 2 * j + 1)], axis=1)
                x1[rows, pl.ds(j * C4, C4)] = v
            for _ in outer(pb1, r, slice(None), emit):
                yield
                yield

        def pre3(i, r):
            for g in range(4):
                rows = rows_of(i, g, r)
                m, rs = yield from tied(_ln_stages(x1[rows, :]))
                ustat[0, rows_of(0, g, r), :] = jnp.broadcast_to(m, (16, 128))
                ustat[1, rows_of(0, g, r), :] = jnp.broadcast_to(0.5 * rs, (16, 128))
                before_next(rs)
                yield
                yield

        def sums3(i, r):
            for c in range(2):
                x = [[(x1[rows_of(i, g, r), pl.ds(k * C4 + c * 128, 128)]
                       - ustat[0, rows_of(0, g, r), :]) * ustat[1, rows_of(0, g, r), :]
                      for k in range(4)] for g in range(4)]
                yield from store_sums(yc, r, c, x, isinstance(i, int))

        pieces = {pre1: 20, last_stats: 8, post1: 16, pre2: 14, post2: 8, pre3: 16, sums3: 14}

        def spread(stages, slots):
            stages = [(fn, i) for fn, i in stages if not isinstance(i, int) or 0 <= i < NB]
            return _spread([fn(i, r) for fn, i in stages for r in range(R // 16)],
                           sum(pieces[fn] for fn, _ in stages) * (R // 16), slots)

        def mixer(i, src, at, dst, stages):
            if not 0 <= i < NB:
                return spread(stages, 1)()
            side = spread(stages, 49)
            for p in range(7):
                inner(dst, p, lambda n: _dot(operand(src, n, (0, 1)),
                                             weights(n, at, (C4, 0, C4), (0, 1))),
                      side)

        if not 0:
            for c in range(8):
                gbuf[c, pl.ds(0, HALO), :] = jnp.zeros((HALO, 128), f32)
                gbuf[c, pl.ds(HALO + S, HALO), :] = jnp.zeros((HALO, 128), f32)
            for i in range(-1, NB + 3):
                mixer(i, ac0, W1_AT, pb0, [(pre2, i - 2), (post2, i - 3)]
                      + ([(last_stats, i)] if i < 4 else [(pre3, 0)] if i == NB - 1 else []))
                mixer(i - 2, ac1, W2_AT, pb1, [(pre1, i + 1), (post1, i)]
                      + {9: [(sums3, 0)]}.get(i, []))

        def out_copy(i):
            rows = pl.ds(_mult(i * (RB // 2), RB // 2), RB // 2)
            return pltpu.make_async_copy(obuf.at[rows], out_hbm.at[rows],
                                         sems.at[SEM_OUT + i])

        nb = (nb0, nb1)

        def activate(c, r):
            act = [[None] * 4 for _ in range(4)]

            def emit(g, j, v):
                act[g][j] = _gelu_of_double(v)
            for _ in outer(nb[c % 2], r, slice(None), emit):
                yield
                yield
            yield from store_sums(hc, r, c, act, False)

        pieces[activate] = 15

        def mlp_up():
            for c in range(7):
                side = spread([(activate, c - 1)], 49)
                for p in range(7):
                    inner(nb[c % 2], p, lambda n: _dot(
                        operand(yc, n, (0, 1)), weights(n, W3_AT, (C4, 0, C4), (c,))), side)

        def mlp_down(i, stages):
            def down(p, side, k0=0, k1=F4):
                inner(db, p, lambda n: _dot(operand(hc, n, range(k0 // 128, k1 // 128)),
                                            weights(n, W4_AT, (F4, k0, k1 - k0), (0, 1))),
                      side, add=k0 > 0)

            def finish(bi, bj, plus, minus=()):
                for a in range(2):
                    for b in range(2):
                        rows = pl.ds(_mult(i * RB + (2 * bi + a) * R, R), R)
                        cols = pl.ds((2 * bj + b) * C4, C4)
                        v = x1[rows, cols] + jnp.concatenate(
                            [hbuf[4 * bj + 2 * b + c, rows, :] for c in range(2)], axis=1)
                        for p in minus:
                            v = v - db[p, 2 * a + b]
                        for p in plus:
                            v = v + db[p, 2 * a + b]
                        obuf[rows, cols] = v.astype(bf16)

            down(0, spread([(activate, 6)], 6), 0, F4 - 128)
            down(0, lambda: None, F4 - 128)
            side = spread(stages, 35)
            for p in range(1, 7):
                down(p, side)
                if p == 3:
                    finish(0, 1, (1, 2))
                if p == 5:
                    finish(0, 0, (0, 3, 4), (1,))
            finish(1, 0, (4, 5))
            finish(1, 1, (2, 3, 6), (5,))

        if not 0:
            @pl.loop(0, NB)
            def _(i):
                ties.clear()
                mlp_up()
                nxt = jnp.minimum(i + 1, NB - 1)
                mlp_down(i, [(pre3, nxt), (sums3, nxt)])
                out_copy(2 * i).start()
                out_copy(2 * i + 1).start()

            for i in range(2 * NB):
                out_copy(i).wait()

    if 0:
        hbuf[0, :16] = sum(_load(*wsum[n], n=16).astype(f32) for n in range(49)) + hbuf[0, :16] + hstat[0, :16]
        cp = pltpu.make_async_copy(hbuf.at[0], hbuf.at[1], sems.at[0]); cp.start(); cp.wait()
    pl.run_scoped(
        block_b,
        pltpu.VMEM((8, S + 2 * HALO, 128), f32),
        pltpu.VMEM((2, RB, 128), f32),
        pltpu.VMEM((S, D), f32),
        pltpu.VMEM((S, D), bf16),
        pltpu.VMEM((49, 2, R, 128), bf16),
        pltpu.VMEM((49, 7, R, 128), bf16),
        pltpu.VMEM((7, 4, R, C4), f32),
        *[pltpu.VMEM((7, 4, R, 128), f32)] * 2,
        *[pltpu.VMEM((49, 2, R, 128), bf16)] * 2,
        *[pltpu.VMEM((7, 4, R, C4), f32)] * 2,
    )


@jax.jit
def pallas_sequential_preLN__memory_aug_recurrent_mem_tr__mixer_s_mlp__prompt_kernel(
    A_x: jax.Array,
    A_mem0: jax.Array,
    A_Wq: jax.Array,
    A_Wk: jax.Array,
    A_Wv: jax.Array,
    A_Wo: jax.Array,
    A_seg_len: jax.Array,
    B_x: jax.Array,
    B_w1: jax.Array,
    B_w2: jax.Array,
    B_w3: jax.Array,
    B_w4: jax.Array,
):
    del A_seg_len, B_x
    hbm = pl.BlockSpec(memory_space=pl.ANY)
    vmem = pl.BlockSpec(memory_space=pltpu.VMEM)
    scratch = [
        pltpu.VMEM((8, S, 128), f32),
        pltpu.VMEM((3, S, 128), f32),
        pltpu.SemaphoreType.DMA((NSEM,)),
        pltpu.SMEM((1,), jnp.int32),
    ] + [pltpu.VMEM((4, WROWS, 128), bf16)] * 4 + [pltpu.VMEM((WROWS, 128), bf16)] * 33
    out = pl.pallas_call(
        _kernel,
        out_shape=jax.ShapeDtypeStruct((S, D), A_x.dtype),
        in_specs=[hbm, vmem] + [hbm] * 8,
        out_specs=hbm,
        scratch_shapes=scratch,
        compiler_params=pltpu.CompilerParams(vmem_limit_bytes=128 * 1024 * 1024),
    )(A_x.reshape(NSEG, SEG, D), A_mem0.reshape(MEM, D),
      A_Wq.reshape(2, D // 4, 2 * H, DH), A_Wk.reshape(2, D // 4, 2 * H, DH),
      A_Wv.reshape(2, D // 4, 2 * H, DH), A_Wo.reshape(NP, 2, DH, D),
      B_w1.reshape(4, C4, D), B_w2.reshape(4, C4, D),
      B_w3.reshape(4, C4, F), B_w4.reshape(4, F4, D))
    return out.reshape(A_x.shape)
```

```python
import functools
import itertools

import jax
import jax.numpy as jnp
from jax import lax
import jax.experimental.pallas as pl
import jax.experimental.pallas.tpu as pltpu

S = 2048
D = 1024
H = 32
DH = 128
MEM = 8
SEG = 32
F = 3584
NSEG = S // SEG
NP = H // 2
HD = D // 2
C4 = D // 4
F4 = F // 4
HALO = 8
R = 64
RB = 4 * R
NB = S // RB
EPS = 1e-5
NEG = -1000000000.0
LOG2E = 1.4426950408889634

W1_AT, W2_AT, W3_AT, W4_AT = 0, 2 * C4, 4 * C4, 11 * C4
WROWS = W4_AT + 2 * F4
BATCH = (0, 1, 6, 11, 13, 13)

LAG_QK, LAG_PV, LAG_WO = 2, 4, 6
FILL = (16, 18, 99)

bf16 = jnp.bfloat16
f32 = jnp.float32
u32 = jnp.uint32

SEM_XP, SEM_X, SEM_WO, SEM_STRIP, SEM_OUT, SEM_W = 0, 8, 10, 14, 16, 16 + 2 * NB
NSEM = SEM_W + 12


def _mult(i, n):
    return i if isinstance(i, int) else pl.multiple_of(i, n)


def _ln_stats(x):
    m = jnp.mean(x, axis=-1, keepdims=True)
    d = x - m
    v = jnp.mean(d * d, axis=-1, keepdims=True)
    return m, lax.rsqrt(v + EPS)


def _ln_stages(x):
    m = jnp.mean(x, axis=-1, keepdims=True)
    yield m
    d = x - m
    r = lax.rsqrt(jnp.mean(d * d, axis=-1, keepdims=True) + EPS)
    return m, r


def _ln(x):
    m, r = _ln_stats(x)
    return (x - m) * r


def _gelu_of_double(y):
    c = 0.7978845608028654
    return y + y * jnp.tanh(y * (2 * c + (8 * c * 0.044715) * (y * y)))


def _dot(a, b):
    return jnp.dot(a, b, preferred_element_type=f32)


def _load(ref, *idx, r0=0, n=None):
    n = ref.shape[-2] if n is None else n
    return pltpu.bitcast(
        ref.bitcast(u32)[(*idx, pl.ds(_mult(r0 >> 1, 8), n // 2), slice(None))], bf16)


def _sums_a(a11, a12, a21, a22):
    return [lambda: a12 - a22, lambda: a11 + a12, lambda: a11, lambda: a11 + a22,
            lambda: a22, lambda: a21 + a22, lambda: a21 - a11]


def _sums_b(b11, b12, b21, b22):
    return [lambda: b21 + b22, lambda: b22, lambda: b12 - b22, lambda: b11 + b22,
            lambda: b21 - b11, lambda: b11, lambda: b11 + b12]


def _combine(product, emit):
    c11 = product(0)
    c12 = product(1)
    c11 = c11 - c12
    c22 = product(2)
    emit(0, 1, c12 + c22)
    t = product(3)
    c11 = c11 + t
    c22 = c22 + t
    c21 = product(4)
    emit(0, 0, c11 + c21)
    t = product(5)
    emit(1, 0, c21 + t)
    c22 = c22 - t
    emit(1, 1, c22 + product(6))


def _sums2(sums, x, emit):
    outer = [sums(x[i][j], x[i][2 + j], x[2 + i][j], x[2 + i][2 + j])
             for i in range(2) for j in range(2)]
    for p in range(7):
        for q, v in enumerate(sums(*(o[p]() for o in outer))):
            emit(7 * p + q, v)
        yield


def _spread(tasks, pieces, slots):
    todo = itertools.chain(*tasks)
    calls = itertools.count(1)

    def advance():
        k = next(calls)
        if k > slots:
            return
        for _ in range(pieces * k // slots - pieces * (k - 1) // slots):
            next(todo)
        if k == slots:
            assert next(todo, todo) is todo
    return advance


def _tie(never, words, values, first=0):
    regs = [[w[r:r + 8] for r in range(0, w.shape[0], 8)] for w in words]
    per = len(regs[0])
    for n, v in enumerate(values):
        c, r = divmod(first + (len(regs) * per - first) * n // len(values), per)
        regs[c][r] = jnp.where(never, pltpu.bitcast(v, u32), regs[c][r])
    return [jnp.concatenate(w, axis=0) for w in regs] if values else words


def _upper_operands(a11, a12, a22):
    k = a11.shape[0] - a22.shape[0]
    ops = [jnp.concatenate([a12[:k], a12[k:] - a22], axis=0), a11 + a12, a11,
           jnp.concatenate([a11[:k], a11[k:] + a22], axis=0)]
    return [v.astype(bf16) for v in ops]


PLAIN = {40: 0, 36: 1, 12: 2, 8: 3}
OTHER = [n for n in range(49) if n not in PLAIN]
RAW_SLOT = dict(zip(OTHER[2::3], [(k, j) for k in range(4) for j in range(4) if k != j]))
RAW_SLOT.update({n: (k, k) for n, k in PLAIN.items()})


def _kernel(x_hbm, mem0_ref, wq_hbm, wk_hbm, wv_hbm, wo_hbm, w1_hbm, w2_hbm,
            w3_hbm, w4_hbm, out_hbm, hbuf, hstat, sems, zero_ref, *wbufs):
    zero_ref[0] = 0
    raw, spare = wbufs[:4], wbufs[4:]
    wsum = {n: (raw[j], k) for n, (k, j) in RAW_SLOT.items()}
    wsum.update({n: (b,) for n, b in zip((n for n in OTHER if n not in RAW_SLOT), spare)})

    def load_h(rows):
        return jnp.concatenate([hbuf[c, rows, :] for c in range(8)], axis=1)

    def h_stats(r0, n=16):
        rows = pl.ds(_mult(r0, 16), n)
        hv = load_h(rows)
        m1, r1 = yield from _ln_stages(hv)
        yield r1
        m2, r2 = yield from _ln_stages((hv - m1) * r1)
        stats = (m1 + m2 / r1, r1, 0.5 * r1 * r2)
        for k, v in enumerate(stats):
            hstat[k, rows, :] = jnp.broadcast_to(v, (n, 128))
        yield stats[0] + stats[2]

    def strip_copies(batch):
        strips = [(w, at + u * w.shape[1], u)
                  for w, at in ((w1_hbm, W1_AT), (w2_hbm, W2_AT), (w3_hbm, W3_AT), (w4_hbm, W4_AT))
                  for u in range(w.shape[2] // 512)]
        return [pltpu.make_async_copy(
            w.at[:, :, pl.ds(j * (w.shape[2] // 4) + u * 128, 128)],
            raw[j].at[:, pl.ds(at, w.shape[1]), :], sems.at[SEM_STRIP + batch % 2])
            for w, at, u in strips[BATCH[batch]:BATCH[batch + 1]] for j in range(4)]

    def weight_sums(r0):
        x = [[_load(raw[j], k, r0=r0, n=16).astype(f32) for j in range(4)]
             for k in range(4)]

        def emit(n, v):
            if n not in PLAIN:
                ref, *idx = wsum[n]
                ref[(*idx, pl.ds(_mult(r0, 16), 16), slice(None))] = v().astype(bf16)
        yield from _sums2(_sums_b, x, emit)

    def block_a(xb, xn, lo, *bufs):
        w_on, low, wo_s = bufs[0:3], bufs[3:6], bufs[6:13]
        w_hbm = (wq_hbm, wk_hbm, wv_hbm)
        stage = hbuf.reshape(8, hbuf.shape[1] // 8, 8, DH)
        lhs = spare[2:5]
        w_low = [spare[5 + 3 * m:8 + 3 * m] for m in range(3)]

        def x_copy(i):
            return pltpu.make_async_copy(x_hbm.at[pl.ds(2 * i, 2)], xb.at[i & 3],
                                         sems.at[SEM_X + (i & 1)])

        def wo_copies(n):
            return [pltpu.make_async_copy(
                wo_hbm.at[:, i, :, pl.ds(_mult(j * HD + n * 128, 128), 128)],
                wo_s[slot].at[n], sems.at[SEM_WO + n])
                for slot, i, j in ((5, 0, 0), (2, 0, 1), (4, 1, 0), (1, 1, 1))]

        def chunk_copies(g, m):
            src = w_hbm[m].bitcast(f32)
            return [pltpu.make_async_copy(
                src.at[:, :, pl.ds(_mult(16 * par + 4 * g, 4), 4), :],
                stage.at[pl.ds(2 * m, 2), pl.ds(0, S // 8), pl.ds(4 * par, 4), :],
                sems.at[SEM_W + 3 * g + m]) for par in range(2)]

        def start(copies):
            for c in copies:
                c.start()

        def wait(copies):
            for c in copies:
                c.wait()

        def qkv_sums(g, m, pair, d0):
            b = []
            for half in range(2):
                w = pltpu.bitcast(
                    hbuf[2 * m + half, pl.ds(4 * d0 + pair, 16, stride=4), :], u32)
                b += [pltpu.bitcast(w << 16, f32),
                      pltpu.bitcast(w & jnp.uint32(0xFFFF0000), f32)]
            for k, v in enumerate(_sums_b(*b)):
                v = v()
                if k < 4:
                    w_on[m][4 * g + pair, k, pl.ds(d0, 16), :] = v.astype(bf16)
                else:
                    w_low[m][k - 4][pl.ds(_mult(pair * HD + d0, 16), 16), :] = v.astype(bf16)
            return v

        def wo_sums(n, t, e0):
            b = [_load(wo_s[k], n, t, r0=e0, n=16).astype(f32) for k in (5, 2, 4, 1)]
            for k, v in enumerate(_sums_b(*b)):
                if k not in (1, 5):
                    v = v()
                    wo_s[k][n, t, pl.ds(e0, 16), :] = v.astype(bf16)
            return v

        def prologue(xpb):
            def xp_copy(i):
                segs = pl.ds(8 * i, 8)
                return pltpu.make_async_copy(x_hbm.at[segs, pl.ds(16, 16), :], xpb.at[segs],
                                             sems.at[SEM_XP + i])

            start(chunk_copies(0, 0))
            start([xp_copy(i) for i in range(NSEG // 8)])
            start(chunk_copies(0, 1))
            start(chunk_copies(0, 2))
            lo[...] = jnp.zeros(lo.shape, f32)
            for k in (5, 2, 4, 1):
                wo_s[k][3] = jnp.zeros(wo_s[k].shape[1:], bf16)
            wait(chunk_copies(0, 0))

            @pl.loop(0, 4)
            def _(pair):
                for d0 in range(0, HD, 16):
                    qkv_sums(0, 0, pair, d0)

            @pl.loop(0, NSEG // 8)
            def _(i):
                xp_copy(i).wait()
                for j in range(4):
                    a = [_ln(_load(xpb, 8 * i + 2 * j + k).astype(f32)) for k in range(2)]
                    a1 = jnp.concatenate([a[0][:8], a[1][:8]], axis=0)
                    a2 = jnp.concatenate([a[0][8:], a[1][8:]], axis=0)
                    ops = _sums_a(a1[:, :HD], a1[:, HD:], a2[:, :HD], a2[:, HD:])
                    ops = [v() for v in ops[4:]]
                    for k in range(3):
                        for c in range(4):
                            rows = pl.ds(pl.multiple_of(c * 8 * NSEG + 64 * i + 16 * j, 16), 16)
                            lhs[k][rows, :] = ops[k][:, c * 128:(c + 1) * 128].astype(bf16)

        if not 0:
            pl.run_scoped(prologue, pltpu.VMEM((NSEG, 16, D), bf16))

        def lower_products(g, m):
            m1 = (m + 1) % 3
            never = jnp.full((8, 128), zero_ref[0]) != 0
            g1 = jnp.minimum(g + (1 if m == 2 else 0), 3)
            side = [functools.partial(qkv_sums, g1, m1, pair, d0)
                    for d0 in range(0, HD, 16) for pair in range(4)]
            wait_at = 7
            span = 12 - wait_at
            early = [functools.partial(wo_sums, (g + 3) & 3, t, e0)
                     for t in ((), range(0, 8), range(8, NP))[m] for e0 in range(0, DH, 16)]
            for j in range(12):
                pair, k = divmod(j, 3)
                if j >= wait_at:
                    todo = side[len(side) * (j - wait_at) // span:
                                len(side) * (j - wait_at + 1) // span]
                else:
                    todo = early[len(early) * j // wait_at:len(early) * (j + 1) // wait_at]
                a = [lhs[k].bitcast(u32)[pl.ds(c * 4 * NSEG, 4 * NSEG), :] for c in range(4)]
                a[3:] = _tie(never, a[3:], [fn()[8:] for fn in todo], 8)
                a = jnp.concatenate([pltpu.bitcast(v, bf16) for v in a], axis=1)
                res = _dot(a, _load(w_low[m][k], r0=pair * HD, n=HD))
                if j == wait_at - 1:
                    pl.when(3 * g + m < 11)(lambda: wait(chunk_copies(g1, m1)))
                    pl.when(g < 3)(lambda: start(chunk_copies(g + 1, m)))
                    if m == 0:
                        pl.when(g > 0)(lambda: wait(wo_copies(g - 1)))
                        start(wo_copies(g))

                        @pl.when(g == 3)
                        def _():
                            x_copy(0).start()
                            x_copy(1).start()
                            start(strip_copies(0))
                v = res if k == 0 else res + last if k == 1 else res - last
                last = res
                for n in range(NSEG // 2):
                    low[m][n, 4 * g + pair, k] = v[16 * n:16 * n + 16].astype(bf16)

        if not 0:
            @pl.loop(0, 4)
            def _(g):
                for m in range(3):
                    lower_products(g, m)

        def norm_tokens(i, k):
            for r0 in range(0, SEG, 16):
                v = _load(xb, jnp.minimum(i, NSEG // 2 - 1) & 3, k, r0=r0, n=16).astype(f32)
                m, r = yield from _ln_stages(v)
                xn[k, pl.ds(r0, 16), :] = (v - m) * r
                yield r

        def lower_wo(grp, n, parts, state):
            for k in parts:
                w = jnp.concatenate([_load(wo_s[4 + k], n, t) for t in range(NP)], axis=0)
                state[k] = _dot(lo[grp & 1, k].astype(bf16), w)
            if 2 in parts:
                m4, m2, m6 = state[0], state[1], state[2]
                base = jnp.maximum(grp, 0) * (4 * SEG)
                for j in range(4):
                    seg = slice(8 * j, 8 * j + 8)
                    upper = pl.ds(pl.multiple_of(base + j * SEG + 16, 8), 8)
                    lower = pl.ds(pl.multiple_of(base + j * SEG + 24, 8), 8)
                    hbuf[n, upper, :] += m4[seg]
                    hbuf[n, lower, :] += m2[seg] + m4[seg]
                    hbuf[4 + n, lower, :] += m6[seg] - m2[seg]

        def attention_mask():
            def split(axis):
                r = lax.broadcasted_iota(jnp.int32, (80, 80), axis)
                return (jnp.where(r < 64, r >> 5, (r - 64) >> 3),
                        jnp.where(r < 64, r & 31, 32 + (r & 7)))
            (hq, pq), (hk, pk) = split(0), split(1)
            visible = (pq < MEM) | (pq >= pk)
            return jnp.where(hq == hk, jnp.where(visible, 0.0, NEG * DH ** 0.5), -jnp.inf)

        def step(i, k, mem, fill, side):
            tok = xn[k]
            r0 = jnp.maximum(2 * i + k - 8, 0) * SEG
            norms = itertools.chain(h_stats(r0), h_stats(r0 + 16), norm_tokens(i + 1, k))
            s = 2 * i + k
            a1 = jnp.concatenate([mem, tok[:24]], axis=0)
            ops = _upper_operands(a1[:, :HD], a1[:, HD:], tok[24:, HD:])
            qkvs, scores, outs, lower = {}, {}, {}, {}
            total = [None] * 4

            def qkv(t):
                res = {}
                for m in list(itertools.permutations(range(3)))[5]:
                    r = {j: _dot(ops[j], _load(w_on[m], t, j))
                         for j in list(itertools.permutations(range(4)))[23]}
                    m7, m5, m3, m1 = [r[j] for j in range(4)]
                    m4, c21, m62 = [
                        _load(low[m], i, t, j).astype(f32)[8 * k:8 * k + 8]
                        for j in range(3)]
                    side()
                    c11 = m7 - m5 + m1
                    res[m] = (jnp.concatenate(
                        [c11[:24], c11[24:] + m4, m5 + m3, c21, m3[24:] + m62 + m1[24:]],
                        axis=0).astype(bf16))
                qkvs[t] = [res[m] for m in range(3)]

            def qk(t):
                q, kk, v = qkvs.pop(t)
                sc = lax.dot_general(q, kk, (((1,), (1,)), ((), ())),
                                     preferred_element_type=f32)
                scores[t] = (sc, v)

            def pv(t):
                sc, v = scores.pop(t)
                sc = jnp.where(fill == 0.0, sc, fill)
                tie = next(norms, None) if t >= 3 else None
                if tie is not None:
                    sc = jnp.concatenate([jnp.where(never, tie, sc[:16]), sc[16:]], axis=0)
                mx = jnp.max(sc, axis=1, keepdims=True)
                e = jnp.exp2((sc - mx) * (DH ** -0.5 * LOG2E))
                den = jnp.sum(e, axis=1, keepdims=True)
                inv = pl.reciprocal(den, approx=True)
                inv = inv * (2.0 - den * inv)
                outs[t] = _dot(e.astype(bf16), v) * inv

            def wo(t):
                o = outs.pop(t)
                a11, a12, a21, a22 = o[:32], o[32:64], o[64:72], o[72:]
                rows = pl.ds(pl.multiple_of(8 * (s & 3), 8), 8)
                for j, v in enumerate((a22, a21 + a22, a21 - a11[24:])):
                    lo[(s >> 2) & 1, j, rows, pl.ds(t * DH, DH)] = v
                r = [_dot(a, jnp.concatenate([_load(wo_s[j], n, t) for n in range(4)], axis=1))
                     for j, a in enumerate(_upper_operands(a11, a12, a22))]
                if 0:
                    r = [r[0] - r[1] + r[3], r[1] + r[2], r[2][24:] + r[3][24:]]
                for j, v in enumerate(r):
                    total[j] = v if total[j] is None else total[j] + v

            def attend(t):
                if t % 2 == 1:
                    todo = [(qk, LAG_QK), (pv, LAG_PV)]
                    for fn, lag in todo[::-1] if 0 else todo:
                        for u in (t - 1 - lag, t - lag):
                            if 0 <= u < NP:
                                fn(u)

            for t in range(NP + LAG_WO):
                if 1 == 0:
                    attend(t)
                if 0 and 0 <= t - LAG_WO < NP:
                    wo(t - LAG_WO)
                if t < NP:
                    qkv(t)
                lower_wo((s >> 2) - 1, s & 3, [j for j in range(3) if FILL[j] == t], lower)
                if 1 == 1:
                    attend(t)
                if not 0 and 0 <= t - LAG_WO < NP:
                    wo(t - LAG_WO)

            if 0:
                upper, c22 = jnp.concatenate(total[:2], axis=1), total[2]
            else:
                m7, m5, m3, m1 = total
                upper = jnp.concatenate([m7 - m5 + m1, m5 + m3], axis=1)
                c22 = m3[24:] + m1[24:]
            xv = _load(xb, i & 3, k).astype(f32)
            hv = jnp.concatenate(
                [xv[:24] + upper[MEM:],
                 jnp.concatenate([xv[24:, :HD], xv[24:, HD:] + c22], axis=1)], axis=0)
            for c in range(8):
                hbuf[c, pl.ds(pl.multiple_of(s * SEG, SEG), SEG), :] = hv[:, c * 128:(c + 1) * 128]
            lower_wo((s >> 2) - 1, s & 3, [j for j in range(3) if j not in lower], lower)
            return upper[:MEM]

        fill = attention_mask()
        never = jnp.full((16, 80), zero_ref[0]) != 0
        n_it = NSEG // 2
        per_it = WROWS // 16 // n_it

        def steps(i, mem):
            pl.when(i + 1 < n_it)(lambda: x_copy(i + 1).wait())
            pl.when(i + 2 < n_it)(lambda: x_copy(i + 2).start())

            @pl.when(i < len(BATCH) - 2)
            def _():
                for b in range(len(BATCH) - 2):
                    @pl.when(i == b)
                    def _():
                        wait(strip_copies(b))
                        start(strip_copies(b + 1))

            side = _spread([weight_sums(16 * (per_it * i + j)) for j in range(per_it)],
                           7 * per_it, 72)
            for k in range(2):
                mem = step(i, k, mem, fill, side)
            return mem

        if 0:
            hbuf[0, :16] = sum(b[(0,) * (len(b.shape) - 2)][:16].astype(f32) for b in bufs)
        else:
            wait(wo_copies(3))

            @pl.loop(0, NP)
            def _(t):
                for e0 in range(0, DH, 16):
                    wo_sums(3, t, e0)

            hbuf[:, pl.ds(0, 4 * SEG), :] = jnp.zeros((8, 4 * SEG, 128), f32)
            x_copy(0).wait()
            _spread([norm_tokens(0, 0), norm_tokens(0, 1)], 8, 1)()
            lax.fori_loop(0, n_it, steps, mem0_ref[...].astype(f32))
            for n in range(4):
                lower_wo(NSEG // 4 - 1, n, [0, 1, 2], {})

    pl.run_scoped(
        block_a,
        pltpu.VMEM((4, 2, SEG, D), bf16),
        pltpu.VMEM((2, SEG, D), f32),
        pltpu.VMEM((2, 3, 32, NP * DH), f32),
        *[pltpu.VMEM((NP, 4, HD, DH), bf16)] * 3,
        *[pltpu.VMEM((NSEG // 2, NP, 3, 16, DH), bf16)] * 3,
        *[pltpu.VMEM((4, NP, DH, 128), bf16)] * 7,
    )

    def block_b(gbuf, ustat, x1, obuf, yc, hc, db, nb0, nb1, ac0, ac1, pb0, pb1):
        def weights(n, at, rows, strips):
            return jnp.concatenate(
                [_load(*wsum[n], r0=at + k * rows[0] + rows[1], n=rows[2])
                 for k in strips], axis=1)

        ties = []
        never = jnp.full((8, 128), zero_ref[0]) != 0

        def before_next(value):
            if value.shape[1] == 1:
                value = jnp.broadcast_to(value[:8] + value[8:], (8, 128))
            ties.append(value[-8:, -128:])

        def operand(ref, n, cols):
            words = [ref.bitcast(u32)[n, c] for c in cols]
            words = _tie(never, words, ties)
            ties.clear()
            return jnp.concatenate([pltpu.bitcast(w, bf16) for w in words], axis=1)

        def store_sums(dst, r, c, x, tie=True):
            def emit(n, v):
                v = v()
                dst[n, c, pl.ds(16 * r, 16), :] = v.astype(bf16)
                if tie and n % 2:
                    before_next(v)
            return _sums2(_sums_a, x, emit)

        def inner(dst, p, product, side, add=False):
            def emit(a, b, v):
                dst[p, 2 * a + b] = dst[p, 2 * a + b] + v if add else v

            def run(k):
                r = product(7 * p + k)
                side()
                return r
            _combine(run, emit)

        def outer(src, r, cols, emit):
            for a in range(2):
                for b in range(2):
                    _combine(lambda p: src[p, 2 * a + b, pl.ds(16 * r, 16), cols],
                             lambda i, j, v: emit(2 * i + a, 2 * j + b, v))
                    yield

        def rows_of(i, g, r):
            return pl.ds(_mult(i * RB + g * R + 16 * r, 16), 16)

        def tied(stages):
            while True:
                try:
                    before_next(next(stages))
                except StopIteration as stop:
                    return stop.value
                yield
                yield

        def last_stats(i, r):
            return tied(h_stats(S - RB + i * R + 16 * r))

        def pre1(i, r):
            for c in range(2):
                x = []
                for g in range(4):
                    rows = rows_of(i, g, r)
                    x.append([(hbuf[2 * k + c, rows, :] - hstat[0, rows, :]) * hstat[2, rows, :]
                              for k in range(4)])
                yield from range(3)
                yield from store_sums(ac0, r, c, x)

        def post1(i, r):
            def emit(g, j, v):
                v = _gelu_of_double(v)
                gbuf[2 * j + c, pl.ds(HALO + i * RB + g * R + 16 * r, 16), :] = v
            for c in range(2):
                for _ in outer(pb0, r, pl.ds(c * 128, 128), emit):
                    yield
                    yield

        def pre2(i, r):
            for c in range(2):
                x = [[gbuf[2 * k + c, pl.ds(HALO + i * RB + g * R + 16 * r + off, 16), :]
                      for k, off in enumerate((-1, 1, -2, 2))] for g in range(4)]
                yield from store_sums(ac1, r, c, x)

        def post2(i, r):
            def emit(g, j, v):
                rows = rows_of(i, g, r)
                v = v + jnp.concatenate(
                    [(hbuf[c, rows, :] - hstat[0, rows, :]) * hstat[1, rows, :]
                     for c in (2 * j, 2 * j + 1)], axis=1)
                x1[rows, pl.ds(j * C4, C4)] = v
            for _ in outer(pb1, r, slice(None), emit):
                yield
                yield

        def pre3(i, r):
            for g in range(4):
                rows = rows_of(i, g, r)
                m, rs = yield from tied(_ln_stages(x1[rows, :]))
                ustat[0, rows_of(0, g, r), :] = jnp.broadcast_to(m, (16, 128))
                ustat[1, rows_of(0, g, r), :] = jnp.broadcast_to(0.5 * rs, (16, 128))
                before_next(rs)
                yield
                yield

        def sums3(i, r):
            for c in range(2):
                x = [[(x1[rows_of(i, g, r), pl.ds(k * C4 + c * 128, 128)]
                       - ustat[0, rows_of(0, g, r), :]) * ustat[1, rows_of(0, g, r), :]
                      for k in range(4)] for g in range(4)]
                yield from store_sums(yc, r, c, x, isinstance(i, int))

        pieces = {pre1: 20, last_stats: 8, post1: 16, pre2: 14, post2: 8, pre3: 16, sums3: 14}

        def spread(stages, slots):
            stages = [(fn, i) for fn, i in stages if not isinstance(i, int) or 0 <= i < NB]
            return _spread([fn(i, r) for fn, i in stages for r in range(R // 16)],
                           sum(pieces[fn] for fn, _ in stages) * (R // 16), slots)

        def mixer(i, src, at, dst, stages):
            if not 0 <= i < NB:
                return spread(stages, 1)()
            side = spread(stages, 49)
            for p in range(7):
                inner(dst, p, lambda n: _dot(operand(src, n, (0, 1)),
                                             weights(n, at, (C4, 0, C4), (0, 1))),
                      side)

        if not 0:
            for c in range(8):
                gbuf[c, pl.ds(0, HALO), :] = jnp.zeros((HALO, 128), f32)
                gbuf[c, pl.ds(HALO + S, HALO), :] = jnp.zeros((HALO, 128), f32)
            for i in range(-1, NB + 3):
                mixer(i, ac0, W1_AT, pb0, [(pre2, i - 2), (post2, i - 3)]
                      + ([(last_stats, i)] if i < 4 else [(pre3, 0)] if i == NB - 1 else []))
                mixer(i - 2, ac1, W2_AT, pb1, [(pre1, i + 1), (post1, i)]
                      + {9: [(sums3, 0)]}.get(i, []))

        def out_copy(i):
            rows = pl.ds(_mult(i * (RB // 2), RB // 2), RB // 2)
            return pltpu.make_async_copy(obuf.at[rows], out_hbm.at[rows],
                                         sems.at[SEM_OUT + i])

        nb = (nb0, nb1)

        def activate(c, r):
            act = [[None] * 4 for _ in range(4)]

            def emit(g, j, v):
                act[g][j] = _gelu_of_double(v)
            for _ in outer(nb[c % 2], r, slice(None), emit):
                yield
                yield
            yield from store_sums(hc, r, c, act, False)

        pieces[activate] = 15

        def mlp_up():
            for c in range(7):
                side = spread([(activate, c - 1)], 49)
                for p in range(7):
                    inner(nb[c % 2], p, lambda n: _dot(
                        operand(yc, n, (0, 1)), weights(n, W3_AT, (C4, 0, C4), (c,))), side)

        def mlp_down(i, stages):
            def down(p, side, k0=0, k1=F4):
                inner(db, p, lambda n: _dot(operand(hc, n, range(k0 // 128, k1 // 128)),
                                            weights(n, W4_AT, (F4, k0, k1 - k0), (0, 1))),
                      side, add=k0 > 0)

            def finish(bi, bj, plus, minus=()):
                for a in range(2):
                    for b in range(2):
                        rows = pl.ds(_mult(i * RB + (2 * bi + a) * R, R), R)
                        cols = pl.ds((2 * bj + b) * C4, C4)
                        v = x1[rows, cols] + jnp.concatenate(
                            [hbuf[4 * bj + 2 * b + c, rows, :] for c in range(2)], axis=1)
                        for p in minus:
                            v = v - db[p, 2 * a + b]
                        for p in plus:
                            v = v + db[p, 2 * a + b]
                        obuf[rows, cols] = v.astype(bf16)

            down(0, spread([(activate, 6)], 6), 0, F4 - 128)
            down(0, lambda: None, F4 - 128)
            side = spread(stages, 35)
            for p in range(1, 7):
                down(p, side)
                if p == 3:
                    finish(0, 1, (1, 2))
                if p == 5:
                    finish(0, 0, (0, 3, 4), (1,))
            finish(1, 0, (4, 5))
            finish(1, 1, (2, 3, 6), (5,))

        if not 0:
            @pl.loop(0, NB)
            def _(i):
                ties.clear()
                mlp_up()
                nxt = jnp.minimum(i + 1, NB - 1)
                mlp_down(i, [(pre3, nxt), (sums3, nxt)])
                out_copy(2 * i).start()
                out_copy(2 * i + 1).start()

            for i in range(2 * NB):
                out_copy(i).wait()

    if 0:
        hbuf[0, :16] = sum(_load(*wsum[n], n=16).astype(f32) for n in range(49)) + hbuf[0, :16] + hstat[0, :16]
        cp = pltpu.make_async_copy(hbuf.at[0], hbuf.at[1], sems.at[0]); cp.start(); cp.wait()
    pl.run_scoped(
        block_b,
        pltpu.VMEM((8, S + 2 * HALO, 128), f32),
        pltpu.VMEM((2, RB, 128), f32),
        pltpu.VMEM((S, D), f32),
        pltpu.VMEM((S, D), bf16),
        pltpu.VMEM((49, 2, R, 128), bf16),
        pltpu.VMEM((49, 7, R, 128), bf16),
        pltpu.VMEM((7, 4, R, C4), f32),
        *[pltpu.VMEM((7, 4, R, 128), f32)] * 2,
        *[pltpu.VMEM((49, 2, R, 128), bf16)] * 2,
        *[pltpu.VMEM((7, 4, R, C4), f32)] * 2,
    )


@jax.jit
def pallas_sequential_preLN__memory_aug_recurrent_mem_tr__mixer_s_mlp__prompt_kernel(
    A_x: jax.Array,
    A_mem0: jax.Array,
    A_Wq: jax.Array,
    A_Wk: jax.Array,
    A_Wv: jax.Array,
    A_Wo: jax.Array,
    A_seg_len: jax.Array,
    B_x: jax.Array,
    B_w1: jax.Array,
    B_w2: jax.Array,
    B_w3: jax.Array,
    B_w4: jax.Array,
):
    del A_seg_len, B_x
    hbm = pl.BlockSpec(memory_space=pl.ANY)
    vmem = pl.BlockSpec(memory_space=pltpu.VMEM)
    scratch = [
        pltpu.VMEM((8, S, 128), f32),
        pltpu.VMEM((3, S, 128), f32),
        pltpu.SemaphoreType.DMA((NSEM,)),
        pltpu.SMEM((1,), jnp.int32),
    ] + [pltpu.VMEM((4, WROWS, 128), bf16)] * 4 + [pltpu.VMEM((WROWS, 128), bf16)] * 33
    out = pl.pallas_call(
        _kernel,
        out_shape=jax.ShapeDtypeStruct((S, D), A_x.dtype),
        in_specs=[hbm, vmem] + [hbm] * 8,
        out_specs=hbm,
        scratch_shapes=scratch,
        compiler_params=pltpu.CompilerParams(vmem_limit_bytes=128 * 1024 * 1024),
    )(A_x.reshape(NSEG, SEG, D), A_mem0.reshape(MEM, D),
      A_Wq.reshape(2, D // 4, 2 * H, DH), A_Wk.reshape(2, D // 4, 2 * H, DH),
      A_Wv.reshape(2, D // 4, 2 * H, DH), A_Wo.reshape(NP, 2, DH, D),
      B_w1.reshape(4, C4, D), B_w2.reshape(4, C4, D),
      B_w3.reshape(4, C4, F), B_w4.reshape(4, F4, D))
    return out.reshape(A_x.shape)
```

```python
import functools
import itertools

import jax
import jax.numpy as jnp
from jax import lax
import jax.experimental.pallas as pl
import jax.experimental.pallas.tpu as pltpu

S = 2048
D = 1024
H = 32
DH = 128
MEM = 8
SEG = 32
F = 3584
NSEG = S // SEG
NP = H // 2
HD = D // 2
C4 = D // 4
F4 = F // 4
HALO = 8
R = 64
RB = 4 * R
NB = S // RB
EPS = 1e-5
NEG = -1000000000.0
LOG2E = 1.4426950408889634

W1_AT, W2_AT, W3_AT, W4_AT = 0, 2 * C4, 4 * C4, 11 * C4
WROWS = W4_AT + 2 * F4
BATCH = ((0,), (1, 2, 3, 4, 5), (6, 7, 8, 9, 10), (11, 12), ())

LAG_QK, LAG_PV, LAG_WO = 2, 4, 6
FILL = (14, 18, 99)

bf16 = jnp.bfloat16
f32 = jnp.float32
u32 = jnp.uint32

SEM_XP, SEM_X, SEM_WO, SEM_STRIP, SEM_OUT, SEM_W = 0, 8, 10, 14, 16, 16 + 2 * NB
NSEM = SEM_W + 12


def _mult(i, n):
    return i if isinstance(i, int) else pl.multiple_of(i, n)


def _ln_stats(x):
    m = jnp.mean(x, axis=-1, keepdims=True)
    d = x - m
    v = jnp.mean(d * d, axis=-1, keepdims=True)
    return m, lax.rsqrt(v + EPS)


def _ln_stages(x):
    m = jnp.mean(x, axis=-1, keepdims=True)
    yield m
    d = x - m
    r = lax.rsqrt(jnp.mean(d * d, axis=-1, keepdims=True) + EPS)
    return m, r


def _ln(x):
    m, r = _ln_stats(x)
    return (x - m) * r


def _gelu_of_double(y):
    c = 0.7978845608028654
    return y + y * jnp.tanh(y * (2 * c + (8 * c * 0.044715) * (y * y)))


def _dot(a, b):
    return jnp.dot(a, b, preferred_element_type=f32)


def _load(ref, *idx, r0=0, n=None):
    n = ref.shape[-2] if n is None else n
    return pltpu.bitcast(
        ref.bitcast(u32)[(*idx, pl.ds(_mult(r0 >> 1, 8), n // 2), slice(None))], bf16)


def _sums_a(a11, a12, a21, a22):
    return [lambda: a12 - a22, lambda: a11 + a12, lambda: a11, lambda: a11 + a22,
            lambda: a22, lambda: a21 + a22, lambda: a21 - a11]


def _sums_b(b11, b12, b21, b22):
    return [lambda: b21 + b22, lambda: b22, lambda: b12 - b22, lambda: b11 + b22,
            lambda: b21 - b11, lambda: b11, lambda: b11 + b12]


def _combine(product, emit):
    c11 = product(0)
    c12 = product(1)
    c11 = c11 - c12
    c22 = product(2)
    emit(0, 1, c12 + c22)
    t = product(3)
    c11 = c11 + t
    c22 = c22 + t
    c21 = product(4)
    emit(0, 0, c11 + c21)
    t = product(5)
    emit(1, 0, c21 + t)
    c22 = c22 - t
    emit(1, 1, c22 + product(6))


def _sums2(sums, x, emit):
    outer = [sums(x[i][j], x[i][2 + j], x[2 + i][j], x[2 + i][2 + j])
             for i in range(2) for j in range(2)]
    for p in range(7):
        for q, v in enumerate(sums(*(o[p]() for o in outer))):
            emit(7 * p + q, v)
        yield


def _spread(tasks, pieces, slots):
    todo = itertools.chain(*tasks)
    calls = itertools.count(1)

    def advance():
        k = next(calls)
        if k > slots:
            return
        for _ in range(pieces * k // slots - pieces * (k - 1) // slots):
            next(todo)
        if k == slots:
            assert next(todo, todo) is todo
    return advance


def _tie(never, words, values, first=0):
    regs = [[w[r:r + 8] for r in range(0, w.shape[0], 8)] for w in words]
    per = len(regs[0])
    for n, v in enumerate(values):
        c, r = divmod(first + (len(regs) * per - first) * n // len(values), per)
        regs[c][r] = jnp.where(never, pltpu.bitcast(v, u32), regs[c][r])
    return [jnp.concatenate(w, axis=0) for w in regs] if values else words


def _upper_operands(a11, a12, a22):
    k = a11.shape[0] - a22.shape[0]
    ops = [jnp.concatenate([a12[:k], a12[k:] - a22], axis=0), a11 + a12, a11,
           jnp.concatenate([a11[:k], a11[k:] + a22], axis=0)]
    return [v.astype(bf16) for v in ops]


PLAIN = {40: 0, 36: 1, 12: 2, 8: 3}
OTHER = [n for n in range(49) if n not in PLAIN]
RAW_SLOT = dict(zip(OTHER[2::3], [(k, j) for k in range(4) for j in range(4) if k != j]))
RAW_SLOT.update({n: (k, k) for n, k in PLAIN.items()})


def _kernel(x_hbm, mem0_ref, wq_hbm, wk_hbm, wv_hbm, wo_hbm, w1_hbm, w2_hbm,
            w3_hbm, w4_hbm, out_hbm, hbuf, hstat, sems, zero_ref, *wbufs):
    zero_ref[0] = 0
    raw, spare = wbufs[:4], wbufs[4:]
    wsum = {n: (raw[j], k) for n, (k, j) in RAW_SLOT.items()}
    wsum.update({n: (b,) for n, b in zip((n for n in OTHER if n not in RAW_SLOT), spare)})

    def load_h(rows):
        return jnp.concatenate([hbuf[c, rows, :] for c in range(8)], axis=1)

    def h_stats(r0, n=16):
        rows = pl.ds(_mult(r0, 16), n)
        hv = load_h(rows)
        m1, r1 = yield from _ln_stages(hv)
        yield r1
        m2, r2 = yield from _ln_stages((hv - m1) * r1)
        stats = (m1 + m2 / r1, r1, 0.5 * r1 * r2)
        for k, v in enumerate(stats):
            hstat[k, rows, :] = jnp.broadcast_to(v, (n, 128))
        yield stats[0] + stats[2]

    def strip_copies(batch):
        strips = [(w, at + u * w.shape[1], u)
                  for w, at in ((w1_hbm, W1_AT), (w2_hbm, W2_AT), (w3_hbm, W3_AT), (w4_hbm, W4_AT))
                  for u in range(w.shape[2] // 512)]
        return [pltpu.make_async_copy(
            w.at[:, :, pl.ds(j * (w.shape[2] // 4) + u * 128, 128)],
            raw[j].at[:, pl.ds(at, w.shape[1]), :], sems.at[SEM_STRIP + batch % 2])
            for w, at, u in (strips[n] for n in BATCH[batch]) for j in range(4)]

    def weight_sums(r0):
        x = [[_load(raw[j], k, r0=r0, n=16).astype(f32) for j in range(4)]
             for k in range(4)]

        def emit(n, v):
            if n not in PLAIN:
                ref, *idx = wsum[n]
                ref[(*idx, pl.ds(_mult(r0, 16), 16), slice(None))] = v().astype(bf16)
        yield from _sums2(_sums_b, x, emit)

    def block_a(xb, xn, lo, *bufs):
        w_on, low, wo_s = bufs[0:3], bufs[3:6], bufs[6:13]
        w_hbm = (wq_hbm, wk_hbm, wv_hbm)
        stage = hbuf.reshape(8, hbuf.shape[1] // 8, 8, DH)
        lhs = spare[2:5]
        w_low = [spare[5 + 3 * m:8 + 3 * m] for m in range(3)]

        def x_copy(i):
            return pltpu.make_async_copy(x_hbm.at[pl.ds(2 * i, 2)], xb.at[i & 3],
                                         sems.at[SEM_X + (i & 1)])

        def wo_copies(n):
            return [pltpu.make_async_copy(
                wo_hbm.at[:, i, :, pl.ds(_mult(j * HD + n * 128, 128), 128)],
                wo_s[slot].at[n], sems.at[SEM_WO + n])
                for slot, i, j in ((5, 0, 0), (2, 0, 1), (4, 1, 0), (1, 1, 1))]

        def chunk_copies(g, m):
            src = w_hbm[m].bitcast(f32)
            return [pltpu.make_async_copy(
                src.at[:, :, pl.ds(_mult(16 * par + 4 * g, 4), 4), :],
                stage.at[pl.ds(2 * m, 2), pl.ds(0, S // 8), pl.ds(4 * par, 4), :],
                sems.at[SEM_W + 3 * g + m]) for par in range(2)]

        def start(copies):
            for c in copies:
                c.start()

        def wait(copies):
            for c in copies:
                c.wait()

        def qkv_sums(g, m, duo, d0):
            lower, done = [], []
            for d in (d0, d0 + C4):
                for pair in (2 * duo, 2 * duo + 1):
                    b = []
                    for half in range(2):
                        w = pltpu.bitcast(
                            hbuf[2 * m + half, pl.ds(4 * d + pair, 16, stride=4), :], u32)
                        b += [pltpu.bitcast(w << 16, f32),
                              pltpu.bitcast(w & jnp.uint32(0xFFFF0000), f32)]
                    sums = [v() for v in _sums_b(*b)]
                    for k in range(4):
                        w_on[m][4 * g + pair, k, pl.ds(d, 16), :] = sums[k].astype(bf16)
                    lower.append(sums[4:])
                    done.append(sums[3])
            for k in range(3):
                for q, v in enumerate(_sums_b(*(b[k] for b in lower))):
                    v = v()
                    rows = pl.ds(_mult((7 * duo + q) * C4 + d0, 16), 16)
                    w_low[m][k][rows, :] = v.astype(bf16)
                done.append(v)
            return done

        def wo_sums(n, t, e0):
            b = [_load(wo_s[k], n, t, r0=e0, n=16).astype(f32) for k in (5, 2, 4, 1)]
            for k, v in enumerate(_sums_b(*b)):
                if k not in (1, 5):
                    v = v()
                    wo_s[k][n, t, pl.ds(e0, 16), :] = v.astype(bf16)
            return [v]

        def prologue(xpb):
            def xp_copy(i):
                segs = pl.ds(8 * i, 8)
                return pltpu.make_async_copy(x_hbm.at[segs, pl.ds(16, 16), :], xpb.at[segs],
                                             sems.at[SEM_XP + i])

            start(chunk_copies(0, 0))
            start([xp_copy(i) for i in range(NSEG // 8)])
            start(chunk_copies(0, 1))
            start(chunk_copies(0, 2))
            lo[...] = jnp.zeros(lo.shape, f32)
            for k in (5, 2, 4, 1):
                wo_s[k][3] = jnp.zeros(wo_s[k].shape[1:], bf16)
            wait(chunk_copies(0, 0))

            @pl.loop(0, 2)
            def _(duo):
                for d0 in range(0, C4, 16):
                    qkv_sums(0, 0, duo, d0)

            @pl.loop(0, NSEG // 8)
            def _(i):
                xp_copy(i).wait()
                for j in range(2):
                    ops = []
                    for n in range(2):
                        a = [_ln(_load(xpb, 8 * i + 4 * j + 2 * n + k).astype(f32))
                             for k in range(2)]
                        a1 = jnp.concatenate([a[0][:8], a[1][:8]], axis=0)
                        a2 = jnp.concatenate([a[0][8:], a[1][8:]], axis=0)
                        sums = _sums_a(a1[:, :HD], a1[:, HD:], a2[:, :HD], a2[:, HD:])
                        ops.append([v() for v in sums[4:]])
                    for k in range(3):
                        top, bottom = ops[0][k], ops[1][k]
                        for q, v in enumerate(_sums_a(top[:, :C4], top[:, C4:],
                                                      bottom[:, :C4], bottom[:, C4:])):
                            v = v()
                            for c in range(2):
                                r0 = (2 * q + c) * 4 * NSEG + 32 * i + 16 * j
                                lhs[k][pl.ds(pl.multiple_of(r0, 16), 16), :] = (
                                    v[:, c * 128:(c + 1) * 128].astype(bf16))

        if not 0:
            pl.run_scoped(prologue, pltpu.VMEM((NSEG, 16, D), bf16))

        def lower_products(g, m):
            m1 = (m + 1) % 3
            never = jnp.full((8, 128), zero_ref[0]) != 0
            g1 = jnp.minimum(g + (1 if m == 2 else 0), 3)
            side = [functools.partial(qkv_sums, g1, m1, duo, d0)
                    for duo in range(2) for d0 in range(0, C4, 16)]
            wait_at = 22
            span = 42 - wait_at
            early = [functools.partial(wo_sums, (g + 3) & 3, t, e0)
                     for t in range(NP if m == 2 else 0) for e0 in range(0, DH, 16)]

            def product(duo, k, q):
                j = 21 * duo + 7 * k + q
                if j >= wait_at:
                    todo = side[len(side) * (j - wait_at) // span:
                                len(side) * (j - wait_at + 1) // span]
                else:
                    todo = early[len(early) * j // wait_at:len(early) * (j + 1) // wait_at]
                a = [lhs[k].bitcast(u32)[pl.ds((2 * q + c) * 2 * NSEG, 2 * NSEG), :]
                     for c in range(2)]
                a[1:] = _tie(never, a[1:], [v[8:] for fn in todo for v in fn()], 0)
                a = jnp.concatenate([pltpu.bitcast(v, bf16) for v in a], axis=1)
                res = _dot(a, _load(w_low[m][k], r0=(7 * duo + q) * C4, n=C4))
                if j == wait_at - 1:
                    pl.when(3 * g + m < 11)(lambda: wait(chunk_copies(g1, m1)))
                    pl.when(g < 3)(lambda: start(chunk_copies(g + 1, m)))
                    if m == 1:
                        pl.when(g > 0)(lambda: wait(wo_copies(g - 1)))
                        start(wo_copies(g))
                        pl.when(g == 3)(
                            lambda: start([x_copy(0), x_copy(1)] + strip_copies(0)))
                return res

            for duo in range(2):
                last = {}
                for k in range(3):
                    def emit(a, b, res):
                        v = res if k == 0 else res + last[a, b] if k == 1 else res - last[a, b]
                        last[a, b] = res
                        for n in range(NSEG // 4):
                            low[m][2 * n + a, 4 * g + 2 * duo + b, k] = (
                                v[16 * n:16 * n + 16].astype(bf16))
                    _combine(functools.partial(product, duo, k), emit)

        if not 0:
            @pl.loop(0, 4)
            def _(g):
                for m in range(3):
                    lower_products(g, m)

        def norm_tokens(i, k):
            for r0 in range(0, SEG, 16):
                v = _load(xb, jnp.minimum(i, NSEG // 2 - 1) & 3, k, r0=r0, n=16).astype(f32)
                m, r = yield from _ln_stages(v)
                xn[k, pl.ds(r0, 16), :] = (v - m) * r
                yield r

        def lower_wo(grp, n, parts, state):
            for k in parts:
                w = jnp.concatenate([_load(wo_s[4 + k], n, t) for t in range(NP)], axis=0)
                state[k] = _dot(lo[grp & 1, k].astype(bf16), w)
            if 2 in parts:
                m4, m2, m6 = state[0], state[1], state[2]
                base = jnp.maximum(grp, 0) * (4 * SEG)
                for j in range(4):
                    seg = slice(8 * j, 8 * j + 8)
                    upper = pl.ds(pl.multiple_of(base + j * SEG + 16, 8), 8)
                    lower = pl.ds(pl.multiple_of(base + j * SEG + 24, 8), 8)
                    hbuf[n, upper, :] += m4[seg]
                    hbuf[n, lower, :] += m2[seg] + m4[seg]
                    hbuf[4 + n, lower, :] += m6[seg] - m2[seg]

        def attention_mask():
            def split(axis):
                r = lax.broadcasted_iota(jnp.int32, (80, 80), axis)
                return (jnp.where(r < 64, r >> 5, (r - 64) >> 3),
                        jnp.where(r < 64, r & 31, 32 + (r & 7)))
            (hq, pq), (hk, pk) = split(0), split(1)
            visible = (pq < MEM) | (pq >= pk)
            return jnp.where(hq == hk, jnp.where(visible, 0.0, NEG * DH ** 0.5), -jnp.inf)

        def step(i, k, mem, fill, side):
            tok = xn[k]
            r0 = jnp.maximum(2 * i + k - 8, 0) * SEG
            norms = itertools.chain(h_stats(r0), h_stats(r0 + 16), norm_tokens(i + 1, k))
            s = 2 * i + k
            a1 = jnp.concatenate([mem, tok[:24]], axis=0)
            ops = _upper_operands(a1[:, :HD], a1[:, HD:], tok[24:, HD:])
            qkvs, scores, outs, lower = {}, {}, {}, {}
            total = [None] * 4

            def qkv(t):
                res = {}
                for m in list(itertools.permutations(range(3)))[0]:
                    r = {j: _dot(ops[j], _load(w_on[m], t, j))
                         for j in list(itertools.permutations(range(4)))[0]}
                    m7, m5, m3, m1 = [r[j] for j in range(4)]
                    m4, c21, m62 = [
                        _load(low[m], i, t, j).astype(f32)[8 * k:8 * k + 8]
                        for j in range(3)]
                    side()
                    c11 = m7 - m5 + m1
                    res[m] = (jnp.concatenate(
                        [c11[:24], c11[24:] + m4, m5 + m3, c21, m3[24:] + m62 + m1[24:]],
                        axis=0).astype(bf16))
                qkvs[t] = [res[m] for m in range(3)]

            def qk(t):
                q, kk, v = qkvs.pop(t)
                sc = lax.dot_general(q, kk, (((1,), (1,)), ((), ())),
                                     preferred_element_type=f32)
                scores[t] = (sc, v)

            def pv(t):
                sc, v = scores.pop(t)
                sc = jnp.where(fill == 0.0, sc, fill)
                tie = next(norms, None) if t >= 1 else None
                if tie is not None:
                    sc = jnp.concatenate([jnp.where(never, tie, sc[:16]), sc[16:]], axis=0)
                mx = jnp.max(sc, axis=1, keepdims=True)
                e = jnp.exp2((sc - mx) * (DH ** -0.5 * LOG2E))
                den = jnp.sum(e, axis=1, keepdims=True)
                inv = pl.reciprocal(den, approx=True)
                inv = inv * (2.0 - den * inv)
                outs[t] = _dot(e.astype(bf16), v) * inv

            def wo(t):
                o = outs.pop(t)
                a11, a12, a21, a22 = o[:32], o[32:64], o[64:72], o[72:]
                rows = pl.ds(pl.multiple_of(8 * (s & 3), 8), 8)
                for j, v in enumerate((a22, a21 + a22, a21 - a11[24:])):
                    lo[(s >> 2) & 1, j, rows, pl.ds(t * DH, DH)] = v
                r = [_dot(a, jnp.concatenate([_load(wo_s[j], n, t) for n in range(4)], axis=1))
                     for j, a in enumerate(_upper_operands(a11, a12, a22))]
                if 0:
                    r = [r[0] - r[1] + r[3], r[1] + r[2], r[2][24:] + r[3][24:]]
                for j, v in enumerate(r):
                    total[j] = v if total[j] is None else total[j] + v

            def attend(t):
                if t % 2 == 1:
                    todo = [(qk, LAG_QK), (pv, LAG_PV)]
                    for fn, lag in todo[::-1] if 0 else todo:
                        for u in (t - 1 - lag, t - lag):
                            if 0 <= u < NP:
                                fn(u)

            for t in range(NP + LAG_WO):
                if 1 == 0:
                    attend(t)
                if 0 and 0 <= t - LAG_WO < NP:
                    wo(t - LAG_WO)
                if t < NP:
                    qkv(t)
                lower_wo((s >> 2) - 1, s & 3, [j for j in range(3) if FILL[j] == t], lower)
                if 1 == 1:
                    attend(t)
                if not 0 and 0 <= t - LAG_WO < NP:
                    wo(t - LAG_WO)

            if 0:
                upper, c22 = jnp.concatenate(total[:2], axis=1), total[2]
            else:
                m7, m5, m3, m1 = total
                upper = jnp.concatenate([m7 - m5 + m1, m5 + m3], axis=1)
                c22 = m3[24:] + m1[24:]
            xv = _load(xb, i & 3, k).astype(f32)
            hv = jnp.concatenate(
                [xv[:24] + upper[MEM:],
                 jnp.concatenate([xv[24:, :HD], xv[24:, HD:] + c22], axis=1)], axis=0)
            for c in range(8):
                hbuf[c, pl.ds(pl.multiple_of(s * SEG, SEG), SEG), :] = hv[:, c * 128:(c + 1) * 128]
            lower_wo((s >> 2) - 1, s & 3, [j for j in range(3) if j not in lower], lower)
            return upper[:MEM]

        fill = attention_mask()
        never = jnp.full((16, 80), zero_ref[0]) != 0
        n_it = NSEG // 2
        per_it = WROWS // 16 // n_it

        def steps(i, mem):
            pl.when(i + 1 < n_it)(lambda: x_copy(i + 1).wait())
            pl.when(i + 2 < n_it)(lambda: x_copy(i + 2).start())

            @pl.when(i < len(BATCH) - 1)
            def _():
                for b in range(len(BATCH) - 1):
                    @pl.when(i == b)
                    def _():
                        wait(strip_copies(b))
                        start(strip_copies(b + 1))

            side = _spread([weight_sums(16 * (per_it * i + j)) for j in range(per_it)],
                           7 * per_it, 78)
            for k in range(2):
                mem = step(i, k, mem, fill, side)
            return mem

        if 0:
            hbuf[0, :16] = sum(b[(0,) * (len(b.shape) - 2)][:16].astype(f32) for b in bufs)
        else:
            wait(wo_copies(3))

            @pl.loop(0, NP)
            def _(t):
                for e0 in range(0, DH, 16):
                    wo_sums(3, t, e0)

            hbuf[:, pl.ds(0, 4 * SEG), :] = jnp.zeros((8, 4 * SEG, 128), f32)
            x_copy(0).wait()
            _spread([norm_tokens(0, 0), norm_tokens(0, 1)], 8, 1)()
            lax.fori_loop(0, n_it, steps, mem0_ref[...].astype(f32))
            for n in range(4):
                lower_wo(NSEG // 4 - 1, n, [0, 1, 2], {})

    pl.run_scoped(
        block_a,
        pltpu.VMEM((4, 2, SEG, D), bf16),
        pltpu.VMEM((2, SEG, D), f32),
        pltpu.VMEM((2, 3, 32, NP * DH), f32),
        *[pltpu.VMEM((NP, 4, HD, DH), bf16)] * 3,
        *[pltpu.VMEM((NSEG // 2, NP, 3, 16, DH), bf16)] * 3,
        *[pltpu.VMEM((4, NP, DH, 128), bf16)] * 7,
    )

    def block_b(gbuf, ustat, x1, obuf, yc, hc, db, nb0, nb1, ac0, ac1, pb0, pb1):
        def weights(n, at, rows, strips):
            return jnp.concatenate(
                [_load(*wsum[n], r0=at + k * rows[0] + rows[1], n=rows[2])
                 for k in strips], axis=1)

        ties = []
        never = jnp.full((8, 128), zero_ref[0]) != 0

        def before_next(value):
            if value.shape[1] == 1:
                value = jnp.broadcast_to(value[:8] + value[8:], (8, 128))
            ties.append(value[-8:, -128:])

        def operand(ref, n, cols):
            words = [ref.bitcast(u32)[n, c] for c in cols]
            words = _tie(never, words, ties)
            ties.clear()
            return jnp.concatenate([pltpu.bitcast(w, bf16) for w in words], axis=1)

        def store_sums(dst, r, c, x, tie=True):
            def emit(n, v):
                v = v()
                dst[n, c, pl.ds(16 * r, 16), :] = v.astype(bf16)
                if tie and n % 2:
                    before_next(v)
            return _sums2(_sums_a, x, emit)

        def inner(dst, p, product, side, add=False):
            def emit(a, b, v):
                dst[p, 2 * a + b] = dst[p, 2 * a + b] + v if add else v

            def run(k):
                r = product(7 * p + k)
                side()
                return r
            _combine(run, emit)

        def outer(src, r, cols, emit):
            for a in range(2):
                for b in range(2):
                    _combine(lambda p: src[p, 2 * a + b, pl.ds(16 * r, 16), cols],
                             lambda i, j, v: emit(2 * i + a, 2 * j + b, v))
                    yield

        def rows_of(i, g, r):
            return pl.ds(_mult(i * RB + g * R + 16 * r, 16), 16)

        def tied(stages):
            while True:
                try:
                    before_next(next(stages))
                except StopIteration as stop:
                    return stop.value
                yield
                yield

        def last_stats(i, r):
            return tied(h_stats(S - RB + i * R + 16 * r))

        def pre1(i, r):
            for c in range(2):
                x = []
                for g in range(4):
                    rows = rows_of(i, g, r)
                    x.append([(hbuf[2 * k + c, rows, :] - hstat[0, rows, :]) * hstat[2, rows, :]
                              for k in range(4)])
                yield from range(3)
                yield from store_sums(ac0, r, c, x)

        def post1(i, r):
            def emit(g, j, v):
                v = _gelu_of_double(v)
                gbuf[2 * j + c, pl.ds(HALO + i * RB + g * R + 16 * r, 16), :] = v
            for c in range(2):
                for _ in outer(pb0, r, pl.ds(c * 128, 128), emit):
                    yield
                    yield

        def pre2(i, r):
            for c in range(2):
                x = [[gbuf[2 * k + c, pl.ds(HALO + i * RB + g * R + 16 * r + off, 16), :]
                      for k, off in enumerate((-1, 1, -2, 2))] for g in range(4)]
                yield from store_sums(ac1, r, c, x)

        def post2(i, r):
            def emit(g, j, v):
                rows = rows_of(i, g, r)
                v = v + jnp.concatenate(
                    [(hbuf[c, rows, :] - hstat[0, rows, :]) * hstat[1, rows, :]
                     for c in (2 * j, 2 * j + 1)], axis=1)
                x1[rows, pl.ds(j * C4, C4)] = v
            for _ in outer(pb1, r, slice(None), emit):
                yield
                yield

        def pre3(i, r):
            for g in range(4):
                rows = rows_of(i, g, r)
                m, rs = yield from tied(_ln_stages(x1[rows, :]))
                ustat[0, rows_of(0, g, r), :] = jnp.broadcast_to(m, (16, 128))
                ustat[1, rows_of(0, g, r), :] = jnp.broadcast_to(0.5 * rs, (16, 128))
                before_next(rs)
                yield
                yield

        def sums3(i, r):
            for c in range(2):
                x = [[(x1[rows_of(i, g, r), pl.ds(k * C4 + c * 128, 128)]
                       - ustat[0, rows_of(0, g, r), :]) * ustat[1, rows_of(0, g, r), :]
                      for k in range(4)] for g in range(4)]
                yield from store_sums(yc, r, c, x, isinstance(i, int))

        pieces = {pre1: 20, last_stats: 8, post1: 16, pre2: 14, post2: 8, pre3: 16, sums3: 14}

        def spread(stages, slots):
            stages = [(fn, i) for fn, i in stages if not isinstance(i, int) or 0 <= i < NB]
            return _spread([fn(i, r) for fn, i in stages for r in range(R // 16)],
                           sum(pieces[fn] for fn, _ in stages) * (R // 16), slots)

        def mixer(i, src, at, dst, stages):
            if not 0 <= i < NB:
                return spread(stages, 1)()
            side = spread(stages, 49)
            for p in range(7):
                inner(dst, p, lambda n: _dot(operand(src, n, (0, 1)),
                                             weights(n, at, (C4, 0, C4), (0, 1))),
                      side)

        if not 0:
            for c in range(8):
                gbuf[c, pl.ds(0, HALO), :] = jnp.zeros((HALO, 128), f32)
                gbuf[c, pl.ds(HALO + S, HALO), :] = jnp.zeros((HALO, 128), f32)
            for i in range(-1, NB + 3):
                mixer(i, ac0, W1_AT, pb0, [(pre2, i - 2), (post2, i - 3)]
                      + ([(last_stats, i)] if i < 4 else [(pre3, 0)] if i == NB - 1 else []))
                mixer(i - 2, ac1, W2_AT, pb1, [(pre1, i + 1), (post1, i)]
                      + {9: [(sums3, 0)]}.get(i, []))

        def out_copy(i):
            rows = pl.ds(_mult(i * (RB // 2), RB // 2), RB // 2)
            return pltpu.make_async_copy(obuf.at[rows], out_hbm.at[rows],
                                         sems.at[SEM_OUT + i])

        nb = (nb0, nb1)

        def activate(c, r):
            act = [[None] * 4 for _ in range(4)]

            def emit(g, j, v):
                act[g][j] = _gelu_of_double(v)
            for _ in outer(nb[c % 2], r, slice(None), emit):
                yield
                yield
            yield from store_sums(hc, r, c, act, False)

        pieces[activate] = 15

        def mlp_up():
            for c in range(7):
                side = spread([(activate, c - 1)], 49)
                for p in range(7):
                    inner(nb[c % 2], p, lambda n: _dot(
                        operand(yc, n, (0, 1)), weights(n, W3_AT, (C4, 0, C4), (c,))), side)

        def mlp_down(i, stages):
            def down(p, side, k0=0, k1=F4):
                inner(db, p, lambda n: _dot(operand(hc, n, range(k0 // 128, k1 // 128)),
                                            weights(n, W4_AT, (F4, k0, k1 - k0), (0, 1))),
                      side, add=k0 > 0)

            def finish(bi, bj, plus, minus=()):
                for a in range(2):
                    for b in range(2):
                        rows = pl.ds(_mult(i * RB + (2 * bi + a) * R, R), R)
                        cols = pl.ds((2 * bj + b) * C4, C4)
                        v = x1[rows, cols] + jnp.concatenate(
                            [hbuf[4 * bj + 2 * b + c, rows, :] for c in range(2)], axis=1)
                        for p in minus:
                            v = v - db[p, 2 * a + b]
                        for p in plus:
                            v = v + db[p, 2 * a + b]
                        obuf[rows, cols] = v.astype(bf16)

            down(0, spread([(activate, 6)], 6), 0, F4 - 128)
            down(0, lambda: None, F4 - 128)
            side = spread(stages, 35)
            for p in range(1, 7):
                down(p, side)
                if p == 3:
                    finish(0, 1, (1, 2))
                if p == 5:
                    finish(0, 0, (0, 3, 4), (1,))
            finish(1, 0, (4, 5))
            finish(1, 1, (2, 3, 6), (5,))

        if not 0:
            @pl.loop(0, NB)
            def _(i):
                ties.clear()
                mlp_up()
                nxt = jnp.minimum(i + 1, NB - 1)
                mlp_down(i, [(pre3, nxt), (sums3, nxt)])
                out_copy(2 * i).start()
                out_copy(2 * i + 1).start()

            for i in range(2 * NB):
                out_copy(i).wait()

    if 0:
        hbuf[0, :16] = sum(_load(*wsum[n], n=16).astype(f32) for n in range(49)) + hbuf[0, :16] + hstat[0, :16]
        cp = pltpu.make_async_copy(hbuf.at[0], hbuf.at[1], sems.at[0]); cp.start(); cp.wait()
    pl.run_scoped(
        block_b,
        pltpu.VMEM((8, S + 2 * HALO, 128), f32),
        pltpu.VMEM((2, RB, 128), f32),
        pltpu.VMEM((S, D), f32),
        pltpu.VMEM((S, D), bf16),
        pltpu.VMEM((49, 2, R, 128), bf16),
        pltpu.VMEM((49, 7, R, 128), bf16),
        pltpu.VMEM((7, 4, R, C4), f32),
        *[pltpu.VMEM((7, 4, R, 128), f32)] * 2,
        *[pltpu.VMEM((49, 2, R, 128), bf16)] * 2,
        *[pltpu.VMEM((7, 4, R, C4), f32)] * 2,
    )


@jax.jit
def pallas_sequential_preLN__memory_aug_recurrent_mem_tr__mixer_s_mlp__prompt_kernel(
    A_x: jax.Array,
    A_mem0: jax.Array,
    A_Wq: jax.Array,
    A_Wk: jax.Array,
    A_Wv: jax.Array,
    A_Wo: jax.Array,
    A_seg_len: jax.Array,
    B_x: jax.Array,
    B_w1: jax.Array,
    B_w2: jax.Array,
    B_w3: jax.Array,
    B_w4: jax.Array,
):
    del A_seg_len, B_x
    hbm = pl.BlockSpec(memory_space=pl.ANY)
    vmem = pl.BlockSpec(memory_space=pltpu.VMEM)
    scratch = [
        pltpu.VMEM((8, S, 128), f32),
        pltpu.VMEM((3, S, 128), f32),
        pltpu.SemaphoreType.DMA((NSEM,)),
        pltpu.SMEM((1,), jnp.int32),
    ] + [pltpu.VMEM((4, WROWS, 128), bf16)] * 4 + [pltpu.VMEM((WROWS, 128), bf16)] * 33
    out = pl.pallas_call(
        _kernel,
        out_shape=jax.ShapeDtypeStruct((S, D), A_x.dtype),
        in_specs=[hbm, vmem] + [hbm] * 8,
        out_specs=hbm,
        scratch_shapes=scratch,
        compiler_params=pltpu.CompilerParams(vmem_limit_bytes=128 * 1024 * 1024),
    )(A_x.reshape(NSEG, SEG, D), A_mem0.reshape(MEM, D),
      A_Wq.reshape(2, D // 4, 2 * H, DH), A_Wk.reshape(2, D // 4, 2 * H, DH),
      A_Wv.reshape(2, D // 4, 2 * H, DH), A_Wo.reshape(NP, 2, DH, D),
      B_w1.reshape(4, C4, D), B_w2.reshape(4, C4, D),
      B_w3.reshape(4, C4, F), B_w4.reshape(4, F4, D))
    return out.reshape(A_x.shape)
```

```python
import functools
import itertools

import jax
import jax.numpy as jnp
from jax import lax
import jax.experimental.pallas as pl
import jax.experimental.pallas.tpu as pltpu

S = 2048
D = 1024
H = 32
DH = 128
MEM = 8
SEG = 32
F = 3584
NSEG = S // SEG
NP = H // 2
HD = D // 2
C4 = D // 4
F4 = F // 4
HALO = 8
R = 64
RB = 4 * R
NB = S // RB
EPS = 1e-5
NEG = -1000000000.0
LOG2E = 1.4426950408889634

W1_AT, W2_AT, W3_AT, W4_AT = 0, 2 * C4, 4 * C4, 11 * C4
WROWS = W4_AT + 2 * F4
BATCH = ((0,), (1, 2, 3, 4, 5), (6, 7, 8, 9, 10), (11, 12), ())

LAG_QK, LAG_PV, LAG_WO = 2, 4, 6
FILL_AT = (14, 18)

bf16 = jnp.bfloat16
f32 = jnp.float32
u32 = jnp.uint32

SEM_XP, SEM_X, SEM_WO, SEM_STRIP, SEM_OUT, SEM_W = 0, 8, 10, 14, 16, 16 + 2 * NB
NSEM = SEM_W + 12


def _mult(i, n):
    return i if isinstance(i, int) else pl.multiple_of(i, n)


def _ln(x):
    d = x - jnp.mean(x, axis=-1, keepdims=True)
    return d * lax.rsqrt(jnp.mean(d * d, axis=-1, keepdims=True) + EPS)


def _ln_stages(x):
    m = jnp.mean(x, axis=-1, keepdims=True)
    yield m
    d = x - m
    return m, lax.rsqrt(jnp.mean(d * d, axis=-1, keepdims=True) + EPS)


def _gelu_of_double(y):
    c = 0.7978845608028654
    return y + y * jnp.tanh(y * (2 * c + (8 * c * 0.044715) * (y * y)))


def _dot(a, b):
    return jnp.dot(a, b, preferred_element_type=f32)


def _load(ref, *idx, r0=0, n=None):
    n = ref.shape[-2] if n is None else n
    return pltpu.bitcast(
        ref.bitcast(u32)[(*idx, pl.ds(_mult(r0 >> 1, 8), n // 2), slice(None))], bf16)


def _sums_a(a11, a12, a21, a22):
    return [lambda: a12 - a22, lambda: a11 + a12, lambda: a11, lambda: a11 + a22,
            lambda: a22, lambda: a21 + a22, lambda: a21 - a11]


def _sums_b(b11, b12, b21, b22):
    return [lambda: b21 + b22, lambda: b22, lambda: b12 - b22, lambda: b11 + b22,
            lambda: b21 - b11, lambda: b11, lambda: b11 + b12]


def _combine(product, emit):
    c11 = product(0)
    c12 = product(1)
    c11 = c11 - c12
    c22 = product(2)
    emit(0, 1, c12 + c22)
    t = product(3)
    c11 = c11 + t
    c22 = c22 + t
    c21 = product(4)
    emit(0, 0, c11 + c21)
    t = product(5)
    emit(1, 0, c21 + t)
    c22 = c22 - t
    emit(1, 1, c22 + product(6))


def _sums2(sums, x, emit):
    outer = [sums(x[i][j], x[i][2 + j], x[2 + i][j], x[2 + i][2 + j])
             for i in range(2) for j in range(2)]
    for p in range(7):
        for q, v in enumerate(sums(*(o[p]() for o in outer))):
            emit(7 * p + q, v)
        yield


def _spread(tasks, pieces, slots):
    todo = itertools.chain(*tasks)
    calls = itertools.count(1)

    def advance():
        k = next(calls)
        if k > slots:
            return
        for _ in range(pieces * k // slots - pieces * (k - 1) // slots):
            next(todo)
        if k == slots:
            assert next(todo, todo) is todo
    return advance


def _tie(never, words, values):
    regs = [[w[r:r + 8] for r in range(0, w.shape[0], 8)] for w in words]
    per = len(regs[0])
    for n, v in enumerate(values):
        c, r = divmod(len(regs) * per * n // len(values), per)
        regs[c][r] = jnp.where(never, pltpu.bitcast(v, u32), regs[c][r])
    return [jnp.concatenate(w, axis=0) for w in regs] if values else words


def _upper_operands(a11, a12, a22):
    k = a11.shape[0] - a22.shape[0]
    ops = [jnp.concatenate([a12[:k], a12[k:] - a22], axis=0), a11 + a12, a11,
           jnp.concatenate([a11[:k], a11[k:] + a22], axis=0)]
    return [v.astype(bf16) for v in ops]


PLAIN = {40: 0, 36: 1, 12: 2, 8: 3}
OTHER = [n for n in range(49) if n not in PLAIN]
RAW_SLOT = dict(zip(OTHER[2::3], [(k, j) for k in range(4) for j in range(4) if k != j]))
RAW_SLOT.update({n: (k, k) for n, k in PLAIN.items()})


def _kernel(x_hbm, mem0_ref, wq_hbm, wk_hbm, wv_hbm, wo_hbm, w1_hbm, w2_hbm,
            w3_hbm, w4_hbm, out_hbm, hbuf, hstat, sems, zero_ref, *wbufs):
    zero_ref[0] = 0
    raw, spare = wbufs[:4], wbufs[4:]
    wsum = {n: (raw[j], k) for n, (k, j) in RAW_SLOT.items()}
    wsum.update({n: (b,) for n, b in zip((n for n in OTHER if n not in RAW_SLOT), spare)})

    def load_h(rows):
        return jnp.concatenate([hbuf[c, rows, :] for c in range(8)], axis=1)

    def h_stats(r0):
        rows = pl.ds(_mult(r0, 16), 16)
        hv = load_h(rows)
        m1, r1 = yield from _ln_stages(hv)
        yield r1
        m2, r2 = yield from _ln_stages((hv - m1) * r1)
        stats = (m1 + m2 / r1, r1, 0.5 * r1 * r2)
        for k, v in enumerate(stats):
            hstat[k, rows, :] = jnp.broadcast_to(v, (16, 128))
        yield stats[0] + stats[2]

    def strip_copies(batch):
        strips = [(w, at + u * w.shape[1], u)
                  for w, at in ((w1_hbm, W1_AT), (w2_hbm, W2_AT), (w3_hbm, W3_AT), (w4_hbm, W4_AT))
                  for u in range(w.shape[2] // 512)]
        return [pltpu.make_async_copy(
            w.at[:, :, pl.ds(j * (w.shape[2] // 4) + u * 128, 128)],
            raw[j].at[:, pl.ds(at, w.shape[1]), :], sems.at[SEM_STRIP + batch % 2])
            for w, at, u in (strips[n] for n in BATCH[batch]) for j in range(4)]

    def weight_sums(r0):
        x = [[_load(raw[j], k, r0=r0, n=16).astype(f32) for j in range(4)]
             for k in range(4)]

        def emit(n, v):
            if n not in PLAIN:
                ref, *idx = wsum[n]
                ref[(*idx, pl.ds(_mult(r0, 16), 16), slice(None))] = v().astype(bf16)
        yield from _sums2(_sums_b, x, emit)

    def block_a(xb, xn, lo, *bufs):
        w_on, low, wo_s = bufs[0:3], bufs[3:6], bufs[6:13]
        w_hbm = (wq_hbm, wk_hbm, wv_hbm)
        stage = hbuf.reshape(8, S // 8, 8, DH)
        lhs = spare[2:5]
        w_low = [spare[5 + 3 * m:8 + 3 * m] for m in range(3)]

        def x_copy(i):
            return pltpu.make_async_copy(x_hbm.at[pl.ds(2 * i, 2)], xb.at[i & 3],
                                         sems.at[SEM_X + (i & 1)])

        def wo_copies(n):
            return [pltpu.make_async_copy(
                wo_hbm.at[:, i, :, pl.ds(_mult(j * HD + n * 128, 128), 128)],
                wo_s[slot].at[n], sems.at[SEM_WO + n])
                for slot, i, j in ((5, 0, 0), (2, 0, 1), (4, 1, 0), (1, 1, 1))]

        def chunk_copies(g, m):
            src = w_hbm[m].bitcast(f32)
            return [pltpu.make_async_copy(
                src.at[:, :, pl.ds(_mult(16 * par + 4 * g, 4), 4), :],
                stage.at[pl.ds(2 * m, 2), :, pl.ds(4 * par, 4), :],
                sems.at[SEM_W + 3 * g + m]) for par in range(2)]

        def start(copies):
            for c in copies:
                c.start()

        def wait(copies):
            for c in copies:
                c.wait()

        def qkv_sums(g, m, duo, d0):
            lower, done = [], []
            for d in (d0, d0 + C4):
                for pair in (2 * duo, 2 * duo + 1):
                    b = []
                    for half in range(2):
                        w = pltpu.bitcast(
                            hbuf[2 * m + half, pl.ds(4 * d + pair, 16, stride=4), :], u32)
                        b += [pltpu.bitcast(w << 16, f32),
                              pltpu.bitcast(w & jnp.uint32(0xFFFF0000), f32)]
                    sums = [v() for v in _sums_b(*b)]
                    for k in range(4):
                        w_on[m][4 * g + pair, k, pl.ds(d, 16), :] = sums[k].astype(bf16)
                    lower.append(sums[4:])
                    done.append(sums[3])
            for k in range(3):
                for q, v in enumerate(_sums_b(*(b[k] for b in lower))):
                    v = v()
                    rows = pl.ds(_mult((7 * duo + q) * C4 + d0, 16), 16)
                    w_low[m][k][rows, :] = v.astype(bf16)
                done.append(v)
            return done

        def wo_sums(n, t, e0):
            b = [_load(wo_s[k], n, t, r0=e0, n=16).astype(f32) for k in (5, 2, 4, 1)]
            for k, v in enumerate(_sums_b(*b)):
                if k not in (1, 5):
                    v = v()
                    wo_s[k][n, t, pl.ds(e0, 16), :] = v.astype(bf16)
            return [v]

        def prologue(xpb):
            def xp_copy(i):
                segs = pl.ds(8 * i, 8)
                return pltpu.make_async_copy(x_hbm.at[segs, pl.ds(16, 16), :], xpb.at[segs],
                                             sems.at[SEM_XP + i])

            start(chunk_copies(0, 0))
            start([xp_copy(i) for i in range(NSEG // 8)])
            start(chunk_copies(0, 1))
            start(chunk_copies(0, 2))
            lo[...] = jnp.zeros(lo.shape, f32)
            for k in (5, 2, 4, 1):
                wo_s[k][3] = jnp.zeros(wo_s[k].shape[1:], bf16)
            wait(chunk_copies(0, 0))

            @pl.loop(0, 2)
            def _(duo):
                for d0 in range(0, C4, 16):
                    qkv_sums(0, 0, duo, d0)

            @pl.loop(0, NSEG // 8)
            def _(i):
                xp_copy(i).wait()
                for j in range(2):
                    ops = []
                    for n in range(2):
                        a = [_ln(_load(xpb, 8 * i + 4 * j + 2 * n + k).astype(f32))
                             for k in range(2)]
                        a1 = jnp.concatenate([a[0][:8], a[1][:8]], axis=0)
                        a2 = jnp.concatenate([a[0][8:], a[1][8:]], axis=0)
                        sums = _sums_a(a1[:, :HD], a1[:, HD:], a2[:, :HD], a2[:, HD:])
                        ops.append([v() for v in sums[4:]])
                    for k in range(3):
                        top, bottom = ops[0][k], ops[1][k]
                        for q, v in enumerate(_sums_a(top[:, :C4], top[:, C4:],
                                                      bottom[:, :C4], bottom[:, C4:])):
                            v = v()
                            for c in range(2):
                                r0 = (2 * q + c) * 4 * NSEG + 32 * i + 16 * j
                                lhs[k][pl.ds(pl.multiple_of(r0, 16), 16), :] = (
                                    v[:, c * 128:(c + 1) * 128].astype(bf16))

        pl.run_scoped(prologue, pltpu.VMEM((NSEG, 16, D), bf16))

        def lower_products(g, m):
            m1 = (m + 1) % 3
            never = jnp.full((8, 128), zero_ref[0]) != 0
            g1 = jnp.minimum(g + (1 if m == 2 else 0), 3)
            side = [functools.partial(qkv_sums, g1, m1, duo, d0)
                    for duo in range(2) for d0 in range(0, C4, 16)]
            wait_at = 22
            span = 42 - wait_at
            early = [functools.partial(wo_sums, (g + 3) & 3, t, e0)
                     for t in range(NP if m == 2 else 0) for e0 in range(0, DH, 16)]

            def product(duo, k, q):
                j = 21 * duo + 7 * k + q
                if j >= wait_at:
                    todo = side[len(side) * (j - wait_at) // span:
                                len(side) * (j - wait_at + 1) // span]
                else:
                    todo = early[len(early) * j // wait_at:len(early) * (j + 1) // wait_at]
                a = [lhs[k].bitcast(u32)[pl.ds((2 * q + c) * 2 * NSEG, 2 * NSEG), :]
                     for c in range(2)]
                a[1:] = _tie(never, a[1:], [v[8:] for fn in todo for v in fn()])
                a = jnp.concatenate([pltpu.bitcast(v, bf16) for v in a], axis=1)
                res = _dot(a, _load(w_low[m][k], r0=(7 * duo + q) * C4, n=C4))
                if j == wait_at - 1:
                    pl.when(3 * g + m < 11)(lambda: wait(chunk_copies(g1, m1)))
                    pl.when(g < 3)(lambda: start(chunk_copies(g + 1, m)))
                    if m == 1:
                        pl.when(g > 0)(lambda: wait(wo_copies(g - 1)))
                        start(wo_copies(g))
                        pl.when(g == 3)(
                            lambda: start([x_copy(0), x_copy(1)] + strip_copies(0)))
                return res

            for duo in range(2):
                last = {}
                for k in range(3):
                    def emit(a, b, res):
                        v = res if k == 0 else res + last[a, b] if k == 1 else res - last[a, b]
                        last[a, b] = res
                        for n in range(NSEG // 4):
                            low[m][2 * n + a, 4 * g + 2 * duo + b, k] = (
                                v[16 * n:16 * n + 16].astype(bf16))
                    _combine(functools.partial(product, duo, k), emit)

        @pl.loop(0, 4)
        def _(g):
            for m in range(3):
                lower_products(g, m)

        def norm_tokens(i, k):
            for r0 in range(0, SEG, 16):
                v = _load(xb, jnp.minimum(i, NSEG // 2 - 1) & 3, k, r0=r0, n=16).astype(f32)
                m, r = yield from _ln_stages(v)
                xn[k, pl.ds(r0, 16), :] = (v - m) * r
                yield r

        def lower_wo(grp, n, k):
            w = jnp.concatenate([_load(wo_s[4 + k], n, t) for t in range(NP)], axis=0)
            return _dot(lo[grp & 1, k].astype(bf16), w)

        def add_lower(grp, n, m4, m2, m6):
            for j in range(4):
                seg = slice(8 * j, 8 * j + 8)
                upper = pl.ds(_mult((4 * grp + j) * SEG + 16, 8), 8)
                lower = pl.ds(_mult((4 * grp + j) * SEG + 24, 8), 8)
                hbuf[n, upper, :] += m4[seg]
                hbuf[n, lower, :] += m2[seg] + m4[seg]
                hbuf[4 + n, lower, :] += m6[seg] - m2[seg]

        def attention_mask():
            def split(axis):
                r = lax.broadcasted_iota(jnp.int32, (80, 80), axis)
                return (jnp.where(r < 64, r >> 5, (r - 64) >> 3),
                        jnp.where(r < 64, r & 31, 32 + (r & 7)))
            (hq, pq), (hk, pk) = split(0), split(1)
            visible = (pq < MEM) | (pq >= pk)
            return jnp.where(hq == hk, jnp.where(visible, 0.0, NEG * DH ** 0.5), -jnp.inf)

        def step(i, k, mem, fill, side):
            tok = xn[k]
            r0 = jnp.maximum(2 * i + k - 8, 0) * SEG
            norms = itertools.chain(h_stats(r0), h_stats(r0 + 16), norm_tokens(i + 1, k))
            s = 2 * i + k
            a1 = jnp.concatenate([mem, tok[:24]], axis=0)
            ops = _upper_operands(a1[:, :HD], a1[:, HD:], tok[24:, HD:])
            qkvs, scores, outs, lower = {}, {}, {}, []
            total = [None] * 4

            def qkv(t):
                res = []
                for m in range(3):
                    m7, m5, m3, m1 = [_dot(ops[j], _load(w_on[m], t, j)) for j in range(4)]
                    m4, c21, m62 = [
                        _load(low[m], i, t, j).astype(f32)[8 * k:8 * k + 8]
                        for j in range(3)]
                    side()
                    c11 = m7 - m5 + m1
                    res.append(jnp.concatenate(
                        [c11[:24], c11[24:] + m4, m5 + m3, c21, m3[24:] + m62 + m1[24:]],
                        axis=0).astype(bf16))
                qkvs[t] = res

            def qk(t):
                q, kk, v = qkvs.pop(t)
                sc = lax.dot_general(q, kk, (((1,), (1,)), ((), ())),
                                     preferred_element_type=f32)
                scores[t] = (sc, v)

            def pv(t):
                sc, v = scores.pop(t)
                sc = jnp.where(fill == 0.0, sc, fill)
                tie = next(norms, None) if t >= 1 else None
                if tie is not None:
                    sc = jnp.concatenate([jnp.where(never, tie, sc[:16]), sc[16:]], axis=0)
                mx = jnp.max(sc, axis=1, keepdims=True)
                e = jnp.exp2((sc - mx) * (DH ** -0.5 * LOG2E))
                den = jnp.sum(e, axis=1, keepdims=True)
                inv = pl.reciprocal(den, approx=True)
                inv = inv * (2.0 - den * inv)
                outs[t] = _dot(e.astype(bf16), v) * inv

            def wo(t):
                o = outs.pop(t)
                a11, a12, a21, a22 = o[:32], o[32:64], o[64:72], o[72:]
                rows = pl.ds(pl.multiple_of(8 * (s & 3), 8), 8)
                for j, v in enumerate((a22, a21 + a22, a21 - a11[24:])):
                    lo[(s >> 2) & 1, j, rows, pl.ds(t * DH, DH)] = v
                for j, a in enumerate(_upper_operands(a11, a12, a22)):
                    r = _dot(a, jnp.concatenate(
                        [_load(wo_s[j], n, t) for n in range(4)], axis=1))
                    total[j] = r if total[j] is None else total[j] + r

            for t in range(NP + LAG_WO):
                if t < NP:
                    qkv(t)
                if t in FILL_AT:
                    lower.append(lower_wo((s >> 2) - 1, s & 3, len(lower)))
                if t % 2:
                    for fn, lag in ((qk, LAG_QK), (pv, LAG_PV)):
                        for u in (t - 1 - lag, t - lag):
                            if 0 <= u < NP:
                                fn(u)
                if t >= LAG_WO:
                    wo(t - LAG_WO)

            m7, m5, m3, m1 = total
            upper = jnp.concatenate([m7 - m5 + m1, m5 + m3], axis=1)
            c22 = m3[24:] + m1[24:]
            xv = _load(xb, i & 3, k).astype(f32)
            hv = jnp.concatenate(
                [xv[:24] + upper[MEM:],
                 jnp.concatenate([xv[24:, :HD], xv[24:, HD:] + c22], axis=1)], axis=0)
            for c in range(8):
                hbuf[c, pl.ds(pl.multiple_of(s * SEG, SEG), SEG), :] = hv[:, c * 128:(c + 1) * 128]
            add_lower(jnp.maximum((s >> 2) - 1, 0), s & 3,
                      *lower, lower_wo((s >> 2) - 1, s & 3, 2))
            return upper[:MEM]

        fill = attention_mask()
        never = jnp.full((16, 80), zero_ref[0]) != 0
        n_it = NSEG // 2
        per_it = WROWS // 16 // n_it

        def steps(i, mem):
            pl.when(i + 1 < n_it)(lambda: x_copy(i + 1).wait())
            pl.when(i + 2 < n_it)(lambda: x_copy(i + 2).start())

            @pl.when(i < len(BATCH) - 1)
            def _():
                for b in range(len(BATCH) - 1):
                    @pl.when(i == b)
                    def _():
                        wait(strip_copies(b))
                        start(strip_copies(b + 1))

            side = _spread([weight_sums(16 * (per_it * i + j)) for j in range(per_it)],
                           7 * per_it, 78)
            for k in range(2):
                mem = step(i, k, mem, fill, side)
            return mem

        wait(wo_copies(3))

        @pl.loop(0, NP)
        def _(t):
            for e0 in range(0, DH, 16):
                wo_sums(3, t, e0)

        hbuf[:, pl.ds(0, 4 * SEG), :] = jnp.zeros((8, 4 * SEG, 128), f32)
        x_copy(0).wait()
        _spread([norm_tokens(0, 0), norm_tokens(0, 1)], 8, 1)()
        lax.fori_loop(0, n_it, steps, mem0_ref[...].astype(f32))
        for n in range(4):
            add_lower(NSEG // 4 - 1, n, *(lower_wo(NSEG // 4 - 1, n, k) for k in range(3)))

    pl.run_scoped(
        block_a,
        pltpu.VMEM((4, 2, SEG, D), bf16),
        pltpu.VMEM((2, SEG, D), f32),
        pltpu.VMEM((2, 3, 32, NP * DH), f32),
        *[pltpu.VMEM((NP, 4, HD, DH), bf16)] * 3,
        *[pltpu.VMEM((NSEG // 2, NP, 3, 16, DH), bf16)] * 3,
        *[pltpu.VMEM((4, NP, DH, 128), bf16)] * 7,
    )

    def block_b(gbuf, ustat, x1, obuf, yc, hc, db, nb0, nb1, ac0, ac1, pb0, pb1):
        def weights(n, at, rows, strips):
            return jnp.concatenate(
                [_load(*wsum[n], r0=at + k * rows[0] + rows[1], n=rows[2])
                 for k in strips], axis=1)

        ties = []
        never = jnp.full((8, 128), zero_ref[0]) != 0

        def before_next(value):
            if value.shape[1] == 1:
                value = jnp.broadcast_to(value[:8] + value[8:], (8, 128))
            ties.append(value[-8:, -128:])

        def operand(ref, n, cols):
            words = [ref.bitcast(u32)[n, c] for c in cols]
            words = _tie(never, words, ties)
            ties.clear()
            return jnp.concatenate([pltpu.bitcast(w, bf16) for w in words], axis=1)

        def store_sums(dst, r, c, x, tie=True):
            def emit(n, v):
                v = v()
                dst[n, c, pl.ds(16 * r, 16), :] = v.astype(bf16)
                if tie and n % 2:
                    before_next(v)
            return _sums2(_sums_a, x, emit)

        def inner(dst, p, product, side, add=False):
            def emit(a, b, v):
                dst[p, 2 * a + b] = dst[p, 2 * a + b] + v if add else v

            def run(k):
                r = product(7 * p + k)
                side()
                return r
            _combine(run, emit)

        def outer(src, r, cols, emit):
            for a in range(2):
                for b in range(2):
                    _combine(lambda p: src[p, 2 * a + b, pl.ds(16 * r, 16), cols],
                             lambda i, j, v: emit(2 * i + a, 2 * j + b, v))
                    yield

        def rows_of(i, g, r):
            return pl.ds(_mult(i * RB + g * R + 16 * r, 16), 16)

        def tied(stages):
            while True:
                try:
                    before_next(next(stages))
                except StopIteration as stop:
                    return stop.value
                yield
                yield

        def last_stats(i, r):
            return tied(h_stats(S - RB + i * R + 16 * r))

        def pre1(i, dst, r):
            for c in range(2):
                x = []
                for g in range(4):
                    rows = rows_of(i, g, r)
                    x.append([(hbuf[2 * k + c, rows, :] - hstat[0, rows, :]) * hstat[2, rows, :]
                              for k in range(4)])
                yield from range(3)
                yield from store_sums(dst, r, c, x)

        def post1(i, src, r):
            def emit(g, j, v):
                v = _gelu_of_double(v)
                gbuf[2 * j + c, pl.ds(HALO + i * RB + g * R + 16 * r, 16), :] = v
            for c in range(2):
                for _ in outer(src, r, pl.ds(c * 128, 128), emit):
                    yield
                    yield

        def pre2(i, dst, r):
            for c in range(2):
                x = [[gbuf[2 * k + c, pl.ds(HALO + i * RB + g * R + 16 * r + off, 16), :]
                      for k, off in enumerate((-1, 1, -2, 2))] for g in range(4)]
                yield from store_sums(dst, r, c, x)

        def post2(i, src, r):
            def emit(g, j, v):
                rows = rows_of(i, g, r)
                v = v + jnp.concatenate(
                    [(hbuf[c, rows, :] - hstat[0, rows, :]) * hstat[1, rows, :]
                     for c in (2 * j, 2 * j + 1)], axis=1)
                x1[rows, pl.ds(j * C4, C4)] = v
            for _ in outer(src, r, slice(None), emit):
                yield
                yield

        def pre3(i, r):
            for g in range(4):
                rows = rows_of(i, g, r)
                m, rs = yield from tied(_ln_stages(x1[rows, :]))
                ustat[0, rows_of(0, g, r), :] = jnp.broadcast_to(m, (16, 128))
                ustat[1, rows_of(0, g, r), :] = jnp.broadcast_to(0.5 * rs, (16, 128))
                before_next(rs)
                yield
                yield

        def sums3(i, tie, r):
            for c in range(2):
                x = [[(x1[rows_of(i, g, r), pl.ds(k * C4 + c * 128, 128)]
                       - ustat[0, rows_of(0, g, r), :]) * ustat[1, rows_of(0, g, r), :]
                      for k in range(4)] for g in range(4)]
                yield from store_sums(yc, r, c, x, tie)

        pieces = {pre1: 20, last_stats: 8, post1: 16, pre2: 14, post2: 8, pre3: 16, sums3: 14}

        def spread(stages, slots):
            return _spread([fn(*args, r) for fn, *args in stages for r in range(R // 16)],
                           sum(pieces[fn] for fn, *_ in stages) * (R // 16), slots)

        for c in range(8):
            gbuf[c, pl.ds(0, HALO), :] = jnp.zeros((HALO, 128), f32)
            gbuf[c, pl.ds(HALO + S, HALO), :] = jnp.zeros((HALO, 128), f32)
        first, second = (W1_AT, pre1, post1), (W2_AT, pre2, post2)
        order = [(stage, i - lag) for i in range(NB + 2)
                 for stage, lag in ((first, 0), (second, 2)) if 0 <= i - lag < NB]
        extra = {n: [(last_stats, i)] for i, n in enumerate((0, 4, 6, 8))}
        extra.update({10: [(pre3, 0)], 15: [(sums3, 0, True)]})
        ac, pb = (ac0, ac1), (pb0, pb1)
        spread([(pre1, 0, ac0)], 1)()
        ties.clear()
        for n, ((at, _, _), _) in enumerate(order):
            before = [(post, i, pb[1 - n % 2]) for (_, _, post), i in order[max(n - 1, 0):n]]
            after = [(pre, i, ac[1 - n % 2]) for (_, pre, _), i in order[n + 1:n + 2]]
            stages = before + after if n in (2, 13) else after + before
            side = spread(stages + extra.get(n, []), 47)
            for p in range(7):
                inner(pb[n % 2], p, lambda k: _dot(
                    operand(ac[n % 2], k, (0, 1)), weights(k, at, (C4, 0, C4), (0, 1))), side)
        spread([(post2, NB - 1, pb1)], 1)()

        def out_copy(i):
            rows = pl.ds(_mult(i * (RB // 2), RB // 2), RB // 2)
            return pltpu.make_async_copy(obuf.at[rows], out_hbm.at[rows],
                                         sems.at[SEM_OUT + i])

        nb = (nb0, nb1)

        def activate(c, r):
            act = [[None] * 4 for _ in range(4)]

            def emit(g, j, v):
                act[g][j] = _gelu_of_double(v)
            for _ in outer(nb[c % 2], r, slice(None), emit):
                yield
                yield
            yield from store_sums(hc, r, c, act, False)

        pieces[activate] = 15

        def mlp_up():
            for c in range(7):
                side = spread([(activate, c - 1)] if c else [], 49)
                for p in range(7):
                    inner(nb[c % 2], p, lambda n: _dot(
                        operand(yc, n, (0, 1)), weights(n, W3_AT, (C4, 0, C4), (c,))), side)

        def mlp_down(i, stages):
            def down(p, side, k0=0, k1=F4):
                inner(db, p, lambda n: _dot(operand(hc, n, range(k0 // 128, k1 // 128)),
                                            weights(n, W4_AT, (F4, k0, k1 - k0), (0, 1))),
                      side, add=k0 > 0)

            def finish(bi, bj, plus, minus=()):
                for a in range(2):
                    for b in range(2):
                        rows = pl.ds(_mult(i * RB + (2 * bi + a) * R, R), R)
                        cols = pl.ds((2 * bj + b) * C4, C4)
                        v = x1[rows, cols] + jnp.concatenate(
                            [hbuf[4 * bj + 2 * b + c, rows, :] for c in range(2)], axis=1)
                        for p in minus:
                            v = v - db[p, 2 * a + b]
                        for p in plus:
                            v = v + db[p, 2 * a + b]
                        obuf[rows, cols] = v.astype(bf16)

            down(0, spread([(activate, 6)], 6), 0, F4 - 128)
            down(0, lambda: None, F4 - 128)
            side = spread(stages, 35)
            for p in range(1, 7):
                down(p, side)
                if p == 3:
                    finish(0, 1, (1, 2))
                if p == 5:
                    finish(0, 0, (0, 3, 4), (1,))
            finish(1, 0, (4, 5))
            finish(1, 1, (2, 3, 6), (5,))

        @pl.loop(0, NB)
        def _(i):
            ties.clear()
            mlp_up()
            nxt = jnp.minimum(i + 1, NB - 1)
            mlp_down(i, [(pre3, nxt), (sums3, nxt, False)])
            out_copy(2 * i).start()
            out_copy(2 * i + 1).start()

        for i in range(2 * NB):
            out_copy(i).wait()

    pl.run_scoped(
        block_b,
        pltpu.VMEM((8, S + 2 * HALO, 128), f32),
        pltpu.VMEM((2, RB, 128), f32),
        pltpu.VMEM((S, D), f32),
        pltpu.VMEM((S, D), bf16),
        pltpu.VMEM((49, 2, R, 128), bf16),
        pltpu.VMEM((49, 7, R, 128), bf16),
        pltpu.VMEM((7, 4, R, C4), f32),
        *[pltpu.VMEM((7, 4, R, 128), f32)] * 2,
        *[pltpu.VMEM((49, 2, R, 128), bf16)] * 2,
        *[pltpu.VMEM((7, 4, R, C4), f32)] * 2,
    )


@jax.jit
def pallas_sequential_preLN__memory_aug_recurrent_mem_tr__mixer_s_mlp__prompt_kernel(
    A_x: jax.Array,
    A_mem0: jax.Array,
    A_Wq: jax.Array,
    A_Wk: jax.Array,
    A_Wv: jax.Array,
    A_Wo: jax.Array,
    A_seg_len: jax.Array,
    B_x: jax.Array,
    B_w1: jax.Array,
    B_w2: jax.Array,
    B_w3: jax.Array,
    B_w4: jax.Array,
):
    del A_seg_len, B_x
    hbm = pl.BlockSpec(memory_space=pl.ANY)
    vmem = pl.BlockSpec(memory_space=pltpu.VMEM)
    scratch = [
        pltpu.VMEM((8, S, 128), f32),
        pltpu.VMEM((3, S, 128), f32),
        pltpu.SemaphoreType.DMA((NSEM,)),
        pltpu.SMEM((1,), jnp.int32),
    ] + [pltpu.VMEM((4, WROWS, 128), bf16)] * 4 + [pltpu.VMEM((WROWS, 128), bf16)] * 33
    out = pl.pallas_call(
        _kernel,
        out_shape=jax.ShapeDtypeStruct((S, D), A_x.dtype),
        in_specs=[hbm, vmem] + [hbm] * 8,
        out_specs=hbm,
        scratch_shapes=scratch,
        compiler_params=pltpu.CompilerParams(vmem_limit_bytes=128 * 1024 * 1024),
    )(A_x.reshape(NSEG, SEG, D), A_mem0.reshape(MEM, D),
      A_Wq.reshape(2, D // 4, 2 * H, DH), A_Wk.reshape(2, D // 4, 2 * H, DH),
      A_Wv.reshape(2, D // 4, 2 * H, DH), A_Wo.reshape(NP, 2, DH, D),
      B_w1.reshape(4, C4, D), B_w2.reshape(4, C4, D),
      B_w3.reshape(4, C4, F), B_w4.reshape(4, F4, D))
    return out.reshape(A_x.shape)
```

```python
import functools
import itertools

import jax
import jax.numpy as jnp
from jax import lax
import jax.experimental.pallas as pl
import jax.experimental.pallas.tpu as pltpu

S = 2048
D = 1024
H = 32
DH = 128
MEM = 8
SEG = 32
F = 3584
NSEG = S // SEG
NP = H // 2
HD = D // 2
C4 = D // 4
F4 = F // 4
HALO = 8
R = 64
RB = 4 * R
NB = S // RB
EPS = 1e-5
NEG = -1000000000.0
LOG2E = 1.4426950408889634

W1_AT, W2_AT, W3_AT, W4_AT = 0, 2 * C4, 4 * C4, 11 * C4
WROWS = W4_AT + 2 * F4
WO_ROWS = 4 * DH * 8
WO_AT = WROWS - WO_ROWS
BATCH = ((0,), (1, 2, 3, 4, 5), (6, 7, 8, 9, 10), (11, 12), ())

LAG_QK, LAG_PV, LAG_WO = 2, 4, 6
FILL_AT = (14, 18)

bf16 = jnp.bfloat16
f32 = jnp.float32
u32 = jnp.uint32

SEM_XP, SEM_X, SEM_WO, SEM_STRIP, SEM_OUT, SEM_W = 0, 8, 10, 14, 16, 16 + 2 * NB
NSEM = SEM_W + 12


def _mult(i, n):
    return i if isinstance(i, int) else pl.multiple_of(i, n)


def _ln(x):
    d = x - jnp.mean(x, axis=-1, keepdims=True)
    return d * lax.rsqrt(jnp.mean(d * d, axis=-1, keepdims=True) + EPS)


def _ln_stages(x):
    m = jnp.mean(x, axis=-1, keepdims=True)
    yield m
    d = x - m
    return m, lax.rsqrt(jnp.mean(d * d, axis=-1, keepdims=True) + EPS)


def _gelu_of_double(y):
    c = 0.7978845608028654
    return y + y * jnp.tanh(y * (2 * c + (8 * c * 0.044715) * (y * y)))


def _dot(a, b):
    return jnp.dot(a, b, preferred_element_type=f32)


def _load(ref, *idx, r0=0, n=None):
    n = ref.shape[-2] if n is None else n
    return pltpu.bitcast(
        ref.bitcast(u32)[(*idx, pl.ds(_mult(r0 >> 1, 8), n // 2), slice(None))], bf16)


def _sums_a(a11, a12, a21, a22):
    return [lambda: a12 - a22, lambda: a11 + a12, lambda: a11, lambda: a11 + a22,
            lambda: a22, lambda: a21 + a22, lambda: a21 - a11]


def _sums_b(b11, b12, b21, b22):
    return [lambda: b21 + b22, lambda: b22, lambda: b12 - b22, lambda: b11 + b22,
            lambda: b21 - b11, lambda: b11, lambda: b11 + b12]


def _combine(product, emit):
    c11 = product(0)
    c12 = product(1)
    c11 = c11 - c12
    c22 = product(2)
    emit(0, 1, c12 + c22)
    t = product(3)
    c11 = c11 + t
    c22 = c22 + t
    c21 = product(4)
    emit(0, 0, c11 + c21)
    t = product(5)
    emit(1, 0, c21 + t)
    c22 = c22 - t
    emit(1, 1, c22 + product(6))


def _sums2(sums, x, emit):
    outer = [sums(x[i][j], x[i][2 + j], x[2 + i][j], x[2 + i][2 + j])
             for i in range(2) for j in range(2)]
    for p in range(7):
        for q, v in enumerate(sums(*(o[p]() for o in outer))):
            emit(7 * p + q, v)
        yield


def _spread(tasks, pieces, slots):
    todo = itertools.chain(*tasks)
    calls = itertools.count(1)

    def advance():
        k = next(calls)
        if k > slots:
            return
        for _ in range(pieces * k // slots - pieces * (k - 1) // slots):
            next(todo)
        if k == slots:
            assert next(todo, todo) is todo
    return advance


def _tie(never, words, values):
    regs = [[w[r:r + 8] for r in range(0, w.shape[0], 8)] for w in words]
    per = len(regs[0])
    for n, v in enumerate(values):
        c, r = divmod(len(regs) * per * n // len(values), per)
        regs[c][r] = jnp.where(never, pltpu.bitcast(v, u32), regs[c][r])
    return [jnp.concatenate(w, axis=0) for w in regs] if values else words


def _upper_operands(a11, a12, a22):
    k = a11.shape[0] - a22.shape[0]
    ops = [jnp.concatenate([a12[:k], a12[k:] - a22], axis=0), a11 + a12, a11,
           jnp.concatenate([a11[:k], a11[k:] + a22], axis=0)]
    return [v.astype(bf16) for v in ops]


PLAIN = {40: 0, 36: 1, 12: 2, 8: 3}
OTHER = [n for n in range(49) if n not in PLAIN]
RAW_SLOT = dict(zip(OTHER[2::3], [(k, j) for k in range(4) for j in range(4) if k != j]))
RAW_SLOT.update({n: (k, k) for n, k in PLAIN.items()})


def _kernel(x_hbm, mem0_ref, wq_hbm, wk_hbm, wv_hbm, wo_hbm, w1_hbm, w2_hbm,
            w3_hbm, w4_hbm, out_hbm, hbuf, hstat, sems, zero_ref, *wbufs):
    zero_ref[0] = 0
    raw, spare = wbufs[:4], wbufs[4:]
    wsum = {n: (raw[j], k) for n, (k, j) in RAW_SLOT.items()}
    wsum.update({n: (b,) for n, b in zip((n for n in OTHER if n not in RAW_SLOT), spare)})

    def load_h(rows):
        return jnp.concatenate([hbuf[c, rows, :] for c in range(8)], axis=1)

    def h_stats(r0):
        rows = pl.ds(_mult(r0, 16), 16)
        hv = load_h(rows)
        m1, r1 = yield from _ln_stages(hv)
        yield r1
        m2, r2 = yield from _ln_stages((hv - m1) * r1)
        stats = (m1 + m2 / r1, r1, 0.5 * r1 * r2)
        for k, v in enumerate(stats):
            hstat[k, rows, :] = jnp.broadcast_to(v, (16, 128))
        yield stats[0] + stats[2]

    def strip_copies(batch):
        strips = [(w, at + u * w.shape[1], u)
                  for w, at in ((w1_hbm, W1_AT), (w2_hbm, W2_AT), (w3_hbm, W3_AT), (w4_hbm, W4_AT))
                  for u in range(w.shape[2] // 512)]
        return [pltpu.make_async_copy(
            w.at[:, :, pl.ds(j * (w.shape[2] // 4) + u * 128, 128)],
            raw[j].at[:, pl.ds(at, w.shape[1]), :], sems.at[SEM_STRIP + batch % 2])
            for w, at, u in (strips[n] for n in BATCH[batch]) for j in range(4)]

    def weight_sums(r0):
        x = [[_load(raw[j], k, r0=r0, n=16).astype(f32) for j in range(4)]
             for k in range(4)]

        def emit(n, v):
            if n not in PLAIN:
                ref, *idx = wsum[n]
                ref[(*idx, pl.ds(_mult(r0, 16), 16), slice(None))] = v().astype(bf16)
        yield from _sums2(_sums_b, x, emit)

    def block_a(xb, xn, lo, *bufs):
        w_on, low, wo_s = bufs[0:3], bufs[3:6], bufs[6:13]
        w_hbm = (wq_hbm, wk_hbm, wv_hbm)
        stage = hbuf.reshape(8, S // 8, 8, DH)
        lhs = spare[2:5]
        w_low = [spare[5 + 3 * m:8 + 3 * m] for m in range(3)]

        def x_copy(i):
            return pltpu.make_async_copy(x_hbm.at[pl.ds(2 * i, 2)], xb.at[i & 3],
                                         sems.at[SEM_X + (i & 1)])

        def wo_copies(g):
            return [pltpu.make_async_copy(
                wo_hbm.at[g, duo], raw[duo].at[g, pl.ds(WO_AT, WO_ROWS)], sems.at[SEM_WO + g])
                for duo in range(2)]

        def chunk_copies(g, m):
            src = w_hbm[m].bitcast(f32)
            return [pltpu.make_async_copy(
                src.at[half, :, :, g], stage.at[pl.ds(2 * m, 2), :, pl.ds(4 * half, 4), :],
                sems.at[SEM_W + 3 * g + m]) for half in range(2)]

        def start(copies):
            for c in copies:
                c.start()

        def wait(copies):
            for c in copies:
                c.wait()

        def qkv_sums(g, m, duo, d0):
            lower, done = [], []
            for d in (d0, d0 + C4):
                for pair in (2 * duo, 2 * duo + 1):
                    b = []
                    for half in range(2):
                        rows = pl.ds(8 * d0 + 4 * half + pair, 16, stride=8)
                        w = pltpu.bitcast(hbuf[2 * m + d // C4, rows, :], u32)
                        b += [pltpu.bitcast(w << 16, f32),
                              pltpu.bitcast(w & jnp.uint32(0xFFFF0000), f32)]
                    sums = [v() for v in _sums_b(*b)]
                    for k in range(4):
                        w_on[m][4 * g + pair, k, pl.ds(d, 16), :] = sums[k].astype(bf16)
                    lower.append(sums[4:])
                    done.append(sums[3])
            for k in range(3):
                for q, v in enumerate(_sums_b(*(b[k] for b in lower))):
                    v = v()
                    rows = pl.ds(_mult((7 * duo + q) * C4 + d0, 16), 16)
                    w_low[m][k][rows, :] = v.astype(bf16)
                done.append(v)
            return done

        def wo_sums(g, pair, e0, n0):
            at = WO_AT + pair % 2 * 16 * DH + 8 * e0 + 8 * n0
            tiles = [[_load(raw[pair // 2], g, r0=at + 8 * DH * i + 32 * j + 64 * r, n=16)
                      .astype(f32) for r in range(2)] for i in range(2) for j in range(2)]
            done = []
            for n in range(2):
                b = [jnp.concatenate([v[8 * n:8 * n + 8] for v in t], axis=0) for t in tiles]
                for k, v in enumerate(_sums_b(*b)):
                    v = v()
                    wo_s[k][n0 + n, 4 * g + pair, pl.ds(e0, 16), :] = v.astype(bf16)
                done.append(v)
            return done

        def prologue(xpb):
            def xp_copy(i):
                segs = pl.ds(8 * i, 8)
                return pltpu.make_async_copy(x_hbm.at[segs, pl.ds(16, 16), :], xpb.at[segs],
                                             sems.at[SEM_XP + i])

            start(chunk_copies(0, 0))
            start([xp_copy(i) for i in range(NSEG // 8)])
            start(chunk_copies(0, 1))
            start(chunk_copies(0, 2))
            lo[...] = jnp.zeros(lo.shape, f32)
            for duo in range(2):
                raw[duo][3, pl.ds(WO_AT, WO_ROWS), :] = jnp.zeros((WO_ROWS, 128), bf16)
            wait(chunk_copies(0, 0))

            @pl.loop(0, 2)
            def _(duo):
                for d0 in range(0, C4, 16):
                    qkv_sums(0, 0, duo, d0)

            @pl.loop(0, NSEG // 8)
            def _(i):
                xp_copy(i).wait()
                for j in range(2):
                    ops = []
                    for n in range(2):
                        a = [_ln(_load(xpb, 8 * i + 4 * j + 2 * n + k).astype(f32))
                             for k in range(2)]
                        a1 = jnp.concatenate([a[0][:8], a[1][:8]], axis=0)
                        a2 = jnp.concatenate([a[0][8:], a[1][8:]], axis=0)
                        sums = _sums_a(a1[:, :HD], a1[:, HD:], a2[:, :HD], a2[:, HD:])
                        ops.append([v() for v in sums[4:]])
                    for k in range(3):
                        top, bottom = ops[0][k], ops[1][k]
                        for q, v in enumerate(_sums_a(top[:, :C4], top[:, C4:],
                                                      bottom[:, :C4], bottom[:, C4:])):
                            v = v()
                            for c in range(2):
                                r0 = (2 * q + c) * 4 * NSEG + 32 * i + 16 * j
                                lhs[k][pl.ds(pl.multiple_of(r0, 16), 16), :] = (
                                    v[:, c * 128:(c + 1) * 128].astype(bf16))

        pl.run_scoped(prologue, pltpu.VMEM((NSEG, 16, D), bf16))

        def lower_products(g, m):
            m1 = (m + 1) % 3
            never = jnp.full((8, 128), zero_ref[0]) != 0
            g1 = jnp.minimum(g + (1 if m == 2 else 0), 3)
            side = [functools.partial(qkv_sums, g1, m1, duo, d0)
                    for duo in range(2) for d0 in range(0, C4, 16)]
            wait_at = 16
            span = 42 - wait_at
            early = [functools.partial(wo_sums, (g + 3) & 3, pair, e0, n0)
                     for pair in range(4 if m == 2 else 0)
                     for e0 in range(0, DH, 16) for n0 in (0, 2)]

            def product(duo, k, q):
                j = 21 * duo + 7 * k + q
                if j >= wait_at:
                    todo = side[len(side) * (j - wait_at) // span:
                                len(side) * (j - wait_at + 1) // span]
                else:
                    todo = early[len(early) * j // wait_at:len(early) * (j + 1) // wait_at]
                a = [lhs[k].bitcast(u32)[pl.ds((2 * q + c) * 2 * NSEG, 2 * NSEG), :]
                     for c in range(2)]
                a[1:] = _tie(never, a[1:], [v[8:] for fn in todo for v in fn()])
                a = jnp.concatenate([pltpu.bitcast(v, bf16) for v in a], axis=1)
                res = _dot(a, _load(w_low[m][k], r0=(7 * duo + q) * C4, n=C4))
                if j == wait_at - 1:
                    pl.when(3 * g + m < 11)(lambda: wait(chunk_copies(g1, m1)))
                    pl.when(g < 3)(lambda: start(chunk_copies(g + 1, m)))
                    if m == 1:
                        pl.when(g > 0)(lambda: wait(wo_copies(g - 1)))
                        start(wo_copies(g))
                        pl.when(g == 3)(
                            lambda: start([x_copy(0), x_copy(1)] + strip_copies(0)))
                return res

            for duo in range(2):
                last = {}
                for k in range(3):
                    def emit(a, b, res):
                        v = res if k == 0 else res + last[a, b] if k == 1 else res - last[a, b]
                        last[a, b] = res
                        for n in range(NSEG // 4):
                            low[m][2 * n + a, 4 * g + 2 * duo + b, k] = (
                                v[16 * n:16 * n + 16].astype(bf16))
                    _combine(functools.partial(product, duo, k), emit)

        @pl.loop(0, 4)
        def _(g):
            for m in range(3):
                lower_products(g, m)

        def norm_tokens(i, k):
            for r0 in range(0, SEG, 16):
                v = _load(xb, jnp.minimum(i, NSEG // 2 - 1) & 3, k, r0=r0, n=16).astype(f32)
                m, r = yield from _ln_stages(v)
                xn[k, pl.ds(r0, 16), :] = (v - m) * r
                yield r

        def lower_wo(grp, n, k):
            w = jnp.concatenate([_load(wo_s[4 + k], n, t) for t in range(NP)], axis=0)
            return _dot(lo[grp & 1, k].astype(bf16), w)

        def add_lower(grp, n, m4, m2, m6):
            for j in range(4):
                seg = slice(8 * j, 8 * j + 8)
                upper = pl.ds(_mult((4 * grp + j) * SEG + 16, 8), 8)
                lower = pl.ds(_mult((4 * grp + j) * SEG + 24, 8), 8)
                hbuf[n, upper, :] += m4[seg]
                hbuf[n, lower, :] += m2[seg] + m4[seg]
                hbuf[4 + n, lower, :] += m6[seg] - m2[seg]

        def attention_mask():
            def split(axis):
                r = lax.broadcasted_iota(jnp.int32, (80, 80), axis)
                return (jnp.where(r < 64, r >> 5, (r - 64) >> 3),
                        jnp.where(r < 64, r & 31, 32 + (r & 7)))
            (hq, pq), (hk, pk) = split(0), split(1)
            visible = (pq < MEM) | (pq >= pk)
            return jnp.where(hq == hk, jnp.where(visible, 0.0, NEG * DH ** 0.5), -jnp.inf)

        def step(i, k, mem, fill, side):
            tok = xn[k]
            r0 = jnp.maximum(2 * i + k - 8, 0) * SEG
            norms = itertools.chain(h_stats(r0), h_stats(r0 + 16), norm_tokens(i + 1, k))
            s = 2 * i + k
            a1 = jnp.concatenate([mem, tok[:24]], axis=0)
            ops = _upper_operands(a1[:, :HD], a1[:, HD:], tok[24:, HD:])
            qkvs, scores, outs, lower = {}, {}, {}, []
            total = [None] * 4

            def qkv(t):
                res = []
                for m in range(3):
                    m7, m5, m3, m1 = [_dot(ops[j], _load(w_on[m], t, j)) for j in range(4)]
                    m4, c21, m62 = [
                        _load(low[m], i, t, j).astype(f32)[8 * k:8 * k + 8]
                        for j in range(3)]
                    side()
                    c11 = m7 - m5 + m1
                    res.append(jnp.concatenate(
                        [c11[:24], c11[24:] + m4, m5 + m3, c21, m3[24:] + m62 + m1[24:]],
                        axis=0).astype(bf16))
                qkvs[t] = res

            def qk(t):
                q, kk, v = qkvs.pop(t)
                sc = lax.dot_general(q, kk, (((1,), (1,)), ((), ())),
                                     preferred_element_type=f32)
                scores[t] = (sc, v)

            def pv(t):
                sc, v = scores.pop(t)
                sc = jnp.where(fill == 0.0, sc, fill)
                tie = next(norms, None) if t >= 1 else None
                if tie is not None:
                    sc = jnp.concatenate([jnp.where(never, tie, sc[:16]), sc[16:]], axis=0)
                mx = jnp.max(sc, axis=1, keepdims=True)
                e = jnp.exp2((sc - mx) * (DH ** -0.5 * LOG2E))
                den = jnp.sum(e, axis=1, keepdims=True)
                inv = pl.reciprocal(den, approx=True)
                inv = inv * (2.0 - den * inv)
                outs[t] = _dot(e.astype(bf16), v) * inv

            def wo(t):
                o = outs.pop(t)
                a11, a12, a21, a22 = o[:32], o[32:64], o[64:72], o[72:]
                rows = pl.ds(pl.multiple_of(8 * (s & 3), 8), 8)
                for j, v in enumerate((a22, a21 + a22, a21 - a11[24:])):
                    lo[(s >> 2) & 1, j, rows, pl.ds(t * DH, DH)] = v
                for j, a in enumerate(_upper_operands(a11, a12, a22)):
                    r = _dot(a, jnp.concatenate(
                        [_load(wo_s[j], n, t) for n in range(4)], axis=1))
                    total[j] = r if total[j] is None else total[j] + r

            for t in range(NP + LAG_WO):
                if t < NP:
                    qkv(t)
                if t in FILL_AT:
                    lower.append(lower_wo((s >> 2) - 1, s & 3, len(lower)))
                if t % 2:
                    for fn, lag in ((qk, LAG_QK), (pv, LAG_PV)):
                        for u in (t - 1 - lag, t - lag):
                            if 0 <= u < NP:
                                fn(u)
                if t >= LAG_WO:
                    wo(t - LAG_WO)

            m7, m5, m3, m1 = total
            upper = jnp.concatenate([m7 - m5 + m1, m5 + m3], axis=1)
            c22 = m3[24:] + m1[24:]
            xv = _load(xb, i & 3, k).astype(f32)
            hv = jnp.concatenate(
                [xv[:24] + upper[MEM:],
                 jnp.concatenate([xv[24:, :HD], xv[24:, HD:] + c22], axis=1)], axis=0)
            for c in range(8):
                hbuf[c, pl.ds(pl.multiple_of(s * SEG, SEG), SEG), :] = hv[:, c * 128:(c + 1) * 128]
            add_lower(jnp.maximum((s >> 2) - 1, 0), s & 3,
                      *lower, lower_wo((s >> 2) - 1, s & 3, 2))
            return upper[:MEM]

        fill = attention_mask()
        never = jnp.full((16, 80), zero_ref[0]) != 0
        n_it = NSEG // 2
        per_it = WROWS // 16 // n_it

        def steps(i, mem):
            pl.when(i + 1 < n_it)(lambda: x_copy(i + 1).wait())
            pl.when(i + 2 < n_it)(lambda: x_copy(i + 2).start())

            @pl.when(i < len(BATCH) - 1)
            def _():
                for b in range(len(BATCH) - 1):
                    @pl.when(i == b)
                    def _():
                        wait(strip_copies(b))
                        start(strip_copies(b + 1))

            side = _spread([weight_sums(16 * (per_it * i + j)) for j in range(per_it)],
                           7 * per_it, 90)
            for k in range(2):
                mem = step(i, k, mem, fill, side)
            return mem

        wait(wo_copies(3) + [x_copy(0)])
        for pair in range(4):
            for e0 in range(0, DH, 16):
                for n0 in (0, 2):
                    wo_sums(3, pair, e0, n0)
        hbuf[:, pl.ds(0, 4 * SEG), :] = jnp.zeros((8, 4 * SEG, 128), f32)
        _spread([norm_tokens(0, 0), norm_tokens(0, 1)], 8, 1)()
        lax.fori_loop(0, n_it, steps, mem0_ref[...].astype(f32))
        for n in range(4):
            add_lower(NSEG // 4 - 1, n, *(lower_wo(NSEG // 4 - 1, n, k) for k in range(3)))

    pl.run_scoped(
        block_a,
        pltpu.VMEM((4, 2, SEG, D), bf16),
        pltpu.VMEM((2, SEG, D), f32),
        pltpu.VMEM((2, 3, 32, NP * DH), f32),
        *[pltpu.VMEM((NP, 4, HD, DH), bf16)] * 3,
        *[pltpu.VMEM((NSEG // 2, NP, 3, 16, DH), bf16)] * 3,
        *[pltpu.VMEM((4, NP, DH, 128), bf16)] * 7,
    )

    def block_b(gbuf, ustat, x1, obuf, yc, hc, db, nb0, nb1, ac0, ac1, pb0, pb1):
        def weights(n, at, rows, strips):
            return jnp.concatenate(
                [_load(*wsum[n], r0=at + k * rows[0] + rows[1], n=rows[2])
                 for k in strips], axis=1)

        ties = []
        never = jnp.full((8, 128), zero_ref[0]) != 0

        def before_next(value):
            if value.shape[1] == 1:
                value = jnp.broadcast_to(value[:8] + value[8:], (8, 128))
            ties.append(value[-8:, -128:])

        def operand(ref, n, cols):
            words = [ref.bitcast(u32)[n, c] for c in cols]
            words = _tie(never, words, ties)
            ties.clear()
            return jnp.concatenate([pltpu.bitcast(w, bf16) for w in words], axis=1)

        def store_sums(dst, r, c, x, tie=True):
            def emit(n, v):
                v = v()
                dst[n, c, pl.ds(16 * r, 16), :] = v.astype(bf16)
                if tie and n % 2:
                    before_next(v)
            return _sums2(_sums_a, x, emit)

        def inner(dst, p, product, side, add=False):
            def emit(a, b, v):
                dst[p, 2 * a + b] = dst[p, 2 * a + b] + v if add else v

            def run(k):
                r = product(7 * p + k)
                side()
                return r
            _combine(run, emit)

        def outer(src, r, cols, emit):
            for a in range(2):
                for b in range(2):
                    _combine(lambda p: src[p, 2 * a + b, pl.ds(16 * r, 16), cols],
                             lambda i, j, v: emit(2 * i + a, 2 * j + b, v))
                    yield

        def rows_of(i, g, r):
            return pl.ds(_mult(i * RB + g * R + 16 * r, 16), 16)

        def tied(stages):
            while True:
                try:
                    before_next(next(stages))
                except StopIteration as stop:
                    return stop.value
                yield
                yield

        def last_stats(i, r):
            return tied(h_stats(S - RB + i * R + 16 * r))

        def pre1(i, dst, r):
            for c in range(2):
                x = []
                for g in range(4):
                    rows = rows_of(i, g, r)
                    x.append([(hbuf[2 * k + c, rows, :] - hstat[0, rows, :]) * hstat[2, rows, :]
                              for k in range(4)])
                yield from range(3)
                yield from store_sums(dst, r, c, x)

        def post1(i, src, r):
            def emit(g, j, v):
                v = _gelu_of_double(v)
                gbuf[2 * j + c, pl.ds(HALO + i * RB + g * R + 16 * r, 16), :] = v
            for c in range(2):
                for _ in outer(src, r, pl.ds(c * 128, 128), emit):
                    yield
                    yield

        def pre2(i, dst, r):
            for c in range(2):
                x = [[gbuf[2 * k + c, pl.ds(HALO + i * RB + g * R + 16 * r + off, 16), :]
                      for k, off in enumerate((-1, 1, -2, 2))] for g in range(4)]
                yield from store_sums(dst, r, c, x)

        def post2(i, src, r):
            def emit(g, j, v):
                rows = rows_of(i, g, r)
                v = v + jnp.concatenate(
                    [(hbuf[c, rows, :] - hstat[0, rows, :]) * hstat[1, rows, :]
                     for c in (2 * j, 2 * j + 1)], axis=1)
                x1[rows, pl.ds(j * C4, C4)] = v
            for _ in outer(src, r, slice(None), emit):
                yield
                yield

        def pre3(i, r):
            for g in range(4):
                rows = rows_of(i, g, r)
                m, rs = yield from tied(_ln_stages(x1[rows, :]))
                ustat[0, rows_of(0, g, r), :] = jnp.broadcast_to(m, (16, 128))
                ustat[1, rows_of(0, g, r), :] = jnp.broadcast_to(0.5 * rs, (16, 128))
                before_next(rs)
                yield
                yield

        def sums3(i, tie, r):
            for c in range(2):
                x = [[(x1[rows_of(i, g, r), pl.ds(k * C4 + c * 128, 128)]
                       - ustat[0, rows_of(0, g, r), :]) * ustat[1, rows_of(0, g, r), :]
                      for k in range(4)] for g in range(4)]
                yield from store_sums(yc, r, c, x, tie)

        pieces = {pre1: 20, last_stats: 8, post1: 16, pre2: 14, post2: 8, pre3: 16, sums3: 14}

        def spread(stages, slots):
            return _spread([fn(*args, r) for fn, *args in stages for r in range(R // 16)],
                           sum(pieces[fn] for fn, *_ in stages) * (R // 16), slots)

        for c in range(8):
            gbuf[c, pl.ds(0, HALO), :] = jnp.zeros((HALO, 128), f32)
            gbuf[c, pl.ds(HALO + S, HALO), :] = jnp.zeros((HALO, 128), f32)
        first, second = (W1_AT, pre1, post1), (W2_AT, pre2, post2)
        order = [(stage, i - lag) for i in range(NB + 2)
                 for stage, lag in ((first, 0), (second, 2)) if 0 <= i - lag < NB]
        extra = {n: [(last_stats, i)] for i, n in enumerate((0, 4, 6, 8))}
        extra.update({10: [(pre3, 0)], 15: [(sums3, 0, True)]})
        ac, pb = (ac0, ac1), (pb0, pb1)
        spread([(pre1, 0, ac0)], 1)()
        ties.clear()
        for n, ((at, _, _), _) in enumerate(order):
            before = [(post, i, pb[1 - n % 2]) for (_, _, post), i in order[max(n - 1, 0):n]]
            after = [(pre, i, ac[1 - n % 2]) for (_, pre, _), i in order[n + 1:n + 2]]
            stages = before + after if n in (2, 13) else after + before
            side = spread(stages + extra.get(n, []), 47)
            for p in range(7):
                inner(pb[n % 2], p, lambda k: _dot(
                    operand(ac[n % 2], k, (0, 1)), weights(k, at, (C4, 0, C4), (0, 1))), side)
        spread([(post2, NB - 1, pb1)], 1)()

        def out_copy(i):
            rows = pl.ds(_mult(i * (RB // 2), RB // 2), RB // 2)
            return pltpu.make_async_copy(obuf.at[rows], out_hbm.at[rows],
                                         sems.at[SEM_OUT + i])

        nb = (nb0, nb1)

        def activate(c, r):
            act = [[None] * 4 for _ in range(4)]

            def emit(g, j, v):
                act[g][j] = _gelu_of_double(v)
            for _ in outer(nb[c % 2], r, slice(None), emit):
                yield
                yield
            yield from store_sums(hc, r, c, act, False)

        pieces[activate] = 15

        def mlp_up():
            for c in range(7):
                side = spread([(activate, c - 1)] if c else [], 49)
                for p in range(7):
                    inner(nb[c % 2], p, lambda n: _dot(
                        operand(yc, n, (0, 1)), weights(n, W3_AT, (C4, 0, C4), (c,))), side)

        def mlp_down(i, stages):
            def down(p, side, k0=0, k1=F4):
                inner(db, p, lambda n: _dot(operand(hc, n, range(k0 // 128, k1 // 128)),
                                            weights(n, W4_AT, (F4, k0, k1 - k0), (0, 1))),
                      side, add=k0 > 0)

            def finish(bi, bj, plus, minus=()):
                for a in range(2):
                    for b in range(2):
                        rows = pl.ds(_mult(i * RB + (2 * bi + a) * R, R), R)
                        cols = pl.ds((2 * bj + b) * C4, C4)
                        v = x1[rows, cols] + jnp.concatenate(
                            [hbuf[4 * bj + 2 * b + c, rows, :] for c in range(2)], axis=1)
                        for p in minus:
                            v = v - db[p, 2 * a + b]
                        for p in plus:
                            v = v + db[p, 2 * a + b]
                        obuf[rows, cols] = v.astype(bf16)

            down(0, spread([(activate, 6)], 6), 0, F4 - 128)
            down(0, lambda: None, F4 - 128)
            side = spread(stages, 35)
            for p in range(1, 7):
                down(p, side)
                if p == 3:
                    finish(0, 1, (1, 2))
                if p == 5:
                    finish(0, 0, (0, 3, 4), (1,))
            finish(1, 0, (4, 5))
            finish(1, 1, (2, 3, 6), (5,))

        @pl.loop(0, NB)
        def _(i):
            ties.clear()
            mlp_up()
            nxt = jnp.minimum(i + 1, NB - 1)
            mlp_down(i, [(pre3, nxt), (sums3, nxt, False)])
            out_copy(2 * i).start()
            out_copy(2 * i + 1).start()

        for i in range(2 * NB):
            out_copy(i).wait()

    pl.run_scoped(
        block_b,
        pltpu.VMEM((8, S + 2 * HALO, 128), f32),
        pltpu.VMEM((2, RB, 128), f32),
        pltpu.VMEM((S, D), f32),
        pltpu.VMEM((S, D), bf16),
        pltpu.VMEM((49, 2, R, 128), bf16),
        pltpu.VMEM((49, 7, R, 128), bf16),
        pltpu.VMEM((7, 4, R, C4), f32),
        *[pltpu.VMEM((7, 4, R, 128), f32)] * 2,
        *[pltpu.VMEM((49, 2, R, 128), bf16)] * 2,
        *[pltpu.VMEM((7, 4, R, C4), f32)] * 2,
    )


@jax.jit
def pallas_sequential_preLN__memory_aug_recurrent_mem_tr__mixer_s_mlp__prompt_kernel(
    A_x: jax.Array,
    A_mem0: jax.Array,
    A_Wq: jax.Array,
    A_Wk: jax.Array,
    A_Wv: jax.Array,
    A_Wo: jax.Array,
    A_seg_len: jax.Array,
    B_x: jax.Array,
    B_w1: jax.Array,
    B_w2: jax.Array,
    B_w3: jax.Array,
    B_w4: jax.Array,
):
    del A_seg_len, B_x
    hbm = pl.BlockSpec(memory_space=pl.ANY)
    vmem = pl.BlockSpec(memory_space=pltpu.VMEM)
    scratch = [
        pltpu.VMEM((8, S, 128), f32),
        pltpu.VMEM((3, S, 128), f32),
        pltpu.SemaphoreType.DMA((NSEM,)),
        pltpu.SMEM((1,), jnp.int32),
    ] + [pltpu.VMEM((4, WROWS, 128), bf16)] * 4 + [pltpu.VMEM((WROWS, 128), bf16)] * 33
    out = pl.pallas_call(
        _kernel,
        out_shape=jax.ShapeDtypeStruct((S, D), A_x.dtype),
        in_specs=[hbm, vmem] + [hbm] * 8,
        out_specs=hbm,
        scratch_shapes=scratch,
        compiler_params=pltpu.CompilerParams(vmem_limit_bytes=128 * 1024 * 1024),
    )(A_x.reshape(NSEG, SEG, D), A_mem0.reshape(MEM, D),
      A_Wq.reshape(2, 2, C4, 4, 8, DH), A_Wk.reshape(2, 2, C4, 4, 8, DH),
      A_Wv.reshape(2, 2, C4, 4, 8, DH),
      A_Wo.reshape(H * DH // 8, 8, 8, 128).transpose(0, 2, 1, 3).reshape(4, 2, WO_ROWS, 128),
      B_w1.reshape(4, C4, D), B_w2.reshape(4, C4, D),
      B_w3.reshape(4, C4, F), B_w4.reshape(4, F4, D))
    return out.reshape(A_x.shape)
```

```python
import functools
import itertools

import jax
import jax.numpy as jnp
from jax import lax
import jax.experimental.pallas as pl
import jax.experimental.pallas.tpu as pltpu

S = 2048
D = 1024
H = 32
DH = 128
MEM = 8
SEG = 32
F = 3584
NSEG = S // SEG
NP = H // 2
HD = D // 2
C4 = D // 4
F4 = F // 4
HALO = 8
R = 64
RB = 4 * R
NB = S // RB
EPS = 1e-5
NEG = -1000000000.0
LOG2E = 1.4426950408889634

W1_AT, W2_AT, W3_AT, W4_AT = 0, 2 * C4, 4 * C4, 11 * C4
WROWS = W4_AT + 2 * F4
WO_ROWS = 4 * DH * 8
WO_AT = WROWS - WO_ROWS
BATCH = ((0,), (1, 2, 3, 4, 5), (6, 7, 8, 9, 10), (11, 12), ())

LAG_QK, LAG_PV, LAG_WO = 2, 4, 6
FILL_AT = (14, 18)

bf16 = jnp.bfloat16
f32 = jnp.float32
u32 = jnp.uint32

SEM_XP, SEM_X, SEM_WO, SEM_STRIP, SEM_OUT, SEM_W, SEM_W0, NSEM = 0, 8, 10, 11, 12, 13, 16, 20


def _mult(i, n):
    return i if isinstance(i, int) else pl.multiple_of(i, n)


def _ln(x):
    d = x - jnp.mean(x, axis=-1, keepdims=True)
    return d * lax.rsqrt(jnp.mean(d * d, axis=-1, keepdims=True) + EPS)


def _ln_stages(x):
    m = jnp.mean(x, axis=-1, keepdims=True)
    yield m
    d = x - m
    return m, lax.rsqrt(jnp.mean(d * d, axis=-1, keepdims=True) + EPS)


def _gelu_of_double(y):
    c = 0.7978845608028654
    return y + y * jnp.tanh(y * (2 * c + (8 * c * 0.044715) * (y * y)))


def _dot(a, b):
    return jnp.dot(a, b, preferred_element_type=f32)


def _load(ref, *idx, r0=0, n=None):
    n = ref.shape[-2] if n is None else n
    return pltpu.bitcast(
        ref.bitcast(u32)[(*idx, pl.ds(_mult(r0 >> 1, 8), n // 2), slice(None))], bf16)


def _sums_a(a11, a12, a21, a22):
    return [lambda: a12 - a22, lambda: a11 + a12, lambda: a11, lambda: a11 + a22,
            lambda: a22, lambda: a21 + a22, lambda: a21 - a11]


def _sums_b(b11, b12, b21, b22):
    return [lambda: b21 + b22, lambda: b22, lambda: b12 - b22, lambda: b11 + b22,
            lambda: b21 - b11, lambda: b11, lambda: b11 + b12]


def _combine(product, emit):
    c11 = product(0)
    c12 = product(1)
    c11 = c11 - c12
    c22 = product(2)
    emit(0, 1, c12 + c22)
    t = product(3)
    c11 = c11 + t
    c22 = c22 + t
    c21 = product(4)
    emit(0, 0, c11 + c21)
    t = product(5)
    emit(1, 0, c21 + t)
    c22 = c22 - t
    emit(1, 1, c22 + product(6))


def _sums2(sums, x, emit):
    outer = [sums(x[i][j], x[i][2 + j], x[2 + i][j], x[2 + i][2 + j])
             for i in range(2) for j in range(2)]
    for p in range(7):
        for q, v in enumerate(sums(*(o[p]() for o in outer))):
            emit(7 * p + q, v)
        yield


def _spread(tasks, pieces, slots):
    todo = itertools.chain(*tasks)
    calls = itertools.count(1)

    def advance():
        k = next(calls)
        if k > slots:
            return
        for _ in range(pieces * k // slots - pieces * (k - 1) // slots):
            next(todo)
        if k == slots:
            assert next(todo, todo) is todo
    return advance


def _tie(never, words, values):
    regs = [[w[r:r + 8] for r in range(0, w.shape[0], 8)] for w in words]
    per = len(regs[0])
    for n, v in enumerate(values):
        c, r = divmod(len(regs) * per * n // len(values), per)
        regs[c][r] = jnp.where(never, pltpu.bitcast(v, u32), regs[c][r])
    return [jnp.concatenate(w, axis=0) for w in regs] if values else words


def _upper_operands(a11, a12, a22):
    k = a11.shape[0] - a22.shape[0]
    ops = [jnp.concatenate([a12[:k], a12[k:] - a22], axis=0), a11 + a12, a11,
           jnp.concatenate([a11[:k], a11[k:] + a22], axis=0)]
    return [v.astype(bf16) for v in ops]


PLAIN = {40: 0, 36: 1, 12: 2, 8: 3}
OTHER = [n for n in range(49) if n not in PLAIN]
RAW_SLOT = dict(zip(OTHER[2::3], [(k, j) for k in range(4) for j in range(4) if k != j]))
RAW_SLOT.update({n: (k, k) for n, k in PLAIN.items()})


def _kernel(x_hbm, mem0_ref, wq_hbm, wk_hbm, wv_hbm, wo_hbm, w1_hbm, w2_hbm,
            w3_hbm, w4_hbm, out_hbm, hbuf, hstat, sems, zero_ref, *wbufs):
    zero_ref[0] = 0
    raw, spare = wbufs[:4], wbufs[4:]
    wsum = {n: (raw[j], k) for n, (k, j) in RAW_SLOT.items()}
    wsum.update({n: (b,) for n, b in zip((n for n in OTHER if n not in RAW_SLOT), spare)})

    def load_h(rows):
        return jnp.concatenate([hbuf[c, rows, :] for c in range(8)], axis=1)

    def h_stats(r0):
        rows = pl.ds(_mult(r0, 16), 16)
        hv = load_h(rows)
        m1, r1 = yield from _ln_stages(hv)
        yield r1
        m2, r2 = yield from _ln_stages((hv - m1) * r1)
        stats = (m1 + m2 / r1, r1, 0.5 * r1 * r2)
        for k, v in enumerate(stats):
            hstat[k, rows, :] = jnp.broadcast_to(v, (16, 128))
        yield stats[0] + stats[2]

    def strip_copies(batch):
        strips = [(w, at + u * w.shape[1], u)
                  for w, at in ((w1_hbm, W1_AT), (w2_hbm, W2_AT), (w3_hbm, W3_AT), (w4_hbm, W4_AT))
                  for u in range(w.shape[2] // 512)]
        return [pltpu.make_async_copy(
            w.at[:, :, pl.ds(j * (w.shape[2] // 4) + u * 128, 128)],
            raw[j].at[:, pl.ds(at, w.shape[1]), :], sems.at[SEM_STRIP])
            for w, at, u in (strips[n] for n in BATCH[batch]) for j in range(4)]

    def weight_sums(r0):
        x = [[_load(raw[j], k, r0=r0, n=16).astype(f32) for j in range(4)]
             for k in range(4)]

        def emit(n, v):
            if n not in PLAIN:
                ref, *idx = wsum[n]
                ref[(*idx, pl.ds(_mult(r0, 16), 16), slice(None))] = v().astype(bf16)
        yield from _sums2(_sums_b, x, emit)

    def block_a(xb, xn, lo, *bufs):
        w_on, low, wo_s = bufs[0:3], bufs[3:6], bufs[6:13]
        w_hbm = (wq_hbm, wk_hbm, wv_hbm)
        stage = hbuf.reshape(8, S // 8, 8, DH)
        lhs = spare[2:5]
        w_low = [spare[5 + 3 * m:8 + 3 * m] for m in range(3)]

        def x_copy(i):
            return pltpu.make_async_copy(x_hbm.at[pl.ds(2 * i, 2)], xb.at[i & 3],
                                         sems.at[SEM_X + (i & 1)])

        def wo_copies(g):
            return [pltpu.make_async_copy(
                wo_hbm.at[g, duo], raw[duo].at[g, pl.ds(WO_AT, WO_ROWS)], sems.at[SEM_WO])
                for duo in range(2)]

        def chunk_copies(g, m, rows=slice(None), sem=None):
            src = w_hbm[m].bitcast(f32)
            return [pltpu.make_async_copy(
                src.at[half, :, rows, g],
                stage.at[pl.ds(2 * m, 2), rows, pl.ds(4 * half, 4), :],
                sems.at[SEM_W + m if sem is None else sem]) for half in range(2)]

        def start(copies):
            for c in copies:
                c.start()

        def wait(copies):
            for c in copies:
                c.wait()

        def qkv_sums(g, m, duo, d0):
            lower, done = [], []
            for part in range(2):
                for pair in (2 * duo, 2 * duo + 1):
                    b = []
                    for half in range(2):
                        rows = pl.ds(8 * d0 + 4 * half + pair, 16, stride=8)
                        w = pltpu.bitcast(hbuf[2 * m + part, rows, :], u32)
                        b += [pltpu.bitcast(w << 16, f32),
                              pltpu.bitcast(w & jnp.uint32(0xFFFF0000), f32)]
                    sums = [v() for v in _sums_b(*b)]
                    for k in range(4):
                        w_on[m][4 * g + pair, k, pl.ds(_mult(part * C4 + d0, 16), 16), :] = (
                            sums[k].astype(bf16))
                    lower.append(sums[4:])
                    done.append(sums[3])
            for k in range(3):
                for q, v in enumerate(_sums_b(*(b[k] for b in lower))):
                    v = v()
                    rows = pl.ds(_mult((7 * duo + q) * C4 + d0, 16), 16)
                    w_low[m][k][rows, :] = v.astype(bf16)
                done.append(v)
            return done

        def wo_sums(g, pair, e0, n0):
            at = WO_AT + pair % 2 * 16 * DH + 8 * e0 + 8 * n0
            tiles = [[_load(raw[pair // 2], g, r0=at + 8 * DH * i + 32 * j + 64 * r, n=16)
                      .astype(f32) for r in range(2)] for i in range(2) for j in range(2)]
            done = []
            for n in range(2):
                b = [jnp.concatenate([v[8 * n:8 * n + 8] for v in t], axis=0) for t in tiles]
                for k, v in enumerate(_sums_b(*b)):
                    v = v()
                    wo_s[k][n0 + n, 4 * g + pair, pl.ds(e0, 16), :] = v.astype(bf16)
                done.append(v)
            return done

        def prologue(xpb):
            def xp_copy(i):
                segs = pl.ds(8 * i, 8)
                return pltpu.make_async_copy(x_hbm.at[segs, pl.ds(16, 16), :], xpb.at[segs],
                                             sems.at[SEM_XP + i])

            def first_chunk(i):
                return chunk_copies(0, 0, pl.ds(64 * i, 64), SEM_W0 + i)

            start([xp_copy(i) for i in range(NSEG // 8)])
            for i in range(4):
                start(first_chunk(i))
            start(chunk_copies(0, 1))
            start(chunk_copies(0, 2))
            lo[...] = jnp.zeros(lo.shape, f32)
            for duo in range(2):
                raw[duo][3, pl.ds(WO_AT, WO_ROWS), :] = jnp.zeros((WO_ROWS, 128), bf16)

            @pl.loop(0, NSEG // 8)
            def _(i):
                xp_copy(i).wait()
                for j in range(2):
                    ops = []
                    for n in range(2):
                        a = [_ln(_load(xpb, 8 * i + 4 * j + 2 * n + k).astype(f32))
                             for k in range(2)]
                        a1 = jnp.concatenate([a[0][:8], a[1][:8]], axis=0)
                        a2 = jnp.concatenate([a[0][8:], a[1][8:]], axis=0)
                        sums = _sums_a(a1[:, :HD], a1[:, HD:], a2[:, :HD], a2[:, HD:])
                        ops.append([v() for v in sums[4:]])
                    for k in range(3):
                        top, bottom = ops[0][k], ops[1][k]
                        for q, v in enumerate(_sums_a(top[:, :C4], top[:, C4:],
                                                      bottom[:, :C4], bottom[:, C4:])):
                            v = v()
                            for c in range(2):
                                r0 = (2 * q + c) * 4 * NSEG + 32 * i + 16 * j
                                lhs[k][pl.ds(pl.multiple_of(r0, 16), 16), :] = (
                                    v[:, c * 128:(c + 1) * 128].astype(bf16))

            @pl.loop(0, 4)
            def _(i):
                wait(first_chunk(i))
                for duo in range(2):
                    for d0 in range(0, 64, 16):
                        qkv_sums(0, 0, duo, 64 * i + d0)

        pl.run_scoped(prologue, pltpu.VMEM((NSEG, 16, D), bf16))

        def lower_products(g, m):
            m1 = (m + 1) % 3
            never = jnp.full((8, 128), zero_ref[0]) != 0
            g1 = jnp.minimum(g + (1 if m == 2 else 0), 3)
            side = [functools.partial(qkv_sums, g1, m1, duo, d0)
                    for duo in range(2) for d0 in range(0, C4, 16)]
            wait_at = 16
            span = 42 - wait_at
            early = [functools.partial(wo_sums, (g + 3) & 3, pair, e0, n0)
                     for pair in range(4 if m == 2 else 0)
                     for e0 in range(0, DH, 16) for n0 in (0, 2)]

            def product(duo, k, q):
                j = 21 * duo + 7 * k + q
                if j >= wait_at:
                    todo = side[len(side) * (j - wait_at) // span:
                                len(side) * (j - wait_at + 1) // span]
                else:
                    todo = early[len(early) * j // wait_at:len(early) * (j + 1) // wait_at]
                a = [lhs[k].bitcast(u32)[pl.ds((2 * q + c) * 2 * NSEG, 2 * NSEG), :]
                     for c in range(2)]
                a[1:] = _tie(never, a[1:], [v[8:] for fn in todo for v in fn()])
                a = jnp.concatenate([pltpu.bitcast(v, bf16) for v in a], axis=1)
                res = _dot(a, _load(w_low[m][k], r0=(7 * duo + q) * C4, n=C4))
                if j == wait_at - 1:
                    pl.when(3 * g + m < 11)(lambda: wait(chunk_copies(g1, m1)))
                    pl.when(g < 3)(lambda: start(chunk_copies(g + 1, m)))
                    if m == 1:
                        pl.when(g > 0)(lambda: wait(wo_copies(g - 1)))
                        start(wo_copies(g))
                        pl.when(g == 3)(
                            lambda: start([x_copy(0), x_copy(1)] + strip_copies(0)))
                return res

            for duo in range(2):
                last = {}
                for k in range(3):
                    def emit(a, b, res):
                        v = res if k == 0 else res + last[a, b] if k == 1 else res - last[a, b]
                        last[a, b] = res
                        for n in range(NSEG // 4):
                            low[m][2 * n + a, 4 * g + 2 * duo + b, k] = (
                                v[16 * n:16 * n + 16].astype(bf16))
                    _combine(functools.partial(product, duo, k), emit)

        @pl.loop(0, 4)
        def _(g):
            for m in range(3):
                lower_products(g, m)

        def norm_tokens(i, k):
            for r0 in range(0, SEG, 16):
                v = _load(xb, jnp.minimum(i, NSEG // 2 - 1) & 3, k, r0=r0, n=16).astype(f32)
                m, r = yield from _ln_stages(v)
                xn[k, pl.ds(r0, 16), :] = (v - m) * r
                yield r

        def lower_wo(grp, n, k):
            w = jnp.concatenate([_load(wo_s[4 + k], n, t) for t in range(NP)], axis=0)
            return _dot(lo[grp & 1, k].astype(bf16), w)

        def add_lower(grp, n, m4, m2, m6):
            for j in range(4):
                seg = slice(8 * j, 8 * j + 8)
                upper = pl.ds(_mult((4 * grp + j) * SEG + 16, 8), 8)
                lower = pl.ds(_mult((4 * grp + j) * SEG + 24, 8), 8)
                hbuf[n, upper, :] += m4[seg]
                hbuf[n, lower, :] += m2[seg] + m4[seg]
                hbuf[4 + n, lower, :] += m6[seg] - m2[seg]

        def attention_mask():
            def split(axis):
                r = lax.broadcasted_iota(jnp.int32, (80, 80), axis)
                return (jnp.where(r < 64, r >> 5, (r - 64) >> 3),
                        jnp.where(r < 64, r & 31, 32 + (r & 7)))
            (hq, pq), (hk, pk) = split(0), split(1)
            visible = (pq < MEM) | (pq >= pk)
            return jnp.where(hq == hk, jnp.where(visible, 0.0, NEG * DH ** 0.5), -jnp.inf)

        def step(i, k, mem, fill, side):
            tok = xn[k]
            r0 = jnp.maximum(2 * i + k - 8, 0) * SEG
            norms = itertools.chain(h_stats(r0), h_stats(r0 + 16), norm_tokens(i + 1, k))
            s = 2 * i + k
            a1 = jnp.concatenate([mem, tok[:24]], axis=0)
            ops = _upper_operands(a1[:, :HD], a1[:, HD:], tok[24:, HD:])
            qkvs, scores, outs, lower = {}, {}, {}, []
            total = [None] * 4

            def qkv(t):
                res = []
                for m in range(3):
                    m7, m5, m3, m1 = [_dot(ops[j], _load(w_on[m], t, j)) for j in range(4)]
                    m4, c21, m62 = [
                        _load(low[m], i, t, j).astype(f32)[8 * k:8 * k + 8]
                        for j in range(3)]
                    side()
                    c11 = m7 - m5 + m1
                    res.append(jnp.concatenate(
                        [c11[:24], c11[24:] + m4, m5 + m3, c21, m3[24:] + m62 + m1[24:]],
                        axis=0).astype(bf16))
                qkvs[t] = res

            def qk(t):
                q, kk, v = qkvs.pop(t)
                sc = lax.dot_general(q, kk, (((1,), (1,)), ((), ())),
                                     preferred_element_type=f32)
                scores[t] = (sc, v)

            def pv(t):
                sc, v = scores.pop(t)
                sc = jnp.where(fill == 0.0, sc, fill)
                tie = next(norms, None) if t >= 1 else None
                if tie is not None:
                    sc = jnp.concatenate([jnp.where(never, tie, sc[:16]), sc[16:]], axis=0)
                mx = jnp.max(sc, axis=1, keepdims=True)
                e = jnp.exp2((sc - mx) * (DH ** -0.5 * LOG2E))
                den = jnp.sum(e, axis=1, keepdims=True)
                inv = pl.reciprocal(den, approx=True)
                inv = inv * (2.0 - den * inv)
                outs[t] = _dot(e.astype(bf16), v) * inv

            def wo(t):
                o = outs.pop(t)
                a11, a12, a21, a22 = o[:32], o[32:64], o[64:72], o[72:]
                rows = pl.ds(pl.multiple_of(8 * (s & 3), 8), 8)
                for j, v in enumerate((a22, a21 + a22, a21 - a11[24:])):
                    lo[(s >> 2) & 1, j, rows, pl.ds(t * DH, DH)] = v
                for j, a in enumerate(_upper_operands(a11, a12, a22)):
                    r = _dot(a, jnp.concatenate(
                        [_load(wo_s[j], n, t) for n in range(4)], axis=1))
                    total[j] = r if total[j] is None else total[j] + r

            for t in range(NP + LAG_WO):
                if t < NP:
                    qkv(t)
                if t in FILL_AT:
                    lower.append(lower_wo((s >> 2) - 1, s & 3, len(lower)))
                if t % 2:
                    for fn, lag in ((qk, LAG_QK), (pv, LAG_PV)):
                        for u in (t - 1 - lag, t - lag):
                            if 0 <= u < NP:
                                fn(u)
                if t >= LAG_WO:
                    wo(t - LAG_WO)

            m7, m5, m3, m1 = total
            upper = jnp.concatenate([m7 - m5 + m1, m5 + m3], axis=1)
            c22 = m3[24:] + m1[24:]
            xv = _load(xb, i & 3, k).astype(f32)
            hv = jnp.concatenate(
                [xv[:24] + upper[MEM:],
                 jnp.concatenate([xv[24:, :HD], xv[24:, HD:] + c22], axis=1)], axis=0)
            for c in range(8):
                hbuf[c, pl.ds(pl.multiple_of(s * SEG, SEG), SEG), :] = hv[:, c * 128:(c + 1) * 128]
            add_lower(jnp.maximum((s >> 2) - 1, 0), s & 3,
                      *lower, lower_wo((s >> 2) - 1, s & 3, 2))
            return upper[:MEM]

        fill = attention_mask()
        never = jnp.full((16, 80), zero_ref[0]) != 0
        n_it = NSEG // 2
        per_it = WROWS // 16 // n_it

        def steps(i, mem):
            pl.when(i + 1 < n_it)(lambda: x_copy(i + 1).wait())
            pl.when(i + 2 < n_it)(lambda: x_copy(i + 2).start())

            @pl.when(i < len(BATCH) - 1)
            def _():
                for b in range(len(BATCH) - 1):
                    @pl.when(i == b)
                    def _():
                        wait(strip_copies(b))
                        start(strip_copies(b + 1))

            side = _spread([weight_sums(16 * (per_it * i + j)) for j in range(per_it)],
                           7 * per_it, 90)
            for k in range(2):
                mem = step(i, k, mem, fill, side)
            return mem

        wait(wo_copies(3) + [x_copy(0)])
        for pair in range(4):
            for e0 in range(0, DH, 16):
                for n0 in (0, 2):
                    wo_sums(3, pair, e0, n0)
        hbuf[:, pl.ds(0, 4 * SEG), :] = jnp.zeros((8, 4 * SEG, 128), f32)
        _spread([norm_tokens(0, 0), norm_tokens(0, 1)], 8, 1)()
        lax.fori_loop(0, n_it, steps, mem0_ref[...].astype(f32))
        for n in range(4):
            add_lower(NSEG // 4 - 1, n, *(lower_wo(NSEG // 4 - 1, n, k) for k in range(3)))

    pl.run_scoped(
        block_a,
        pltpu.VMEM((4, 2, SEG, D), bf16),
        pltpu.VMEM((2, SEG, D), f32),
        pltpu.VMEM((2, 3, 32, NP * DH), f32),
        *[pltpu.VMEM((NP, 4, HD, DH), bf16)] * 3,
        *[pltpu.VMEM((NSEG // 2, NP, 3, 16, DH), bf16)] * 3,
        *[pltpu.VMEM((4, NP, DH, 128), bf16)] * 7,
    )

    def block_b(gbuf, ustat, x1, obuf, yc, hc, db, nb0, nb1, ac0, ac1, pb0, pb1):
        def weights(n, at, rows, strips):
            return jnp.concatenate(
                [_load(*wsum[n], r0=at + k * rows[0] + rows[1], n=rows[2])
                 for k in strips], axis=1)

        ties = []
        never = jnp.full((8, 128), zero_ref[0]) != 0

        def before_next(value):
            if value.shape[1] == 1:
                value = jnp.broadcast_to(value[:8] + value[8:], (8, 128))
            ties.append(value[-8:, -128:])

        def operand(ref, n, cols):
            words = [ref.bitcast(u32)[n, c] for c in cols]
            words = _tie(never, words, ties)
            ties.clear()
            return jnp.concatenate([pltpu.bitcast(w, bf16) for w in words], axis=1)

        def store_sums(dst, r, c, x, tie=True):
            def emit(n, v):
                v = v()
                dst[n, c, pl.ds(16 * r, 16), :] = v.astype(bf16)
                if tie and n % 2:
                    before_next(v)
            return _sums2(_sums_a, x, emit)

        def inner(dst, p, product, side, add=False):
            def emit(a, b, v):
                dst[p, 2 * a + b] = dst[p, 2 * a + b] + v if add else v

            def run(k):
                r = product(7 * p + k)
                side()
                return r
            _combine(run, emit)

        def outer(src, r, cols, emit):
            for a in range(2):
                for b in range(2):
                    _combine(lambda p: src[p, 2 * a + b, pl.ds(16 * r, 16), cols],
                             lambda i, j, v: emit(2 * i + a, 2 * j + b, v))
                    yield

        def rows_of(i, g, r):
            return pl.ds(_mult(i * RB + g * R + 16 * r, 16), 16)

        def tied(stages):
            while True:
                try:
                    before_next(next(stages))
                except StopIteration as stop:
                    return stop.value
                yield
                yield

        def last_stats(i, r):
            return tied(h_stats(S - RB + i * R + 16 * r))

        def pre1(i, dst, r):
            for c in range(2):
                x = []
                for g in range(4):
                    rows = rows_of(i, g, r)
                    x.append([(hbuf[2 * k + c, rows, :] - hstat[0, rows, :]) * hstat[2, rows, :]
                              for k in range(4)])
                yield from range(3)
                yield from store_sums(dst, r, c, x)

        def post1(i, src, r):
            def emit(g, j, v):
                v = _gelu_of_double(v)
                gbuf[2 * j + c, pl.ds(HALO + i * RB + g * R + 16 * r, 16), :] = v
            for c in range(2):
                for _ in outer(src, r, pl.ds(c * 128, 128), emit):
                    yield
                    yield

        def pre2(i, dst, r):
            for c in range(2):
                x = [[gbuf[2 * k + c, pl.ds(HALO + i * RB + g * R + 16 * r + off, 16), :]
                      for k, off in enumerate((-1, 1, -2, 2))] for g in range(4)]
                yield from store_sums(dst, r, c, x)

        def post2(i, src, r):
            def emit(g, j, v):
                rows = rows_of(i, g, r)
                v = v + jnp.concatenate(
                    [(hbuf[c, rows, :] - hstat[0, rows, :]) * hstat[1, rows, :]
                     for c in (2 * j, 2 * j + 1)], axis=1)
                x1[rows, pl.ds(j * C4, C4)] = v
            for _ in outer(src, r, slice(None), emit):
                yield
                yield

        def pre3(i, r):
            for g in range(4):
                rows = rows_of(i, g, r)
                m, rs = yield from tied(_ln_stages(x1[rows, :]))
                ustat[0, rows_of(0, g, r), :] = jnp.broadcast_to(m, (16, 128))
                ustat[1, rows_of(0, g, r), :] = jnp.broadcast_to(0.5 * rs, (16, 128))
                before_next(rs)
                yield
                yield

        def sums3(i, tie, r):
            for c in range(2):
                x = [[(x1[rows_of(i, g, r), pl.ds(k * C4 + c * 128, 128)]
                       - ustat[0, rows_of(0, g, r), :]) * ustat[1, rows_of(0, g, r), :]
                      for k in range(4)] for g in range(4)]
                yield from store_sums(yc, r, c, x, tie)

        pieces = {pre1: 20, last_stats: 8, post1: 16, pre2: 14, post2: 8, pre3: 16, sums3: 14}

        def spread(stages, slots):
            return _spread([fn(*args, r) for fn, *args in stages for r in range(R // 16)],
                           sum(pieces[fn] for fn, *_ in stages) * (R // 16), slots)

        for c in range(8):
            gbuf[c, pl.ds(0, HALO), :] = jnp.zeros((HALO, 128), f32)
            gbuf[c, pl.ds(HALO + S, HALO), :] = jnp.zeros((HALO, 128), f32)
        first, second = (W1_AT, pre1, post1), (W2_AT, pre2, post2)
        order = [(stage, i - lag) for i in range(NB + 2)
                 for stage, lag in ((first, 0), (second, 2)) if 0 <= i - lag < NB]
        extra = {n: [(last_stats, i)] for i, n in enumerate((0, 4, 6, 8))}
        extra.update({10: [(pre3, 0)], 15: [(sums3, 0, True)]})
        ac, pb = (ac0, ac1), (pb0, pb1)
        spread([(pre1, 0, ac0)], 1)()
        ties.clear()
        for n, ((at, _, _), _) in enumerate(order):
            before = [(post, i, pb[1 - n % 2]) for (_, _, post), i in order[max(n - 1, 0):n]]
            after = [(pre, i, ac[1 - n % 2]) for (_, pre, _), i in order[n + 1:n + 2]]
            stages = before + after if n in (2, 13) else after + before
            side = spread(stages + extra.get(n, []), 47)
            for p in range(7):
                inner(pb[n % 2], p, lambda k: _dot(
                    operand(ac[n % 2], k, (0, 1)), weights(k, at, (C4, 0, C4), (0, 1))), side)
        spread([(post2, NB - 1, pb1)], 1)()

        def out_copy(i):
            rows = pl.ds(_mult(i * RB, RB), RB)
            return pltpu.make_async_copy(obuf.at[rows], out_hbm.at[rows], sems.at[SEM_OUT])

        nb = (nb0, nb1)

        def activate(c, r):
            act = [[None] * 4 for _ in range(4)]

            def emit(g, j, v):
                act[g][j] = _gelu_of_double(v)
            for _ in outer(nb[c % 2], r, slice(None), emit):
                yield
                yield
            yield from store_sums(hc, r, c, act, False)

        pieces[activate] = 15

        def mlp_up():
            for c in range(7):
                side = spread([(activate, c - 1)] if c else [], 49)
                for p in range(7):
                    inner(nb[c % 2], p, lambda n: _dot(
                        operand(yc, n, (0, 1)), weights(n, W3_AT, (C4, 0, C4), (c,))), side)

        def mlp_down(i, stages):
            def down(p, side, k0=0, k1=F4):
                inner(db, p, lambda n: _dot(operand(hc, n, range(k0 // 128, k1 // 128)),
                                            weights(n, W4_AT, (F4, k0, k1 - k0), (0, 1))),
                      side, add=k0 > 0)

            def finish(bi, bj, plus, minus=()):
                for a in range(2):
                    for b in range(2):
                        rows = pl.ds(_mult(i * RB + (2 * bi + a) * R, R), R)
                        cols = pl.ds((2 * bj + b) * C4, C4)
                        v = x1[rows, cols] + jnp.concatenate(
                            [hbuf[4 * bj + 2 * b + c, rows, :] for c in range(2)], axis=1)
                        for p in minus:
                            v = v - db[p, 2 * a + b]
                        for p in plus:
                            v = v + db[p, 2 * a + b]
                        obuf[rows, cols] = v.astype(bf16)

            down(0, spread([(activate, 6)], 6), 0, F4 - 128)
            down(0, lambda: None, F4 - 128)
            side = spread(stages, 35)
            for p in range(1, 7):
                down(p, side)
                if p == 3:
                    finish(0, 1, (1, 2))
                if p == 5:
                    finish(0, 0, (0, 3, 4), (1,))
            finish(1, 0, (4, 5))
            finish(1, 1, (2, 3, 6), (5,))

        @pl.loop(0, NB)
        def _(i):
            ties.clear()
            mlp_up()
            nxt = jnp.minimum(i + 1, NB - 1)
            mlp_down(i, [(pre3, nxt), (sums3, nxt, False)])
            out_copy(i).start()

        for i in range(NB):
            out_copy(i).wait()

    pl.run_scoped(
        block_b,
        pltpu.VMEM((8, S + 2 * HALO, 128), f32),
        pltpu.VMEM((2, RB, 128), f32),
        pltpu.VMEM((S, D), f32),
        pltpu.VMEM((S, D), bf16),
        pltpu.VMEM((49, 2, R, 128), bf16),
        pltpu.VMEM((49, 7, R, 128), bf16),
        pltpu.VMEM((7, 4, R, C4), f32),
        *[pltpu.VMEM((7, 4, R, 128), f32)] * 2,
        *[pltpu.VMEM((49, 2, R, 128), bf16)] * 2,
        *[pltpu.VMEM((7, 4, R, C4), f32)] * 2,
    )


@jax.jit
def pallas_sequential_preLN__memory_aug_recurrent_mem_tr__mixer_s_mlp__prompt_kernel(
    A_x: jax.Array,
    A_mem0: jax.Array,
    A_Wq: jax.Array,
    A_Wk: jax.Array,
    A_Wv: jax.Array,
    A_Wo: jax.Array,
    A_seg_len: jax.Array,
    B_x: jax.Array,
    B_w1: jax.Array,
    B_w2: jax.Array,
    B_w3: jax.Array,
    B_w4: jax.Array,
):
    del A_seg_len, B_x
    hbm = pl.BlockSpec(memory_space=pl.ANY)
    vmem = pl.BlockSpec(memory_space=pltpu.VMEM)
    scratch = [
        pltpu.VMEM((8, S, 128), f32),
        pltpu.VMEM((3, S, 128), f32),
        pltpu.SemaphoreType.DMA((NSEM,)),
        pltpu.SMEM((1,), jnp.int32),
    ] + [pltpu.VMEM((4, WROWS, 128), bf16)] * 4 + [pltpu.VMEM((WROWS, 128), bf16)] * 33
    out = pl.pallas_call(
        _kernel,
        out_shape=jax.ShapeDtypeStruct((S, D), A_x.dtype),
        in_specs=[hbm, vmem] + [hbm] * 8,
        out_specs=hbm,
        scratch_shapes=scratch,
        compiler_params=pltpu.CompilerParams(vmem_limit_bytes=128 * 1024 * 1024),
    )(A_x.reshape(NSEG, SEG, D), A_mem0.reshape(MEM, D),
      A_Wq.reshape(2, 2, C4, 4, 8, DH), A_Wk.reshape(2, 2, C4, 4, 8, DH),
      A_Wv.reshape(2, 2, C4, 4, 8, DH),
      A_Wo.reshape(H * DH // 8, 8, 8, 128).transpose(0, 2, 1, 3).reshape(4, 2, WO_ROWS, 128),
      B_w1.reshape(4, C4, D), B_w2.reshape(4, C4, D),
      B_w3.reshape(4, C4, F), B_w4.reshape(4, F4, D))
    return out.reshape(A_x.shape)
```

```python
import functools
import itertools

import jax
import jax.numpy as jnp
from jax import lax
import jax.experimental.pallas as pl
import jax.experimental.pallas.tpu as pltpu

S = 2048
D = 1024
H = 32
DH = 128
MEM = 8
SEG = 32
F = 3584
NSEG = S // SEG
NP = H // 2
HD = D // 2
C4 = D // 4
F4 = F // 4
HALO = 8
R = 64
RB = 4 * R
NB = S // RB
EPS = 1e-5
NEG = -1000000000.0
LOG2E = 1.4426950408889634

W1_AT, W2_AT, W3_AT, W4_AT = 0, 2 * C4, 4 * C4, 11 * C4
WROWS = W4_AT + 2 * F4
WO_ROWS = 4 * DH * 8
WO_AT = WROWS - WO_ROWS
BATCH = ((0,), (1, 2, 3, 4, 5), (6, 7, 8, 9, 10), (11, 12), ())

LAG_QK, LAG_PV, LAG_WO = 2, 4, 6
FILL_AT = (14, 18)

bf16 = jnp.bfloat16
f32 = jnp.float32
u32 = jnp.uint32

SEM_XP, SEM_X, SEM_WO, SEM_STRIP, SEM_OUT, SEM_W, SEM_W0, NSEM = 0, 8, 10, 11, 12, 13, 16, 20


def _mult(i, n):
    return i if isinstance(i, int) else pl.multiple_of(i, n)


def _ln(x):
    d = x - jnp.mean(x, axis=-1, keepdims=True)
    return d * lax.rsqrt(jnp.mean(d * d, axis=-1, keepdims=True) + EPS)


def _ln_stages(x):
    m = jnp.mean(x, axis=-1, keepdims=True)
    yield m
    d = x - m
    return m, lax.rsqrt(jnp.mean(d * d, axis=-1, keepdims=True) + EPS)


def _gelu_of_double(y):
    c = 0.7978845608028654
    return y + y * jnp.tanh(y * (2 * c + (8 * c * 0.044715) * (y * y)))


def _dot(a, b):
    return jnp.dot(a, b, preferred_element_type=f32)


def _load(ref, *idx, r0=0, n=None):
    n = ref.shape[-2] if n is None else n
    return pltpu.bitcast(
        ref.bitcast(u32)[(*idx, pl.ds(r0 // 2, n // 2), slice(None))], bf16)


def _sums_a(a11, a12, a21, a22):
    return [lambda: a12 - a22, lambda: a11 + a12, lambda: a11, lambda: a11 + a22,
            lambda: a22, lambda: a21 + a22, lambda: a21 - a11]


def _sums_b(b11, b12, b21, b22):
    return [lambda: b21 + b22, lambda: b22, lambda: b12 - b22, lambda: b11 + b22,
            lambda: b21 - b11, lambda: b11, lambda: b11 + b12]


def _combine(product, emit):
    c11 = product(0)
    c12 = product(1)
    c11 = c11 - c12
    c22 = product(2)
    emit(0, 1, c12 + c22)
    t = product(3)
    c11 = c11 + t
    c22 = c22 + t
    c21 = product(4)
    emit(0, 0, c11 + c21)
    t = product(5)
    emit(1, 0, c21 + t)
    c22 = c22 - t
    emit(1, 1, c22 + product(6))


def _sums2(sums, x, emit):
    outer = [sums(x[i][j], x[i][2 + j], x[2 + i][j], x[2 + i][2 + j])
             for i in range(2) for j in range(2)]
    for p in range(7):
        for q, v in enumerate(sums(*(o[p]() for o in outer))):
            emit(7 * p + q, v)
        yield


def _spread(tasks, pieces, slots):
    todo = itertools.chain(*tasks)
    calls = itertools.count(1)

    def advance():
        k = next(calls)
        if k > slots:
            return
        for _ in range(pieces * k // slots - pieces * (k - 1) // slots):
            next(todo)
        if k == slots:
            assert next(todo, todo) is todo
    return advance


def _tie(never, words, values):
    regs = [[w[r:r + 8] for r in range(0, w.shape[0], 8)] for w in words]
    per = len(regs[0])
    for n, v in enumerate(values):
        c, r = divmod(len(regs) * per * n // len(values), per)
        regs[c][r] = jnp.where(never, pltpu.bitcast(v, u32), regs[c][r])
    return [jnp.concatenate(w, axis=0) for w in regs] if values else words


def _upper_operands(a11, a12, a22):
    k = a11.shape[0] - a22.shape[0]
    ops = [jnp.concatenate([a12[:k], a12[k:] - a22], axis=0), a11 + a12, a11,
           jnp.concatenate([a11[:k], a11[k:] + a22], axis=0)]
    return [v.astype(bf16) for v in ops]


PLAIN = {40: 0, 36: 1, 12: 2, 8: 3}
OTHER = [n for n in range(49) if n not in PLAIN]
RAW_SLOT = dict(zip(OTHER[2::3], [(k, j) for k in range(4) for j in range(4) if k != j]))
RAW_SLOT.update({n: (k, k) for n, k in PLAIN.items()})


def _kernel(x_hbm, mem0_ref, wq_hbm, wk_hbm, wv_hbm, wo_hbm, w1_hbm, w2_hbm,
            w3_hbm, w4_hbm, out_hbm, hbuf, hstat, sems, zero_ref, *wbufs):
    zero_ref[0] = 0
    raw, spare = wbufs[:4], wbufs[4:]
    wsum = {n: (raw[j], k) for n, (k, j) in RAW_SLOT.items()}
    wsum.update({n: (b,) for n, b in zip((n for n in OTHER if n not in RAW_SLOT), spare)})

    def load_h(rows):
        return jnp.concatenate([hbuf[c, rows, :] for c in range(8)], axis=1)

    def h_stats(r0):
        rows = pl.ds(_mult(r0, 16), 16)
        hv = load_h(rows)
        m1, r1 = yield from _ln_stages(hv)
        yield r1
        m2, r2 = yield from _ln_stages((hv - m1) * r1)
        stats = (m1 + m2 / r1, r1, 0.5 * r1 * r2)
        for k, v in enumerate(stats):
            hstat[k, rows, :] = jnp.broadcast_to(v, (16, 128))
        yield stats[0] + stats[2]

    def strip_copies(batch):
        strips = [(w, at + u * w.shape[1], u)
                  for w, at in ((w1_hbm, W1_AT), (w2_hbm, W2_AT), (w3_hbm, W3_AT), (w4_hbm, W4_AT))
                  for u in range(w.shape[2] // 512)]
        return [pltpu.make_async_copy(
            w.at[:, :, pl.ds(j * (w.shape[2] // 4) + u * 128, 128)],
            raw[j].at[:, pl.ds(at, w.shape[1]), :], sems.at[SEM_STRIP])
            for w, at, u in (strips[n] for n in BATCH[batch]) for j in range(4)]

    def weight_sums(r0):
        x = [[raw[j][k, pl.ds(_mult(r0, 16), 16), :].astype(f32) for j in range(4)]
             for k in range(4)]

        def emit(n, v):
            if n not in PLAIN:
                ref, *idx = wsum[n]
                ref[(*idx, pl.ds(_mult(r0, 16), 16), slice(None))] = v().astype(bf16)
        yield from _sums2(_sums_b, x, emit)

    def block_a(xb, xn, lo, *bufs):
        w_on, low, wo_s = bufs[0:3], bufs[3:6], bufs[6:13]
        w_hbm = (wq_hbm, wk_hbm, wv_hbm)
        stage = hbuf.reshape(8, S // 8, 8, DH)
        lhs = spare[:3]
        w_low = [spare[3 + 3 * m:6 + 3 * m] for m in range(3)]

        def x_copy(i):
            return pltpu.make_async_copy(x_hbm.at[pl.ds(2 * i, 2)], xb.at[i & 3],
                                         sems.at[SEM_X + (i & 1)])

        def wo_copies(g):
            return [pltpu.make_async_copy(
                wo_hbm.at[g, duo], raw[duo].at[g, pl.ds(WO_AT, WO_ROWS)], sems.at[SEM_WO])
                for duo in range(2)]

        def chunk_copies(g, m, rows=slice(None), sem=None):
            src = w_hbm[m].bitcast(f32)
            return [pltpu.make_async_copy(
                src.at[half, :, rows, g],
                stage.at[pl.ds(2 * m, 2), rows, pl.ds(4 * half, 4), :],
                sems.at[SEM_W + m if sem is None else sem]) for half in range(2)]

        def start(copies):
            for c in copies:
                c.start()

        def wait(copies):
            for c in copies:
                c.wait()

        def qkv_sums(g, m, duo, d0):
            lower, done = [], []
            for part in range(2):
                for pair in (2 * duo, 2 * duo + 1):
                    b = []
                    for half in range(2):
                        rows = pl.ds(8 * d0 + 4 * half + pair, 16, stride=8)
                        w = pltpu.bitcast(hbuf[2 * m + part, rows, :], u32)
                        b += [pltpu.bitcast(w << 16, f32),
                              pltpu.bitcast(w & jnp.uint32(0xFFFF0000), f32)]
                    sums = [v() for v in _sums_b(*b)]
                    for k in range(4):
                        w_on[m][4 * g + pair, k, pl.ds(_mult(part * C4 + d0, 16), 16), :] = (
                            sums[k].astype(bf16))
                    lower.append(sums[4:])
                    done.append(sums[3])
            for k in range(3):
                for q, v in enumerate(_sums_b(*(b[k] for b in lower))):
                    v = v()
                    rows = pl.ds(_mult((7 * duo + q) * C4 + d0, 16), 16)
                    w_low[m][k][rows, :] = v.astype(bf16)
                done.append(v)
            return done

        def wo_sums(g, pair, e0, n0):
            at = WO_AT + pair % 2 * 16 * DH + 8 * e0 + 8 * n0
            tiles = [[raw[pair // 2][g, pl.ds(at + 8 * DH * i + 32 * j + 64 * r, 16), :]
                      .astype(f32) for r in range(2)] for i in range(2) for j in range(2)]
            done = []
            for n in range(2):
                b = [jnp.concatenate([v[8 * n:8 * n + 8] for v in t], axis=0) for t in tiles]
                for k, v in enumerate(_sums_b(*b)):
                    v = v()
                    wo_s[k][n0 + n, 4 * g + pair, pl.ds(e0, 16), :] = v.astype(bf16)
                done.append(v)
            return done

        def prologue(xpb):
            def xp_copy(i):
                segs = pl.ds(8 * i, 8)
                return pltpu.make_async_copy(x_hbm.at[segs, pl.ds(16, 16), :], xpb.at[segs],
                                             sems.at[SEM_XP + i])

            def first_chunk(i):
                return chunk_copies(0, 0, pl.ds(64 * i, 64), SEM_W0 + i)

            start([xp_copy(i) for i in range(NSEG // 8)])
            for i in range(4):
                start(first_chunk(i))
            start(chunk_copies(0, 1))
            start(chunk_copies(0, 2))
            lo[...] = jnp.zeros(lo.shape, f32)
            for duo in range(2):
                raw[duo][3, pl.ds(WO_AT, WO_ROWS), :] = jnp.zeros((WO_ROWS, 128), bf16)

            @pl.loop(0, NSEG // 8)
            def _(i):
                xp_copy(i).wait()
                for j in range(2):
                    ops = []
                    for n in range(2):
                        a = [_ln(xpb[8 * i + 4 * j + 2 * n + k].astype(f32))
                             for k in range(2)]
                        a1 = jnp.concatenate([a[0][:8], a[1][:8]], axis=0)
                        a2 = jnp.concatenate([a[0][8:], a[1][8:]], axis=0)
                        sums = _sums_a(a1[:, :HD], a1[:, HD:], a2[:, :HD], a2[:, HD:])
                        ops.append([v() for v in sums[4:]])
                    for k in range(3):
                        top, bottom = ops[0][k], ops[1][k]
                        for q, v in enumerate(_sums_a(top[:, :C4], top[:, C4:],
                                                      bottom[:, :C4], bottom[:, C4:])):
                            v = v()
                            for c in range(2):
                                r0 = (2 * q + c) * 4 * NSEG + 32 * i + 16 * j
                                lhs[k][pl.ds(pl.multiple_of(r0, 16), 16), :] = (
                                    v[:, c * 128:(c + 1) * 128].astype(bf16))

            @pl.loop(0, 4)
            def _(i):
                wait(first_chunk(i))
                for duo in range(2):
                    for d0 in range(0, 64, 16):
                        qkv_sums(0, 0, duo, 64 * i + d0)

        pl.run_scoped(prologue, pltpu.VMEM((NSEG, 16, D), bf16))

        def lower_products(g, m):
            m1 = (m + 1) % 3
            never = jnp.full((8, 128), zero_ref[0]) != 0
            g1 = jnp.minimum(g + (1 if m == 2 else 0), 3)
            side = [functools.partial(qkv_sums, g1, m1, duo, d0)
                    for duo in range(2) for d0 in range(0, C4, 16)]
            wait_at = 16
            span = 42 - wait_at
            early = [functools.partial(wo_sums, (g + 3) & 3, pair, e0, n0)
                     for pair in range(4 if m == 2 else 0)
                     for e0 in range(0, DH, 16) for n0 in (0, 2)]

            def product(duo, k, q):
                j = 21 * duo + 7 * k + q
                if j >= wait_at:
                    todo = side[len(side) * (j - wait_at) // span:
                                len(side) * (j - wait_at + 1) // span]
                else:
                    todo = early[len(early) * j // wait_at:len(early) * (j + 1) // wait_at]
                a = [lhs[k].bitcast(u32)[pl.ds((2 * q + c) * 2 * NSEG, 2 * NSEG), :]
                     for c in range(2)]
                a[1:] = _tie(never, a[1:], [v[8:] for fn in todo for v in fn()])
                a = jnp.concatenate([pltpu.bitcast(v, bf16) for v in a], axis=1)
                res = _dot(a, _load(w_low[m][k], r0=(7 * duo + q) * C4, n=C4))
                if j == wait_at - 1:
                    pl.when(3 * g + m < 11)(lambda: wait(chunk_copies(g1, m1)))
                    pl.when(g < 3)(lambda: start(chunk_copies(g + 1, m)))
                    if m == 1:
                        pl.when(g > 0)(lambda: wait(wo_copies(g - 1)))
                        start(wo_copies(g))
                        pl.when(g == 3)(
                            lambda: start([x_copy(0), x_copy(1)] + strip_copies(0)))
                return res

            for duo in range(2):
                last = {}
                for k in range(3):
                    def emit(a, b, res):
                        v = res if k == 0 else res + last[a, b] if k == 1 else res - last[a, b]
                        last[a, b] = res
                        for n in range(NSEG // 4):
                            low[m][2 * n + a, 4 * g + 2 * duo + b, k] = (
                                v[16 * n:16 * n + 16].astype(bf16))
                    _combine(functools.partial(product, duo, k), emit)

        @pl.loop(0, 4)
        def _(g):
            for m in range(3):
                lower_products(g, m)

        def norm_tokens(i, k):
            for r0 in range(0, SEG, 16):
                v = xb[jnp.minimum(i, NSEG // 2 - 1) & 3, k, pl.ds(r0, 16), :].astype(f32)
                m, r = yield from _ln_stages(v)
                xn[k, pl.ds(r0, 16), :] = (v - m) * r
                yield r

        def lower_wo(grp, n, k):
            w = jnp.concatenate([_load(wo_s[4 + k], n, t) for t in range(NP)], axis=0)
            return _dot(lo[grp & 1, k].astype(bf16), w)

        def add_lower(grp, n, m4, m2, m6):
            for j in range(4):
                seg = slice(8 * j, 8 * j + 8)
                upper = pl.ds(_mult((4 * grp + j) * SEG + 16, 8), 8)
                lower = pl.ds(_mult((4 * grp + j) * SEG + 24, 8), 8)
                hbuf[n, upper, :] += m4[seg]
                hbuf[n, lower, :] += m2[seg] + m4[seg]
                hbuf[4 + n, lower, :] += m6[seg] - m2[seg]

        def attention_mask():
            def split(axis):
                r = lax.broadcasted_iota(jnp.int32, (80, 80), axis)
                return (jnp.where(r < 64, r >> 5, (r - 64) >> 3),
                        jnp.where(r < 64, r & 31, 32 + (r & 7)))
            (hq, pq), (hk, pk) = split(0), split(1)
            visible = (pq < MEM) | (pq >= pk)
            return jnp.where(hq == hk, jnp.where(visible, 0.0, NEG * DH ** 0.5), -jnp.inf)

        def step(i, k, mem, fill, side):
            tok = xn[k]
            r0 = jnp.maximum(2 * i + k - 8, 0) * SEG
            norms = itertools.chain(h_stats(r0), h_stats(r0 + 16), norm_tokens(i + 1, k))
            s = 2 * i + k
            a1 = jnp.concatenate([mem, tok[:24]], axis=0)
            ops = _upper_operands(a1[:, :HD], a1[:, HD:], tok[24:, HD:])
            qkvs, scores, outs, lower = {}, {}, {}, []
            total = [None] * 4

            def qkv(t):
                res = []
                for m in range(3):
                    m7, m5, m3, m1 = [_dot(ops[j], _load(w_on[m], t, j)) for j in range(4)]
                    m4, c21, m62 = [
                        _load(low[m], i, t, j).astype(f32)[8 * k:8 * k + 8]
                        for j in range(3)]
                    side()
                    c11 = m7 - m5 + m1
                    res.append(jnp.concatenate(
                        [c11[:24], c11[24:] + m4, m5 + m3, c21, m3[24:] + m62 + m1[24:]],
                        axis=0).astype(bf16))
                qkvs[t] = res

            def qk(t):
                q, kk, v = qkvs.pop(t)
                sc = lax.dot_general(q, kk, (((1,), (1,)), ((), ())),
                                     preferred_element_type=f32)
                scores[t] = (sc, v)

            def pv(t):
                sc, v = scores.pop(t)
                sc = jnp.where(fill == 0.0, sc, fill)
                tie = next(norms, None) if t >= 1 else None
                if tie is not None:
                    sc = jnp.concatenate([jnp.where(never, tie, sc[:16]), sc[16:]], axis=0)
                mx = jnp.max(sc, axis=1, keepdims=True)
                e = jnp.exp2((sc - mx) * (DH ** -0.5 * LOG2E))
                den = jnp.sum(e, axis=1, keepdims=True)
                inv = pl.reciprocal(den, approx=True)
                inv = inv * (2.0 - den * inv)
                outs[t] = _dot(e.astype(bf16), v) * inv

            def wo(t):
                o = outs.pop(t)
                a11, a12, a21, a22 = o[:32], o[32:64], o[64:72], o[72:]
                rows = pl.ds(pl.multiple_of(8 * (s & 3), 8), 8)
                for j, v in enumerate((a22, a21 + a22, a21 - a11[24:])):
                    lo[(s >> 2) & 1, j, rows, pl.ds(t * DH, DH)] = v
                for j, a in enumerate(_upper_operands(a11, a12, a22)):
                    r = _dot(a, jnp.concatenate(
                        [_load(wo_s[j], n, t) for n in range(4)], axis=1))
                    total[j] = r if total[j] is None else total[j] + r

            for t in range(NP + LAG_WO):
                if t < NP:
                    qkv(t)
                if t in FILL_AT:
                    lower.append(lower_wo((s >> 2) - 1, s & 3, len(lower)))
                if t % 2:
                    for fn, lag in ((qk, LAG_QK), (pv, LAG_PV)):
                        for u in (t - 1 - lag, t - lag):
                            if 0 <= u < NP:
                                fn(u)
                if t >= LAG_WO:
                    wo(t - LAG_WO)

            m7, m5, m3, m1 = total
            upper = jnp.concatenate([m7 - m5 + m1, m5 + m3], axis=1)
            c22 = m3[24:] + m1[24:]
            xv = xb[i & 3, k].astype(f32)
            hv = jnp.concatenate(
                [xv[:24] + upper[MEM:],
                 jnp.concatenate([xv[24:, :HD], xv[24:, HD:] + c22], axis=1)], axis=0)
            for c in range(8):
                hbuf[c, pl.ds(pl.multiple_of(s * SEG, SEG), SEG), :] = hv[:, c * 128:(c + 1) * 128]
            add_lower(jnp.maximum((s >> 2) - 1, 0), s & 3,
                      *lower, lower_wo((s >> 2) - 1, s & 3, 2))
            return upper[:MEM]

        fill = attention_mask()
        never = jnp.full((16, 80), zero_ref[0]) != 0
        n_it = NSEG // 2
        per_it = WROWS // 16 // n_it

        def steps(i, mem):
            pl.when(i + 1 < n_it)(lambda: x_copy(i + 1).wait())
            pl.when(i + 2 < n_it)(lambda: x_copy(i + 2).start())

            @pl.when(i < len(BATCH) - 1)
            def _():
                for b in range(len(BATCH) - 1):
                    @pl.when(i == b)
                    def _():
                        wait(strip_copies(b))
                        start(strip_copies(b + 1))

            side = _spread([weight_sums(16 * (per_it * i + j)) for j in range(per_it)],
                           7 * per_it, 94)
            for k in range(2):
                mem = step(i, k, mem, fill, side)
            return mem

        wait(wo_copies(3) + [x_copy(0)])
        for pair in range(4):
            for e0 in range(0, DH, 16):
                for n0 in (0, 2):
                    wo_sums(3, pair, e0, n0)
        hbuf[:, pl.ds(0, 4 * SEG), :] = jnp.zeros((8, 4 * SEG, 128), f32)
        _spread([norm_tokens(0, 0), norm_tokens(0, 1)], 8, 1)()
        lax.fori_loop(0, n_it, steps, mem0_ref[...].astype(f32))
        for n in range(4):
            add_lower(NSEG // 4 - 1, n, *(lower_wo(NSEG // 4 - 1, n, k) for k in range(3)))

    pl.run_scoped(
        block_a,
        pltpu.VMEM((4, 2, SEG, D), bf16),
        pltpu.VMEM((2, SEG, D), f32),
        pltpu.VMEM((2, 3, 32, NP * DH), f32),
        *[pltpu.VMEM((NP, 4, HD, DH), bf16)] * 3,
        *[pltpu.VMEM((NSEG // 2, NP, 3, 16, DH), bf16)] * 3,
        *[pltpu.VMEM((4, NP, DH, 128), bf16)] * 7,
    )

    def block_b(gbuf, ustat, x1, obuf, yc, hc, db, nb0, nb1, ac0, ac1, pb0, pb1):
        def weights(n, at, rows, strips):
            return jnp.concatenate(
                [_load(*wsum[n], r0=at + k * rows[0] + rows[1], n=rows[2])
                 for k in strips], axis=1)

        ties = []
        never = jnp.full((8, 128), zero_ref[0]) != 0

        def before_next(value):
            if value.shape[1] == 1:
                value = jnp.broadcast_to(value[:8] + value[8:], (8, 128))
            ties.append(value[-8:, -128:])

        def operand(ref, n, cols):
            words = [ref.bitcast(u32)[n, c] for c in cols]
            words = _tie(never, words, ties)
            ties.clear()
            return jnp.concatenate([pltpu.bitcast(w, bf16) for w in words], axis=1)

        def store_sums(dst, r, c, x, tie=True):
            def emit(n, v):
                v = v()
                dst[n, c, pl.ds(16 * r, 16), :] = v.astype(bf16)
                if tie and n % 2:
                    before_next(v)
            return _sums2(_sums_a, x, emit)

        def inner(dst, p, product, side, add=False):
            def emit(a, b, v):
                dst[p, 2 * a + b] = dst[p, 2 * a + b] + v if add else v

            def run(k):
                r = product(7 * p + k)
                side()
                return r
            _combine(run, emit)

        def outer(src, r, cols, emit):
            for a in range(2):
                for b in range(2):
                    _combine(lambda p: src[p, 2 * a + b, pl.ds(16 * r, 16), cols],
                             lambda i, j, v: emit(2 * i + a, 2 * j + b, v))
                    yield

        def rows_of(i, g, r):
            return pl.ds(_mult(i * RB + g * R + 16 * r, 16), 16)

        def tied(stages):
            while True:
                try:
                    before_next(next(stages))
                except StopIteration as stop:
                    return stop.value
                yield
                yield

        def last_stats(i, r):
            return tied(h_stats(S - RB + i * R + 16 * r))

        def pre1(i, dst, r):
            for c in range(2):
                x = []
                for g in range(4):
                    rows = rows_of(i, g, r)
                    x.append([(hbuf[2 * k + c, rows, :] - hstat[0, rows, :]) * hstat[2, rows, :]
                              for k in range(4)])
                yield from range(3)
                yield from store_sums(dst, r, c, x)

        def post1(i, src, r):
            def emit(g, j, v):
                v = _gelu_of_double(v)
                gbuf[2 * j + c, pl.ds(HALO + i * RB + g * R + 16 * r, 16), :] = v
            for c in range(2):
                for _ in outer(src, r, pl.ds(c * 128, 128), emit):
                    yield
                    yield

        def pre2(i, dst, r):
            for c in range(2):
                x = [[gbuf[2 * k + c, pl.ds(HALO + i * RB + g * R + 16 * r + off, 16), :]
                      for k, off in enumerate((-1, 1, -2, 2))] for g in range(4)]
                yield from store_sums(dst, r, c, x)

        def post2(i, src, r):
            def emit(g, j, v):
                rows = rows_of(i, g, r)
                v = v + jnp.concatenate(
                    [(hbuf[c, rows, :] - hstat[0, rows, :]) * hstat[1, rows, :]
                     for c in (2 * j, 2 * j + 1)], axis=1)
                x1[rows, pl.ds(j * C4, C4)] = v
            for _ in outer(src, r, slice(None), emit):
                yield
                yield

        def pre3(i, r):
            for g in range(4):
                rows = rows_of(i, g, r)
                m, rs = yield from tied(_ln_stages(x1[rows, :]))
                ustat[0, rows_of(0, g, r), :] = jnp.broadcast_to(m, (16, 128))
                ustat[1, rows_of(0, g, r), :] = jnp.broadcast_to(0.5 * rs, (16, 128))
                before_next(rs)
                yield
                yield

        def sums3(i, tie, r):
            for c in range(2):
                x = [[(x1[rows_of(i, g, r), pl.ds(k * C4 + c * 128, 128)]
                       - ustat[0, rows_of(0, g, r), :]) * ustat[1, rows_of(0, g, r), :]
                      for k in range(4)] for g in range(4)]
                yield from store_sums(yc, r, c, x, tie)

        pieces = {pre1: 20, last_stats: 8, post1: 16, pre2: 14, post2: 8, pre3: 16, sums3: 14}

        def spread(stages, slots):
            return _spread([fn(*args, r) for fn, *args in stages for r in range(R // 16)],
                           sum(pieces[fn] for fn, *_ in stages) * (R // 16), slots)

        for c in range(8):
            gbuf[c, pl.ds(0, HALO), :] = jnp.zeros((HALO, 128), f32)
            gbuf[c, pl.ds(HALO + S, HALO), :] = jnp.zeros((HALO, 128), f32)
        first, second = (W1_AT, pre1, post1), (W2_AT, pre2, post2)
        order = [(stage, i - lag) for i in range(NB + 2)
                 for stage, lag in ((first, 0), (second, 2)) if 0 <= i - lag < NB]
        extra = {n: [(last_stats, i)] for i, n in enumerate((0, 4, 6, 8))}
        extra.update({10: [(pre3, 0)], 15: [(sums3, 0, True)]})
        ac, pb = (ac0, ac1), (pb0, pb1)
        spread([(pre1, 0, ac0)], 1)()
        ties.clear()
        for n, ((at, _, _), _) in enumerate(order):
            before = [(post, i, pb[1 - n % 2]) for (_, _, post), i in order[max(n - 1, 0):n]]
            after = [(pre, i, ac[1 - n % 2]) for (_, pre, _), i in order[n + 1:n + 2]]
            stages = before + after if n in (2, 13) else after + before
            side = spread(stages + extra.get(n, []), 47)
            for p in range(7):
                inner(pb[n % 2], p, lambda k: _dot(
                    operand(ac[n % 2], k, (0, 1)), weights(k, at, (C4, 0, C4), (0, 1))), side)
        spread([(post2, NB - 1, pb1)], 1)()

        def out_copy(i):
            rows = pl.ds(_mult(i * RB, RB), RB)
            return pltpu.make_async_copy(obuf.at[rows], out_hbm.at[rows], sems.at[SEM_OUT])

        nb = (nb0, nb1)

        def activate(c, r):
            act = [[None] * 4 for _ in range(4)]

            def emit(g, j, v):
                act[g][j] = _gelu_of_double(v)
            for _ in outer(nb[c % 2], r, slice(None), emit):
                yield
                yield
            yield from store_sums(hc, r, c, act, False)

        pieces[activate] = 15

        def mlp_up():
            for c in range(7):
                side = spread([(activate, c - 1)] if c else [], 49)
                for p in range(7):
                    inner(nb[c % 2], p, lambda n: _dot(
                        operand(yc, n, (0, 1)), weights(n, W3_AT, (C4, 0, C4), (c,))), side)

        def mlp_down(i, stages):
            def down(p, side, k0=0, k1=F4):
                inner(db, p, lambda n: _dot(operand(hc, n, range(k0 // 128, k1 // 128)),
                                            weights(n, W4_AT, (F4, k0, k1 - k0), (0, 1))),
                      side, add=k0 > 0)

            def finish(bi, bj, plus, minus=()):
                for a in range(2):
                    for b in range(2):
                        rows = pl.ds(_mult(i * RB + (2 * bi + a) * R, R), R)
                        cols = pl.ds((2 * bj + b) * C4, C4)
                        v = x1[rows, cols] + jnp.concatenate(
                            [hbuf[4 * bj + 2 * b + c, rows, :] for c in range(2)], axis=1)
                        for p in minus:
                            v = v - db[p, 2 * a + b]
                        for p in plus:
                            v = v + db[p, 2 * a + b]
                        obuf[rows, cols] = v.astype(bf16)

            down(0, spread([(activate, 6)], 6), 0, F4 - 128)
            down(0, lambda: None, F4 - 128)
            side = spread(stages, 35)
            for p in range(1, 7):
                down(p, side)
                if p == 3:
                    finish(0, 1, (1, 2))
                if p == 5:
                    finish(0, 0, (0, 3, 4), (1,))
            finish(1, 0, (4, 5))
            finish(1, 1, (2, 3, 6), (5,))

        @pl.loop(0, NB)
        def _(i):
            ties.clear()
            mlp_up()
            nxt = jnp.minimum(i + 1, NB - 1)
            mlp_down(i, [(pre3, nxt), (sums3, nxt, False)])
            out_copy(i).start()

        for i in range(NB):
            out_copy(i).wait()

    pl.run_scoped(
        block_b,
        pltpu.VMEM((8, S + 2 * HALO, 128), f32),
        pltpu.VMEM((2, RB, 128), f32),
        pltpu.VMEM((S, D), f32),
        pltpu.VMEM((S, D), bf16),
        pltpu.VMEM((49, 2, R, 128), bf16),
        pltpu.VMEM((49, 7, R, 128), bf16),
        pltpu.VMEM((7, 4, R, C4), f32),
        *[pltpu.VMEM((7, 4, R, 128), f32)] * 2,
        *[pltpu.VMEM((49, 2, R, 128), bf16)] * 2,
        *[pltpu.VMEM((7, 4, R, C4), f32)] * 2,
    )


@jax.jit
def pallas_sequential_preLN__memory_aug_recurrent_mem_tr__mixer_s_mlp__prompt_kernel(
    A_x: jax.Array,
    A_mem0: jax.Array,
    A_Wq: jax.Array,
    A_Wk: jax.Array,
    A_Wv: jax.Array,
    A_Wo: jax.Array,
    A_seg_len: jax.Array,
    B_x: jax.Array,
    B_w1: jax.Array,
    B_w2: jax.Array,
    B_w3: jax.Array,
    B_w4: jax.Array,
):
    del A_seg_len, B_x
    hbm = pl.BlockSpec(memory_space=pl.ANY)
    vmem = pl.BlockSpec(memory_space=pltpu.VMEM)
    scratch = [
        pltpu.VMEM((8, S, 128), f32),
        pltpu.VMEM((3, S, 128), f32),
        pltpu.SemaphoreType.DMA((NSEM,)),
        pltpu.SMEM((1,), jnp.int32),
    ] + [pltpu.VMEM((4, WROWS, 128), bf16)] * 4 + [pltpu.VMEM((WROWS, 128), bf16)] * 33
    out = pl.pallas_call(
        _kernel,
        out_shape=jax.ShapeDtypeStruct((S, D), A_x.dtype),
        in_specs=[hbm, vmem] + [hbm] * 8,
        out_specs=hbm,
        scratch_shapes=scratch,
        compiler_params=pltpu.CompilerParams(vmem_limit_bytes=128 * 1024 * 1024),
    )(A_x.reshape(NSEG, SEG, D), A_mem0.reshape(MEM, D),
      A_Wq.reshape(2, 2, C4, 4, 8, DH), A_Wk.reshape(2, 2, C4, 4, 8, DH),
      A_Wv.reshape(2, 2, C4, 4, 8, DH),
      A_Wo.reshape(H * DH // 8, 8, 8, 128).transpose(0, 2, 1, 3).reshape(4, 2, WO_ROWS, 128),
      B_w1.reshape(4, C4, D), B_w2.reshape(4, C4, D),
      B_w3.reshape(4, C4, F), B_w4.reshape(4, F4, D))
    return out.reshape(A_x.shape)
```

```python
import functools
import itertools

import jax
import jax.numpy as jnp
from jax import lax
import jax.experimental.pallas as pl
import jax.experimental.pallas.tpu as pltpu

S = 2048
D = 1024
H = 32
DH = 128
MEM = 8
SEG = 32
F = 3584
NSEG = S // SEG
NP = H // 2
HD = D // 2
C4 = D // 4
F4 = F // 4
HALO = 8
R = 64
RB = 4 * R
NB = S // RB
EPS = 1e-5
NEG = -1000000000.0
LOG2E = 1.4426950408889634

W1_AT, W2_AT, W3_AT, W4_AT = 0, 2 * C4, 4 * C4, 11 * C4
WROWS = W4_AT + 2 * F4
WO_ROWS = 4 * DH * 8
WO_AT = WROWS - WO_ROWS
BATCH = ((0,), (1, 2, 3, 4, 5), (6, 7, 8, 9, 10), (11, 12), ())

LAG_QK, LAG_PV, LAG_WO = 2, 4, 6
FILL_AT = (14, 18)

bf16 = jnp.bfloat16
f32 = jnp.float32
u32 = jnp.uint32

SEM_XP, SEM_X, SEM_WO, SEM_STRIP, SEM_OUT, SEM_W, SEM_W0, NSEM = 0, 8, 10, 11, 12, 13, 16, 20


def _mult(i, n):
    return i if isinstance(i, int) else pl.multiple_of(i, n)


def _ln(x):
    d = x - jnp.mean(x, axis=-1, keepdims=True)
    return d * lax.rsqrt(jnp.mean(d * d, axis=-1, keepdims=True) + EPS)


def _ln_stages(x):
    m = jnp.mean(x, axis=-1, keepdims=True)
    yield m
    d = x - m
    return m, lax.rsqrt(jnp.mean(d * d, axis=-1, keepdims=True) + EPS)


def _gelu_of_double(y):
    c = 0.7978845608028654
    return y + y * jnp.tanh(y * (2 * c + (8 * c * 0.044715) * (y * y)))


def _dot(a, b):
    return jnp.dot(a, b, preferred_element_type=f32)


def _load(ref, *idx, r0=0, n=None):
    n = ref.shape[-2] if n is None else n
    return pltpu.bitcast(
        ref.bitcast(u32)[(*idx, pl.ds(r0 // 2, n // 2), slice(None))], bf16)


def _sums_a(a11, a12, a21, a22):
    return [lambda: a12 - a22, lambda: a11 + a12, lambda: a11, lambda: a11 + a22,
            lambda: a22, lambda: a21 + a22, lambda: a21 - a11]


def _sums_b(b11, b12, b21, b22):
    return [lambda: b21 + b22, lambda: b22, lambda: b12 - b22, lambda: b11 + b22,
            lambda: b21 - b11, lambda: b11, lambda: b11 + b12]


def _combine(product, emit):
    c11 = product(0)
    c12 = product(1)
    c11 = c11 - c12
    c22 = product(2)
    emit(0, 1, c12 + c22)
    t = product(3)
    c11 = c11 + t
    c22 = c22 + t
    c21 = product(4)
    emit(0, 0, c11 + c21)
    t = product(5)
    emit(1, 0, c21 + t)
    c22 = c22 - t
    emit(1, 1, c22 + product(6))


def _sums2(sums, x, emit):
    outer = [sums(x[i][j], x[i][2 + j], x[2 + i][j], x[2 + i][2 + j])
             for i in range(2) for j in range(2)]
    for p in range(7):
        for q, v in enumerate(sums(*(o[p]() for o in outer))):
            emit(7 * p + q, v)
        yield


def _spread(tasks, pieces, slots):
    todo = itertools.chain(*tasks)
    calls = itertools.count(1)

    def advance():
        k = next(calls)
        if k > slots:
            return
        for _ in range(pieces * k // slots - pieces * (k - 1) // slots):
            next(todo)
        if k == slots:
            assert next(todo, todo) is todo
    return advance


def _tie(never, words, values):
    regs = [[w[r:r + 8] for r in range(0, w.shape[0], 8)] for w in words]
    per = len(regs[0])
    for n, v in enumerate(values):
        c, r = divmod(len(regs) * per * n // len(values), per)
        regs[c][r] = jnp.where(never, pltpu.bitcast(v, u32), regs[c][r])
    return [jnp.concatenate(w, axis=0) for w in regs] if values else words


def _upper_operands(a11, a12, a22):
    k = a11.shape[0] - a22.shape[0]
    ops = [jnp.concatenate([a12[:k], a12[k:] - a22], axis=0), a11 + a12, a11,
           jnp.concatenate([a11[:k], a11[k:] + a22], axis=0)]
    return [v.astype(bf16) for v in ops]


PLAIN = {40: 0, 36: 1, 12: 2, 8: 3}
OTHER = [n for n in range(49) if n not in PLAIN]
RAW_SLOT = dict(zip(OTHER[2::3], [(k, j) for k in range(4) for j in range(4) if k != j]))
RAW_SLOT.update({n: (k, k) for n, k in PLAIN.items()})


def _kernel(x_hbm, mem0_ref, wq_hbm, wk_hbm, wv_hbm, wo_hbm, w1_hbm, w2_hbm,
            w3_hbm, w4_hbm, out_hbm, hbuf, hstat, sems, zero_ref, *wbufs):
    zero_ref[0] = 0
    raw, spare = wbufs[:4], wbufs[4:]
    wsum = {n: (raw[j], k) for n, (k, j) in RAW_SLOT.items()}
    wsum.update({n: (b,) for n, b in zip((n for n in OTHER if n not in RAW_SLOT), spare)})

    def load_h(rows):
        return jnp.concatenate([hbuf[c, rows, :] for c in range(8)], axis=1)

    def h_stats(r0):
        rows = pl.ds(_mult(r0, 16), 16)
        hv = load_h(rows)
        m1, r1 = yield from _ln_stages(hv)
        yield r1
        m2, r2 = yield from _ln_stages((hv - m1) * r1)
        stats = (m1 + m2 / r1, r1, 0.5 * r1 * r2)
        for k, v in enumerate(stats):
            hstat[k, rows, :] = jnp.broadcast_to(v, (16, 128))
        yield stats[0] + stats[2]

    def strip_copies(batch):
        strips = [(w, at + u * w.shape[1], u)
                  for w, at in ((w1_hbm, W1_AT), (w2_hbm, W2_AT), (w3_hbm, W3_AT), (w4_hbm, W4_AT))
                  for u in range(w.shape[2] // 512)]
        return [pltpu.make_async_copy(
            w.at[:, :, pl.ds(j * (w.shape[2] // 4) + u * 128, 128)],
            raw[j].at[:, pl.ds(at, w.shape[1]), :], sems.at[SEM_STRIP])
            for w, at, u in (strips[n] for n in BATCH[batch]) for j in range(4)]

    def weight_sums(r0):
        x = [[raw[j][k, pl.ds(_mult(r0, 16), 16), :].astype(f32) for j in range(4)]
             for k in range(4)]

        def emit(n, v):
            if n not in PLAIN:
                ref, *idx = wsum[n]
                ref[(*idx, pl.ds(_mult(r0, 16), 16), slice(None))] = v().astype(bf16)
        yield from _sums2(_sums_b, x, emit)

    def block_a(xb, xn, lo, *bufs):
        w_on, low, wo_s = bufs[0:3], bufs[3:6], bufs[6:13]
        w_hbm = (wq_hbm, wk_hbm, wv_hbm)
        stage = hbuf.reshape(8, S // 8, 8, DH)
        lhs = spare[:3]
        w_low = [spare[3 + 3 * m:6 + 3 * m] for m in range(3)]

        def x_copy(i):
            return pltpu.make_async_copy(x_hbm.at[pl.ds(2 * i, 2)], xb.at[i & 3],
                                         sems.at[SEM_X + (i & 1)])

        def wo_copies(g):
            return [pltpu.make_async_copy(
                wo_hbm.at[g, duo], raw[duo].at[g, pl.ds(WO_AT, WO_ROWS)], sems.at[SEM_WO])
                for duo in range(2)]

        def chunk_copies(g, m, rows=slice(None), sem=None):
            src = w_hbm[m].bitcast(f32)
            return [pltpu.make_async_copy(
                src.at[half, :, rows, g],
                stage.at[pl.ds(2 * m, 2), rows, pl.ds(4 * half, 4), :],
                sems.at[SEM_W + m if sem is None else sem]) for half in range(2)]

        def start(copies):
            for c in copies:
                c.start()

        def wait(copies):
            for c in copies:
                c.wait()

        def qkv_sums(g, m, duo, d0):
            lower, done = [], []
            for part in range(2):
                for pair in (2 * duo, 2 * duo + 1):
                    b = []
                    for half in range(2):
                        rows = pl.ds(8 * d0 + 4 * half + pair, 16, stride=8)
                        w = pltpu.bitcast(hbuf[2 * m + part, rows, :], u32)
                        b += [pltpu.bitcast(w << 16, f32),
                              pltpu.bitcast(w & jnp.uint32(0xFFFF0000), f32)]
                    sums = [v() for v in _sums_b(*b)]
                    for k in range(4):
                        w_on[m][4 * g + pair, k, pl.ds(_mult(part * C4 + d0, 16), 16), :] = (
                            sums[k].astype(bf16))
                    lower.append(sums[4:])
                    done.append(sums[3])
            for k in range(3):
                for q, v in enumerate(_sums_b(*(b[k] for b in lower))):
                    v = v()
                    rows = pl.ds(_mult((7 * duo + q) * C4 + d0, 16), 16)
                    w_low[m][k][rows, :] = v.astype(bf16)
                done.append(v)
            return done

        def wo_sums(g, pair, e0, n0):
            at = WO_AT + pair % 2 * 16 * DH + 8 * e0 + 8 * n0
            tiles = [[raw[pair // 2][g, pl.ds(at + 8 * DH * i + 32 * j + 64 * r, 16), :]
                      .astype(f32) for r in range(2)] for i in range(2) for j in range(2)]
            done = []
            for n in range(2):
                b = [jnp.concatenate([v[8 * n:8 * n + 8] for v in t], axis=0) for t in tiles]
                for k, v in enumerate(_sums_b(*b)):
                    v = v()
                    wo_s[k][n0 + n, 4 * g + pair, pl.ds(e0, 16), :] = v.astype(bf16)
                done.append(v)
            return done

        def prologue(xpb):
            def xp_copy(i):
                segs = pl.ds(8 * i, 8)
                return pltpu.make_async_copy(x_hbm.at[segs, pl.ds(16, 16), :], xpb.at[segs],
                                             sems.at[SEM_XP + i])

            def first_chunk(i):
                return chunk_copies(0, 0, pl.ds(64 * i, 64), SEM_W0 + i)

            start([xp_copy(i) for i in range(NSEG // 8)])
            for i in range(4):
                start(first_chunk(i))
            start(chunk_copies(0, 1))
            start(chunk_copies(0, 2))
            lo[...] = jnp.zeros(lo.shape, f32)
            for duo in range(2):
                raw[duo][3, pl.ds(WO_AT, WO_ROWS), :] = jnp.zeros((WO_ROWS, 128), bf16)

            @pl.loop(0, NSEG // 8)
            def _(i):
                xp_copy(i).wait()
                for j in range(2):
                    ops = []
                    for n in range(2):
                        a = [_ln(xpb[8 * i + 4 * j + 2 * n + k].astype(f32))
                             for k in range(2)]
                        a1 = jnp.concatenate([a[0][:8], a[1][:8]], axis=0)
                        a2 = jnp.concatenate([a[0][8:], a[1][8:]], axis=0)
                        sums = _sums_a(a1[:, :HD], a1[:, HD:], a2[:, :HD], a2[:, HD:])
                        ops.append([v() for v in sums[4:]])
                    for k in range(3):
                        top, bottom = ops[0][k], ops[1][k]
                        for q, v in enumerate(_sums_a(top[:, :C4], top[:, C4:],
                                                      bottom[:, :C4], bottom[:, C4:])):
                            v = v()
                            for c in range(2):
                                r0 = (2 * q + c) * 4 * NSEG + 32 * i + 16 * j
                                lhs[k][pl.ds(pl.multiple_of(r0, 16), 16), :] = (
                                    v[:, c * 128:(c + 1) * 128].astype(bf16))

            @pl.loop(0, 4)
            def _(i):
                wait(first_chunk(i))
                for duo in range(2):
                    for d0 in range(0, 64, 16):
                        qkv_sums(0, 0, duo, 64 * i + d0)

        pl.run_scoped(prologue, pltpu.VMEM((NSEG, 16, D), bf16))

        def lower_products(g, m):
            m1 = (m + 1) % 3
            never = jnp.full((8, 128), zero_ref[0]) != 0
            g1 = jnp.minimum(g + (1 if m == 2 else 0), 3)
            side = [functools.partial(qkv_sums, g1, m1, duo, d0)
                    for duo in range(2) for d0 in range(0, C4, 16)]
            wait_at = 16
            span = 42 - wait_at
            early = [functools.partial(wo_sums, (g + 3) & 3, pair, e0, n0)
                     for pair in range(4 if m == 2 else 0)
                     for e0 in range(0, DH, 16) for n0 in (0, 2)]

            def product(duo, k, q):
                j = 21 * duo + 7 * k + q
                if j >= wait_at:
                    todo = side[len(side) * (j - wait_at) // span:
                                len(side) * (j - wait_at + 1) // span]
                else:
                    todo = early[len(early) * j // wait_at:len(early) * (j + 1) // wait_at]
                a = [lhs[k].bitcast(u32)[pl.ds((2 * q + c) * 2 * NSEG, 2 * NSEG), :]
                     for c in range(2)]
                a[1:] = _tie(never, a[1:], [v[8:] for fn in todo for v in fn()])
                a = jnp.concatenate([pltpu.bitcast(v, bf16) for v in a], axis=1)
                res = _dot(a, _load(w_low[m][k], r0=(7 * duo + q) * C4, n=C4))
                if j == wait_at - 1:
                    pl.when(3 * g + m < 11)(lambda: wait(chunk_copies(g1, m1)))
                    pl.when(g < 3)(lambda: start(chunk_copies(g + 1, m)))
                    if m == 1:
                        pl.when(g > 0)(lambda: wait(wo_copies(g - 1)))
                        start(wo_copies(g))
                        pl.when(g == 3)(
                            lambda: start([x_copy(0), x_copy(1)] + strip_copies(0)))
                return res

            for duo in range(2):
                last = {}
                for k in range(3):
                    def emit(a, b, res):
                        v = res if k == 0 else res + last[a, b] if k == 1 else res - last[a, b]
                        last[a, b] = res
                        for n in range(NSEG // 4):
                            low[m][2 * n + a, 4 * g + 2 * duo + b, k] = (
                                v[16 * n:16 * n + 16].astype(bf16))
                    _combine(functools.partial(product, duo, k), emit)

        @pl.loop(0, 4)
        def _(g):
            for m in range(3):
                lower_products(g, m)

        def norm_tokens(i, k):
            for r0 in range(0, SEG, 16):
                v = xb[jnp.minimum(i, NSEG // 2 - 1) & 3, k, pl.ds(r0, 16), :].astype(f32)
                m, r = yield from _ln_stages(v)
                xn[k, pl.ds(r0, 16), :] = (v - m) * r
                yield r

        def lower_wo(grp, n, k):
            w = jnp.concatenate([_load(wo_s[4 + k], n, t) for t in range(NP)], axis=0)
            return _dot(lo[grp & 1, k].astype(bf16), w)

        def add_lower(grp, n, m4, m2, m6):
            for j in range(4):
                seg = slice(8 * j, 8 * j + 8)
                upper = pl.ds(_mult((4 * grp + j) * SEG + 16, 8), 8)
                lower = pl.ds(_mult((4 * grp + j) * SEG + 24, 8), 8)
                hbuf[n, upper, :] += m4[seg]
                hbuf[n, lower, :] += m2[seg] + m4[seg]
                hbuf[4 + n, lower, :] += m6[seg] - m2[seg]

        def attention_mask():
            def split(axis):
                r = lax.broadcasted_iota(jnp.int32, (80, 80), axis)
                return (jnp.where(r < 64, r >> 5, (r - 64) >> 3),
                        jnp.where(r < 64, r & 31, 32 + (r & 7)))
            (hq, pq), (hk, pk) = split(0), split(1)
            visible = (pq < MEM) | (pq >= pk)
            return jnp.where(hq == hk, jnp.where(visible, 0.0, NEG * DH ** 0.5), -jnp.inf)

        def step(i, k, mem, fill, side):
            tok = xn[k]
            r0 = jnp.maximum(2 * i + k - 8, 0) * SEG
            norms = itertools.chain(h_stats(r0), h_stats(r0 + 16), norm_tokens(i + 1, k))
            s = 2 * i + k
            a1 = jnp.concatenate([mem, tok[:24]], axis=0)
            ops = _upper_operands(a1[:, :HD], a1[:, HD:], tok[24:, HD:])
            qkvs, scores, outs, lower = {}, {}, {}, []
            total = [None] * 4

            def qkv(t):
                res = []
                for m in range(3):
                    m7, m5, m3, m1 = [_dot(ops[j], _load(w_on[m], t, j)) for j in range(4)]
                    m4, c21, m62 = [
                        _load(low[m], i, t, j).astype(f32)[8 * k:8 * k + 8]
                        for j in range(3)]
                    side()
                    c11 = m7 - m5 + m1
                    res.append(jnp.concatenate(
                        [c11[:24], c11[24:] + m4, m5 + m3, c21, m3[24:] + m62 + m1[24:]],
                        axis=0).astype(bf16))
                qkvs[t] = res

            def qk(t):
                q, kk, v = qkvs.pop(t)
                sc = lax.dot_general(q, kk, (((1,), (1,)), ((), ())),
                                     preferred_element_type=f32)
                scores[t] = (sc, v)

            def pv(t):
                sc, v = scores.pop(t)
                sc = jnp.where(fill == 0.0, sc, fill)
                tie = next(norms, None) if t >= 1 else None
                if tie is not None:
                    sc = jnp.concatenate([jnp.where(never, tie, sc[:16]), sc[16:]], axis=0)
                mx = jnp.max(sc, axis=1, keepdims=True)
                e = jnp.exp2((sc - mx) * (DH ** -0.5 * LOG2E))
                den = jnp.sum(e, axis=1, keepdims=True)
                inv = pl.reciprocal(den, approx=True)
                inv = inv * (2.0 - den * inv)
                outs[t] = _dot(e.astype(bf16), v) * inv

            def wo(t):
                o = outs.pop(t)
                a11, a12, a21, a22 = o[:32], o[32:64], o[64:72], o[72:]
                rows = pl.ds(pl.multiple_of(8 * (s & 3), 8), 8)
                for j, v in enumerate((a22, a21 + a22, a21 - a11[24:])):
                    lo[(s >> 2) & 1, j, rows, pl.ds(t * DH, DH)] = v
                for j, a in enumerate(_upper_operands(a11, a12, a22)):
                    r = _dot(a, jnp.concatenate(
                        [_load(wo_s[j], n, t) for n in range(4)], axis=1))
                    total[j] = r if total[j] is None else total[j] + r

            for t in range(NP + LAG_WO):
                if t < NP:
                    qkv(t)
                if t in FILL_AT:
                    lower.append(lower_wo((s >> 2) - 1, s & 3, len(lower)))
                if t % 2:
                    for fn, lag in ((qk, LAG_QK), (pv, LAG_PV)):
                        for u in (t - 1 - lag, t - lag):
                            if 0 <= u < NP:
                                fn(u)
                if t >= LAG_WO:
                    wo(t - LAG_WO)

            m7, m5, m3, m1 = total
            upper = jnp.concatenate([m7 - m5 + m1, m5 + m3], axis=1)
            c22 = m3[24:] + m1[24:]
            xv = xb[i & 3, k].astype(f32)
            hv = jnp.concatenate(
                [xv[:24] + upper[MEM:],
                 jnp.concatenate([xv[24:, :HD], xv[24:, HD:] + c22], axis=1)], axis=0)
            for c in range(8):
                hbuf[c, pl.ds(pl.multiple_of(s * SEG, SEG), SEG), :] = hv[:, c * 128:(c + 1) * 128]
            add_lower(jnp.maximum((s >> 2) - 1, 0), s & 3,
                      *lower, lower_wo((s >> 2) - 1, s & 3, 2))
            return upper[:MEM]

        fill = attention_mask()
        never = jnp.full((16, 80), zero_ref[0]) != 0
        n_it = NSEG // 2
        per_it = WROWS // 16 // n_it

        def steps(i, mem):
            pl.when(i + 1 < n_it)(lambda: x_copy(i + 1).wait())
            pl.when(i + 2 < n_it)(lambda: x_copy(i + 2).start())

            @pl.when(i < len(BATCH) - 1)
            def _():
                for b in range(len(BATCH) - 1):
                    @pl.when(i == b)
                    def _():
                        wait(strip_copies(b))
                        start(strip_copies(b + 1))

            side = _spread([weight_sums(16 * (per_it * i + j)) for j in range(per_it)],
                           7 * per_it, 94)
            for k in range(2):
                mem = step(i, k, mem, fill, side)
            return mem

        wait(wo_copies(3) + [x_copy(0)])
        for pair in range(4):
            for e0 in range(0, DH, 16):
                for n0 in (0, 2):
                    wo_sums(3, pair, e0, n0)
        hbuf[:, pl.ds(0, 4 * SEG), :] = jnp.zeros((8, 4 * SEG, 128), f32)
        _spread([norm_tokens(0, 0), norm_tokens(0, 1)], 8, 1)()
        lax.fori_loop(0, n_it, steps, mem0_ref[...].astype(f32))
        for n in range(4):
            add_lower(NSEG // 4 - 1, n, *(lower_wo(NSEG // 4 - 1, n, k) for k in range(3)))

    pl.run_scoped(
        block_a,
        pltpu.VMEM((4, 2, SEG, D), bf16),
        pltpu.VMEM((2, SEG, D), f32),
        pltpu.VMEM((2, 3, 32, NP * DH), f32),
        *[pltpu.VMEM((NP, 4, HD, DH), bf16)] * 3,
        *[pltpu.VMEM((NSEG // 2, NP, 3, 16, DH), bf16)] * 3,
        *[pltpu.VMEM((4, NP, DH, 128), bf16)] * 7,
    )

    def block_b(gbuf, ustat, x1, obuf, yc, hc, db, nb0, nb1, ac0, ac1, pb0, pb1):
        def weights(n, at, rows, strips):
            return jnp.concatenate(
                [_load(*wsum[n], r0=at + k * rows[0] + rows[1], n=rows[2])
                 for k in strips], axis=1)

        ties = []
        never = jnp.full((8, 128), zero_ref[0]) != 0

        def before_next(value):
            if value.shape[1] == 1:
                value = jnp.broadcast_to(value[:8] + value[8:], (8, 128))
            ties.append(value[-8:, -128:])

        def operand(ref, n, cols):
            words = [ref.bitcast(u32)[n, c] for c in cols]
            words = _tie(never, words, ties)
            ties.clear()
            return jnp.concatenate([pltpu.bitcast(w, bf16) for w in words], axis=1)

        def store_sums(dst, r, c, x, tie=True):
            def emit(n, v):
                v = v()
                dst[n, c, pl.ds(16 * r, 16), :] = v.astype(bf16)
                if tie and n % 2:
                    before_next(v)
            return _sums2(_sums_a, x, emit)

        def inner(dst, p, product, side, add=False):
            def emit(a, b, v):
                dst[p, 2 * a + b] = dst[p, 2 * a + b] + v if add else v

            def run(k):
                r = product(7 * p + k)
                side()
                return r
            _combine(run, emit)

        def outer(src, r, cols, emit):
            for a in range(2):
                for b in range(2):
                    _combine(lambda p: src[p, 2 * a + b, pl.ds(16 * r, 16), cols],
                             lambda i, j, v: emit(2 * i + a, 2 * j + b, v))
                    yield

        def rows_of(i, g, r):
            return pl.ds(_mult(i * RB + g * R + 16 * r, 16), 16)

        def tied(stages):
            while True:
                try:
                    before_next(next(stages))
                except StopIteration as stop:
                    return stop.value
                yield
                yield

        def last_stats(i, r):
            return tied(h_stats(S - RB + i * R + 16 * r))

        def pre1(i, dst, r):
            for c in range(2):
                x = []
                for g in range(4):
                    rows = rows_of(i, g, r)
                    x.append([(hbuf[2 * k + c, rows, :] - hstat[0, rows, :]) * hstat[2, rows, :]
                              for k in range(4)])
                yield from range(3)
                yield from store_sums(dst, r, c, x)

        def post1(i, src, r):
            def emit(g, j, v):
                r0 = HALO + i * RB + g * R + 16 * r + (1, -1, 2, -2)[j]
                gbuf[2 * j + c, pl.ds(r0, 16), :] = _gelu_of_double(v)
            for c in range(2):
                for _ in outer(src, r, pl.ds(c * 128, 128), emit):
                    yield
                    yield

        def pre2(i, dst, r):
            for c in range(2):
                x = [[gbuf[2 * k + c, pl.ds(HALO + i * RB + g * R + 16 * r, 16), :]
                      for k in range(4)] for g in range(4)]
                yield from store_sums(dst, r, c, x)

        def post2(i, src, r):
            def emit(g, j, v):
                rows = rows_of(i, g, r)
                v = v + jnp.concatenate(
                    [(hbuf[c, rows, :] - hstat[0, rows, :]) * hstat[1, rows, :]
                     for c in (2 * j, 2 * j + 1)], axis=1)
                x1[rows, pl.ds(j * C4, C4)] = v
            for _ in outer(src, r, slice(None), emit):
                yield
                yield

        def pre3(i, r):
            for g in range(4):
                rows = rows_of(i, g, r)
                m, rs = yield from tied(_ln_stages(x1[rows, :]))
                ustat[0, rows_of(0, g, r), :] = jnp.broadcast_to(m, (16, 128))
                ustat[1, rows_of(0, g, r), :] = jnp.broadcast_to(0.5 * rs, (16, 128))
                before_next(rs)
                yield
                yield

        def sums3(i, tie, r):
            for c in range(2):
                x = [[(x1[rows_of(i, g, r), pl.ds(k * C4 + c * 128, 128)]
                       - ustat[0, rows_of(0, g, r), :]) * ustat[1, rows_of(0, g, r), :]
                      for k in range(4)] for g in range(4)]
                yield from store_sums(yc, r, c, x, tie)

        pieces = {pre1: 20, last_stats: 8, post1: 16, pre2: 14, post2: 8, pre3: 16, sums3: 14}

        def spread(stages, slots):
            return _spread([fn(*args, r) for fn, *args in stages for r in range(R // 16)],
                           sum(pieces[fn] for fn, *_ in stages) * (R // 16), slots)

        for c in range(8):
            gbuf[c, pl.ds(HALO, HALO), :] = jnp.zeros((HALO, 128), f32)
            gbuf[c, pl.ds(S, HALO), :] = jnp.zeros((HALO, 128), f32)
        first, second = (W1_AT, pre1, post1), (W2_AT, pre2, post2)
        order = [(stage, i - lag) for i in range(NB + 2)
                 for stage, lag in ((first, 0), (second, 2)) if 0 <= i - lag < NB]
        extra = {n: [(last_stats, i)] for i, n in enumerate((0, 4, 6, 8))}
        extra.update({10: [(pre3, 0)], 15: [(sums3, 0, True)]})
        ac, pb = (ac0, ac1), (pb0, pb1)
        spread([(pre1, 0, ac0)], 1)()
        ties.clear()
        for n, ((at, _, _), _) in enumerate(order):
            before = [(post, i, pb[1 - n % 2]) for (_, _, post), i in order[max(n - 1, 0):n]]
            after = [(pre, i, ac[1 - n % 2]) for (_, pre, _), i in order[n + 1:n + 2]]
            stages = before + after if n in (2, 13) else after + before
            side = spread(stages + extra.get(n, []), 47)
            for p in range(7):
                inner(pb[n % 2], p, lambda k: _dot(
                    operand(ac[n % 2], k, (0, 1)), weights(k, at, (C4, 0, C4), (0, 1))), side)
        spread([(post2, NB - 1, pb1)], 1)()

        def out_copy(i):
            rows = pl.ds(_mult(i * RB, RB), RB)
            return pltpu.make_async_copy(obuf.at[rows], out_hbm.at[rows], sems.at[SEM_OUT])

        nb = (nb0, nb1)

        def activate(c, r):
            act = [[None] * 4 for _ in range(4)]

            def emit(g, j, v):
                act[g][j] = _gelu_of_double(v)
            for _ in outer(nb[c % 2], r, slice(None), emit):
                yield
                yield
            yield from store_sums(hc, r, c, act, False)

        pieces[activate] = 15

        def mlp_up():
            for c in range(7):
                side = spread([(activate, c - 1)] if c else [], 49)
                for p in range(7):
                    inner(nb[c % 2], p, lambda n: _dot(
                        operand(yc, n, (0, 1)), weights(n, W3_AT, (C4, 0, C4), (c,))), side)

        def mlp_down(i, stages):
            def down(p, side, k0=0, k1=F4):
                inner(db, p, lambda n: _dot(operand(hc, n, range(k0 // 128, k1 // 128)),
                                            weights(n, W4_AT, (F4, k0, k1 - k0), (0, 1))),
                      side, add=k0 > 0)

            def finish(bi, bj, plus, minus=()):
                for a in range(2):
                    for b in range(2):
                        rows = pl.ds(_mult(i * RB + (2 * bi + a) * R, R), R)
                        cols = pl.ds((2 * bj + b) * C4, C4)
                        v = x1[rows, cols] + jnp.concatenate(
                            [hbuf[4 * bj + 2 * b + c, rows, :] for c in range(2)], axis=1)
                        for p in minus:
                            v = v - db[p, 2 * a + b]
                        for p in plus:
                            v = v + db[p, 2 * a + b]
                        obuf[rows, cols] = v.astype(bf16)

            down(0, spread([(activate, 6)], 6), 0, F4 - 128)
            down(0, lambda: None, F4 - 128)
            side = spread(stages, 35)
            for p in range(1, 7):
                down(p, side)
                if p == 3:
                    finish(0, 1, (1, 2))
                if p == 5:
                    finish(0, 0, (0, 3, 4), (1,))
            finish(1, 0, (4, 5))
            finish(1, 1, (2, 3, 6), (5,))

        @pl.loop(0, NB)
        def _(i):
            ties.clear()
            mlp_up()
            nxt = jnp.minimum(i + 1, NB - 1)
            mlp_down(i, [(pre3, nxt), (sums3, nxt, False)])
            out_copy(i).start()

        for i in range(NB):
            out_copy(i).wait()

    pl.run_scoped(
        block_b,
        pltpu.VMEM((8, S + 2 * HALO, 128), f32),
        pltpu.VMEM((2, RB, 128), f32),
        pltpu.VMEM((S, D), f32),
        pltpu.VMEM((S, D), bf16),
        pltpu.VMEM((49, 2, R, 128), bf16),
        pltpu.VMEM((49, 7, R, 128), bf16),
        pltpu.VMEM((7, 4, R, C4), f32),
        *[pltpu.VMEM((7, 4, R, 128), f32)] * 2,
        *[pltpu.VMEM((49, 2, R, 128), bf16)] * 2,
        *[pltpu.VMEM((7, 4, R, C4), f32)] * 2,
    )


@jax.jit
def pallas_sequential_preLN__memory_aug_recurrent_mem_tr__mixer_s_mlp__prompt_kernel(
    A_x: jax.Array,
    A_mem0: jax.Array,
    A_Wq: jax.Array,
    A_Wk: jax.Array,
    A_Wv: jax.Array,
    A_Wo: jax.Array,
    A_seg_len: jax.Array,
    B_x: jax.Array,
    B_w1: jax.Array,
    B_w2: jax.Array,
    B_w3: jax.Array,
    B_w4: jax.Array,
):
    del A_seg_len, B_x
    hbm = pl.BlockSpec(memory_space=pl.ANY)
    vmem = pl.BlockSpec(memory_space=pltpu.VMEM)
    scratch = [
        pltpu.VMEM((8, S, 128), f32),
        pltpu.VMEM((3, S, 128), f32),
        pltpu.SemaphoreType.DMA((NSEM,)),
        pltpu.SMEM((1,), jnp.int32),
    ] + [pltpu.VMEM((4, WROWS, 128), bf16)] * 4 + [pltpu.VMEM((WROWS, 128), bf16)] * 33
    out = pl.pallas_call(
        _kernel,
        out_shape=jax.ShapeDtypeStruct((S, D), A_x.dtype),
        in_specs=[hbm, vmem] + [hbm] * 8,
        out_specs=hbm,
        scratch_shapes=scratch,
        compiler_params=pltpu.CompilerParams(vmem_limit_bytes=128 * 1024 * 1024),
    )(A_x.reshape(NSEG, SEG, D), A_mem0.reshape(MEM, D),
      A_Wq.reshape(2, 2, C4, 4, 8, DH), A_Wk.reshape(2, 2, C4, 4, 8, DH),
      A_Wv.reshape(2, 2, C4, 4, 8, DH),
      A_Wo.reshape(H * DH // 8, 8, 8, 128).transpose(0, 2, 1, 3).reshape(4, 2, WO_ROWS, 128),
      B_w1.reshape(4, C4, D), B_w2.reshape(4, C4, D),
      B_w3.reshape(4, C4, F), B_w4.reshape(4, F4, D))
    return out.reshape(A_x.shape)
```
